```python
import jax
import jax.numpy as jnp

def _softmax(x, axis=-1):
    return jax.nn.softmax(x, axis=axis)
def _gelu(x):
    return jax.nn.gelu(x, approximate=True)
def _silu(x):
    return jax.nn.silu(x)
def _sigmoid(x):
    return jax.nn.sigmoid(x)
def _layernorm(x, axis=-1, eps=1e-5):
    m = jnp.mean(x, axis=axis, keepdims=True)
    v = jnp.var(x, axis=axis, keepdims=True)
    return (x - m) / jnp.sqrt(v + eps)
def _scatter_add(tgt, idx, src, axis=0):
    return tgt.at[idx].add(src)
def _segment_sum(src, seg, n):
    return jax.ops.segment_sum(src, seg, n)
class _Rng:
    def __init__(self, key):
        self._k = key
    def _next(self):
        self._k, sub = jax.random.split(self._k)
        return sub
    def normal(self, shape):
        return jax.random.normal(self._next(), shape, dtype=jnp.bfloat16)
    def randint(self, lo, hi, shape):
        return jax.random.randint(self._next(), shape, lo, hi, dtype=jnp.int32)
    def uniform(self, shape, lo=0.0, hi=1.0):
        return jax.random.uniform(self._next(), shape, jnp.bfloat16, lo, hi)
    def permutation(self, n):
        return jax.random.permutation(self._next(), n)


kernel_name = 'interleave_layers__sliding_local_dilated__dense_activation_mish__prompt'

def setup_inputs():
    _rng = _Rng(jax.random.key(int.from_bytes(__import__("os").urandom(4), "little")))
    _w = (lambda a: (lambda t: t.astype(jnp.bfloat16) if jnp.issubdtype(t.dtype, jnp.floating) else t)(jnp.asarray(a)))
    def _A_setup():
        B, S, D = 1, 2048, 1024
        return {
            "x": _w((lambda *s: _rng.normal(s) * 0.05)(B, S, D)),
            "wqkv": _w((lambda *s: _rng.normal(s) * 0.05)(D, 3 * D)),
            "wo": _w((lambda *s: _rng.normal(s) * 0.05)(D, D)),
        }
    _A_in = _A_setup()

    def _B_setup():
        B, S, D, F = 1, 2048, 1024, 3584
        return {
            "x": _w((lambda *s: _rng.normal(s) * 0.05)(B, S, D)),
            "w1": _w((lambda *s: _rng.normal(s) * 0.05)(D, F) * (D ** -0.5)),
            "b1": _w((lambda *s: _rng.normal(s) * 0.05)(F)),
            "w2": _w((lambda *s: _rng.normal(s) * 0.05)(F, D) * (F ** -0.5)),
        }
    _B_in = _B_setup()

    return {
        "A_x": _A_in["x"],
        "A_wqkv": _A_in["wqkv"],
        "A_wo": _A_in["wo"],
        "B_x": _B_in["x"],
        "B_w1": _B_in["w1"],
        "B_b1": _B_in["b1"],
        "B_w2": _B_in["w2"],
    }

def reference(A_x, A_wqkv, A_wo, B_x, B_w1, B_b1, B_w2):
    def _A_ref(x, wqkv, wo):
        B, S, D = x.shape
        H = 32; Dh = D // H
        W, dil = 8, 2
        qkv = (lambda x, *d: x.transpose(*d))((x @ wqkv).reshape(B, S, 3, H, Dh), 2, 0, 3, 1, 4)
        q, k, v = qkv[0], qkv[1], qkv[2]
        scale = Dh ** -0.5
        pos = jnp.arange(S)
        off = jnp.arange(W) * dil
        idx = pos[:, None] - off[None, :]
        mask = idx >= 0
        idx_c = jnp.where(mask, idx, 0).reshape(-1)
        kg = k[:, :, idx_c, :].reshape(B, H, S, W, Dh)
        vg = v[:, :, idx_c, :].reshape(B, H, S, W, Dh)
        logits = jnp.einsum("bhsd,bhswd->bhsw", q, kg) * scale
        logits = jnp.where(mask[None, None, :, :], logits, -1e9)
        attn = _softmax(logits, axis=-1)
        o = jnp.einsum("bhsw,bhswd->bhsd", attn, vg)
        return (lambda x, *d: x.transpose(*d))(o, 0, 2, 1, 3).reshape(B, S, D) @ wo

    def _B_ref(x, w1, b1, w2):
        h = jnp.einsum("bsd,df->bsf", x, w1) + b1
        sp = jnp.log1p(jnp.exp(-jnp.abs(h))) + jnp.where(h > 0, h, jnp.zeros_like(h))
        act = h * jnp.tanh(sp)
        return jnp.einsum("bsf,fd->bsd", act, w2)

    x = A_x
    x = x + _A_ref(_layernorm(x, axis=-1), A_wqkv, A_wo)
    x = x + _B_ref(_layernorm(x, axis=-1), B_w1, B_b1, B_w2)
    x = x + _A_ref(_layernorm(x, axis=-1), A_wqkv, A_wo)
    x = x + _B_ref(_layernorm(x, axis=-1), B_w1, B_b1, B_w2)
    return x
```

```python
import functools
import jax
import jax.numpy as jnp
from jax import lax
import jax.experimental.pallas as pl
import jax.experimental.pallas.tpu as pltpu

S, D, F = 2048, 1024, 3584
H, DH, W, DIL = 32, 32, 8, 2
NG = D // 128
HALO = 16
T = 256
R = 16
EPS = 1e-5
f32, bf16 = jnp.float32, jnp.bfloat16


def _layernorm(x):
    m = jnp.mean(x, axis=-1, keepdims=True)
    xc = x - m
    v = jnp.mean(xc * xc, axis=-1, keepdims=True)
    return xc * lax.rsqrt(v + EPS)


def _permute_lanes(groups):
    shape = groups[0].shape
    lane = lax.broadcasted_iota(jnp.int32, shape, 1)
    mid = [g if j == 7 else pltpu.roll(g, (j - 7) % 128, 1) for j, g in enumerate(groups)]
    for b in (1, 2, 4):
        m = (lane & b) != 0
        mid = [jnp.where(m, mid[(j + b) % 8], mid[j]) for j in range(8)]
    return [g if j == 0 else pltpu.roll(g, j, 1) for j, g in enumerate(mid)]


def _kernel(x_ref, b1_ref, wqkv_hbm, wo_hbm, w1_hbm, w2_hbm, o_ref,
            wqkv_raw, wqkv_p, wo_raw, wo_stage, wo_p, w1_v, w2_v, q_s, k_s, v_s, o_s, sems):
    step = pl.program_id(0)

    @pl.when(step == 0)
    def _():
        cps = [pltpu.make_async_copy(wqkv_hbm, wqkv_raw, sems.at[0]),
               pltpu.make_async_copy(wo_hbm, wo_raw, sems.at[1]),
               pltpu.make_async_copy(w1_hbm, w1_v, sems.at[2]),
               pltpu.make_async_copy(w2_hbm, w2_v, sems.at[3])]
        for c in cps:
            c.start()
        k_s[:, :, 0:HALO, :] = jnp.zeros((2, NG, HALO, 128), f32)
        v_s[:, :, 0:HALO, :] = jnp.zeros((2, NG, HALO, 128), f32)
        cps[0].wait()

        def body(i, c):
            r0 = pl.multiple_of(i * 16, 16)
            for p in range(3):
                blk = pltpu.bitcast(wqkv_raw[pl.ds(r0, 16), p * D:(p + 1) * D], jnp.int32)
                outs = _permute_lanes([blk[:, j * 128:(j + 1) * 128] for j in range(NG)])
                for j in range(NG):
                    wqkv_p[pl.ds(r0, 16), p * D + j * 128:p * D + (j + 1) * 128] = pltpu.bitcast(outs[j], bf16)
            return c
        lax.fori_loop(0, D // 16, body, 0)
        cps[1].wait()
        for g in range(NG):
            wo_stage[g] = wo_raw[:, g * 128:(g + 1) * 128].astype(f32)
        for jp in range(NG):
            for ae in range(0, 16, 2):
                for g in range(NG):
                    lo = wo_stage[g, pl.ds(8 * ae + 7 - jp, 8, stride=128), :]
                    hi = wo_stage[g, pl.ds(8 * (ae + 1) + 7 - jp, 8, stride=128), :]
                    wo_p[jp * 128 + 8 * ae:jp * 128 + 8 * ae + 16, g * 128:(g + 1) * 128] = jnp.concatenate([lo, hi], axis=0).astype(bf16)
        cps[2].wait()
        cps[3].wait()

    @pl.when(step > 0)
    def _():
        k_s[:, :, 0:HALO, :] = k_s[:, :, T:T + HALO, :]
        v_s[:, :, 0:HALO, :] = v_s[:, :, T:T + HALO, :]

    scale = DH ** -0.5
    lane = lax.broadcasted_iota(jnp.int32, (R, 128), 1)
    b3 = (lane & 8) != 0
    b4 = (lane & 16) != 0
    row = lax.broadcasted_iota(jnp.int32, (R, 128), 0) + step * T

    def layer(l, x):
        xn = _layernorm(x).astype(bf16)
        qkv = jnp.dot(xn, wqkv_p[...], preferred_element_type=f32)
        for j in range(NG):
            q_s[j] = qkv[:, j * 128:(j + 1) * 128]
            k_s[l, j, HALO:HALO + T, :] = qkv[:, D + j * 128:D + (j + 1) * 128]
            v_s[l, j, HALO:HALO + T, :] = qkv[:, 2 * D + j * 128:2 * D + (j + 1) * 128]
        for c in range(T // R):
            r0 = c * R
            q = q_s[:, r0:r0 + R, :]
            lg = []
            for w in range(W):
                kw = k_s[l, :, pl.ds(HALO + r0 - DIL * w, R), :]
                p = jnp.sum(q * kw, axis=0)
                p = p + jnp.where(b3, pltpu.roll(p, 8, 1), pltpu.roll(p, 120, 1))
                p = p + jnp.where(b4, pltpu.roll(p, 16, 1), pltpu.roll(p, 112, 1))
                p = p * scale
                if c == 0 and w > 0:
                    p = jnp.where(row >= DIL * w, p, -1e9)
                lg.append(p)
            m = functools.reduce(jnp.maximum, lg)
            e = [jnp.exp(p - m) for p in lg]
            inv = 1.0 / functools.reduce(jnp.add, e)
            a = [t * inv for t in e]
            for j in range(NG):
                acc = a[0] * v_s[l, j, pl.ds(HALO + r0, R), :]
                for w in range(1, W):
                    acc = acc + a[w] * v_s[l, j, pl.ds(HALO + r0 - DIL * w, R), :]
                o_s[r0:r0 + R, j * 128:(j + 1) * 128] = acc.astype(bf16)
        x = x + jnp.dot(o_s[...], wo_p[...], preferred_element_type=f32)
        xn = _layernorm(x).astype(bf16)
        h = jnp.dot(xn, w1_v[...], preferred_element_type=f32) + b1_ref[...].astype(f32)
        ex = jnp.exp(jnp.minimum(h, 30.0))
        n = ex * (ex + 2.0)
        act = (h * n / (n + 2.0)).astype(bf16)
        x = x + jnp.dot(act, w2_v[...], preferred_element_type=f32)
        return x

    x = lax.fori_loop(0, 2, layer, x_ref[...].astype(f32))
    o_ref[...] = x.astype(o_ref.dtype)


@jax.jit
def pallas_interleave_layers__sliding_local_dilated__dense_activation_mish__prompt_kernel(A_x, A_wqkv, A_wo, B_x, B_w1, B_b1, B_w2):
    x = A_x.reshape(S, D)
    b1 = B_b1.reshape(1, F)
    out = pl.pallas_call(
        _kernel,
        grid=(S // T,),
        in_specs=[
            pl.BlockSpec((T, D), lambda i: (i, 0)),
            pl.BlockSpec((1, F), lambda i: (0, 0)),
            pl.BlockSpec(memory_space=pl.ANY),
            pl.BlockSpec(memory_space=pl.ANY),
            pl.BlockSpec(memory_space=pl.ANY),
            pl.BlockSpec(memory_space=pl.ANY),
        ],
        out_specs=pl.BlockSpec((T, D), lambda i: (i, 0)),
        out_shape=jax.ShapeDtypeStruct((S, D), bf16),
        scratch_shapes=[
            pltpu.VMEM((D, 3 * D), bf16), pltpu.VMEM((D, 3 * D), bf16),
            pltpu.VMEM((D, D), bf16), pltpu.VMEM((NG, D, 128), f32), pltpu.VMEM((D, D), bf16),
            pltpu.VMEM((D, F), bf16), pltpu.VMEM((F, D), bf16),
            pltpu.VMEM((NG, T, 128), f32),
            pltpu.VMEM((2, NG, T + HALO, 128), f32), pltpu.VMEM((2, NG, T + HALO, 128), f32),
            pltpu.VMEM((T, D), bf16),
            pltpu.SemaphoreType.DMA((4,)),
        ],
        compiler_params=pltpu.CompilerParams(
            dimension_semantics=("arbitrary",), vmem_limit_bytes=100 * 1024 * 1024),
        name="fused",
    )(x, b1, A_wqkv, A_wo, B_w1, B_w2)
    return out.reshape(1, S, D)
```

```python
import functools
import jax
import jax.numpy as jnp
from jax import lax
import jax.experimental.pallas as pl
import jax.experimental.pallas.tpu as pltpu

S, D, F = 2048, 1024, 3584
H, DH, W, DIL = 32, 32, 8, 2
NG = D // 128
NF = F // 128
HALO = 16
T = 256
C = T // 2
R = 8
NCH = C // R
NB = S // T
NITEM = 2 * NB
SKEW = 2
EPS = 1e-5
f32, bf16, i32 = jnp.float32, jnp.bfloat16, jnp.int32
QA, KA, VA, QB, KB, VB, DUMMY = range(7)
SCHED = (15, 39, 31, 47)


def _layernorm(x):
    m = jnp.mean(x, axis=-1, keepdims=True)
    xc = x - m
    v = jnp.mean(xc * xc, axis=-1, keepdims=True)
    return xc * lax.rsqrt(v + EPS)


def _perm_matrix(j):
    src = lax.broadcasted_iota(i32, (128, 128), 0)
    m = lax.broadcasted_iota(i32, (128, 128), 1)
    jp = (j + 128 - m) & 7
    l = (m + jp) & 127
    want = 32 * ((l >> 3) & 3) + 4 * jp + (l >> 5)
    return jnp.where(src == want, 1.0, 0.0).astype(bf16)


def _exchange_and_roll(mid):
    lane = lax.broadcasted_iota(i32, mid[0].shape, 1)
    for b in (1, 2, 4):
        m = (lane & b) != 0
        mid = [jnp.where(m, mid[(j + b) % 8], mid[j]) for j in range(8)]
    return [g if j == 0 else pltpu.roll(g, j, 1) for j, g in enumerate(mid)]


def _dot(x, w_ref, n):
    w = w_ref[:, n * 128:(n + 1) * 128]
    if w.dtype != bf16:
        w = pltpu.bitcast(w, bf16)
    return jnp.dot(x, w, preferred_element_type=f32)


NWCH = 8
SEM_X, SEM_W, SEM_Q, SEM_O, NSEM = 0, NB, NB + 3, NB + 3 + NWCH, 2 * NB + 3 + NWCH
PITCH = 129


def _kernel(x_hbm, b1_ref, wqkv_hbm, wo_hbm, w1_hbm, w2_hbm, out_hbm,
            wqkv_raw, wqkv_p, wo_raw, wo_stage, pm, wo_p, w1_v, w2_v,
            xs, xn1, xn2, att, o_a, o_b, hk, hv, zero_ref, sems):
    step = pl.program_id(0)

    def x_copy(b):
        return pltpu.make_async_copy(x_hbm.at[pl.ds(b * T, T)], xs.at[pl.ds(b * T, T)], sems.at[SEM_X + b])

    def out_copy(b):
        r0 = pl.multiple_of(b * T, T)
        return pltpu.make_async_copy(xs.at[pl.ds(r0, T)], out_hbm.at[pl.ds(r0, T)], sems.at[SEM_O + b])

    rows = D // NWCH
    q_cps = [pltpu.make_async_copy(wqkv_hbm.at[pl.ds(i * rows, rows)], wqkv_raw.at[pl.ds(i * rows, rows)], sems.at[SEM_Q + i])
             for i in range(NWCH)]
    wo_cp = pltpu.make_async_copy(wo_hbm, wo_raw, sems.at[SEM_W + 0])
    w1_cp = pltpu.make_async_copy(w1_hbm, w1_v, sems.at[SEM_W + 1])
    w2_cp = pltpu.make_async_copy(w2_hbm, w2_v, sems.at[SEM_W + 2])

    @pl.when(step == 0)
    def _():
        x_copy(0).start()
        wo_cp.start()
        for c in q_cps:
            c.start()
        for b in range(1, SKEW + 1):
            x_copy(b).start()
        w1_cp.start()
        w2_cp.start()
        for b in range(SKEW + 1, NB):
            x_copy(b).start()
        zero_ref[0] = 0
        hk[...] = jnp.zeros(hk.shape, f32)
        hv[...] = jnp.zeros(hv.shape, f32)
        x_copy(0).wait()
        xn1[...] = _layernorm(xs[0:C, :].astype(f32)).astype(bf16)

        for j in range(NG):
            pm[j] = _perm_matrix(j)
        wo_cp.wait()
        for g in range(NG):
            for j in range(NG):
                wo_stage[g, j * PITCH:j * PITCH + 128, :] = wo_raw[j * 128:(j + 1) * 128, g * 128:(g + 1) * 128].astype(f32)

        def body2(jp, c):
            for t in range(4):
                for a in range(0, 4, 2):
                    for g in range(NG):
                        lo = wo_stage[g, pl.ds(32 * a + 4 * jp + t, 8, stride=PITCH), :]
                        hi = wo_stage[g, pl.ds(32 * (a + 1) + 4 * jp + t, 8, stride=PITCH), :]
                        wo_p[pl.ds(pl.multiple_of(jp * 64 + 16 * t + 4 * a, 8), 8), g * 128:(g + 1) * 128] = pltpu.bitcast(
                            jnp.concatenate([lo, hi], axis=0).astype(bf16), i32)
            return c
        lax.fori_loop(0, NG, body2, 0)

        def body(i, c):
            pltpu.make_async_copy(wqkv_hbm.at[pl.ds(0, rows)], wqkv_raw.at[pl.ds(0, rows)], sems.at[SEM_Q + i]).wait()
            r0 = pl.multiple_of(i * rows, rows)
            r1 = pl.multiple_of(i * (rows // 2), rows // 2)
            for p in range(3):
                mid = [pltpu.bitcast(jnp.dot(wqkv_raw[pl.ds(r0, rows), p * D + j * 128:p * D + (j + 1) * 128], pm[j],
                                             preferred_element_type=f32).astype(bf16), i32) for j in range(NG)]
                outs = _exchange_and_roll(mid)
                for j in range(NG):
                    wqkv_p[pl.ds(r1, rows // 2), p * D + j * 128:p * D + (j + 1) * 128] = outs[j]
            return c
        lax.fori_loop(0, NWCH, body, 0)

    u = step - SKEW
    npair = NITEM - SKEW
    is_a = jnp.logical_or(u < 0, jnp.logical_and(u < 2 * npair, u % 2 == 1))
    item_a = jnp.where(u < 0, step, SKEW + u // 2)
    item_b = jnp.where(u < 2 * npair, u // 2, u - npair)

    @pl.when(is_a)
    def _attention_item():
        item = item_a
        blk = item % NB
        nxt = jnp.minimum(item + 1, NITEM - 1) % NB
        base = pl.multiple_of(blk * T, T)

        @pl.when(item + 1 < NB)
        def _():
            pltpu.make_async_copy(x_hbm.at[pl.ds(0, T)], xs.at[pl.ds(0, T)], sems.at[SEM_X + item + 1]).wait()

        z = zero_ref[0]
        scale = DH ** -0.5
        row = lax.broadcasted_iota(i32, (R, 128), 0) + blk * T

        def logits_pieces(qs, ks, c, first, out):
            r0 = c * R
            st = {}

            def piece(w):
                if w == 0:
                    st['q'] = att[qs + z, :, HALO + r0:HALO + r0 + R, :]
                    st['lg'] = []
                kw = att[ks + z, :, pl.ds(HALO + r0 - DIL * w, R), :]
                p = jnp.sum(st['q'] * kw, axis=0)
                p = p + pltpu.roll(p, 64, 1)
                p = p + pltpu.roll(p, 32, 1)
                if first and r0 < DIL * w:
                    p = jnp.where(row + r0 >= DIL * w, p, -1e9 / scale)
                st['lg'].append(p)
                if w == W - 1:
                    lg = st['lg']
                    m = functools.reduce(jnp.maximum, lg)
                    e = [jnp.exp2((p - m) * (scale * 1.4426950408889634)) for p in lg]
                    inv = pl.reciprocal(functools.reduce(jnp.add, e), approx=True)
                    out[c] = [t * inv for t in e]
            return [functools.partial(piece, w) for w in range(W)]

        def av_pieces(probs, vs, o_s, c):
            r0 = c * R

            def piece(j):
                a = probs[c]
                acc = a[0] * att[vs + z, j, pl.ds(HALO + r0, R), :]
                for w in range(1, W):
                    acc = acc + a[w] * att[vs + z, j, pl.ds(HALO + r0 - DIL * w, R), :]
                o_s[r0:r0 + R, j * 128:(j + 1) * 128] = acc.astype(bf16)
            return [functools.partial(piece, j) for j in range(NG)]

        def paced_store(r, slot, j, pieces):
            nst = C // 8
            k = 0
            for i in range(nst):
                if slot is not None:
                    att[slot, j, HALO + 8 * i:HALO + 8 * i + 8, :] = r[8 * i:8 * i + 8]
                hi = ((i + 1) * len(pieces)) // nst
                if hi > k and slot is None:
                    att[DUMMY, 0, 0:8, :] = r[8 * i:8 * i + 8]
                while k < hi:
                    pieces[k]()
                    k += 1

        pa, pb = {}, {}
        La = [logits_pieces(QA, KA, c, True, pa) for c in range(NCH)]
        Lb = [logits_pieces(QB, KB, c, False, pb) for c in range(NCH)]
        Aa = [av_pieces(pa, VA, o_a, 2 * c) + av_pieces(pa, VA, o_a, 2 * c + 1) for c in range(NCH // 2)]
        Ab = [av_pieces(pb, VB, o_b, 2 * c) + av_pieces(pb, VB, o_b, 2 * c + 1) for c in range(NCH // 2)]

        def merge(*lists):
            lists = [l for l in lists if l]
            n = max([len(l) for l in lists], default=0)
            out = []
            for i in range(n):
                for l in lists:
                    out.extend(l[(i * len(l)) // n:((i + 1) * len(l)) // n])
            return out

        def get(lst, i):
            return lst[i] if 0 <= i < len(lst) else []

        LA0, AA0, LB0, AB0 = SCHED

        def pieces_at(t):
            return merge(get(La, t - LA0), get(Aa, t - AA0), get(Lb, t - LB0), get(Ab, t - AB0))

        att[KA, :, 0:HALO, :] = hk[...]
        att[VA, :, 0:HALO, :] = hv[...]

        xna = xn1[...]
        xb = xs[pl.ds(base + C, C), :].astype(f32)
        xnb = _layernorm(xb).astype(bf16)
        t = 0
        for chain, part in ((0, 0), (0, 1), (1, 0), (1, 1), (0, 2), (1, 2)):
            for j in range(NG):
                r = _dot(xnb if chain else xna, wqkv_p, part * NG + j)
                if part > 0:
                    if chain == 0:
                        att[QB + part, j, 0:HALO, :] = r[C - HALO:C]
                    else:
                        (hk if part == 1 else hv)[j] = r[C - HALO:C]
                paced_store(r, (QB if chain else QA) + part, j, pieces_at(t))
                t += 1
            if (chain, part) == (0, 1):
                nb0 = pl.multiple_of(nxt * T, T)
                xn_next = _layernorm(xs[pl.ds(nb0, C), :].astype(f32)).astype(bf16)
        xn1[...] = xn_next
        oa = o_a[...]
        xa = []
        for n in range(NG):
            r = _dot(oa, wo_p, n)
            paced_store(r, None, None, pieces_at(t))
            xa.append(xs[pl.ds(base, C), n * 128:(n + 1) * 128].astype(f32) + r)
            t += 1
        xa = jnp.concatenate(xa, axis=1).astype(bf16)
        xb = xb + jnp.dot(o_b[...], pltpu.bitcast(wo_p[...], bf16), preferred_element_type=f32)
        xs[pl.ds(base, C), :] = xa
        xn2[item % (SKEW + 1)] = _layernorm(xa.astype(f32)).astype(bf16)
        xs[pl.ds(base + C, C), :] = xb.astype(bf16)

    @pl.when(jnp.logical_not(is_a))
    def _mlp_item():
        item = item_b
        blk = item % NB
        base = pl.multiple_of(blk * T, T)

        @pl.when(item == 0)
        def _():
            w1_cp.wait()
            w2_cp.wait()

        def mish(h):
            ex = jnp.exp(jnp.minimum(h, 30.0))
            n = ex * (ex + 2.0)
            return (h * n * pl.reciprocal(n + 2.0, approx=True)).astype(bf16)

        def mlp1(xn):
            return jnp.concatenate(
                [mish(_dot(xn, w1_v, n) + b1_ref[n:n + 1, :].astype(f32)) for n in range(NF)], axis=1)

        act_a = mlp1(xn2[item % (SKEW + 1)])
        xb = xs[pl.ds(base + C, C), :].astype(f32)
        act_b = mlp1(_layernorm(xb).astype(bf16))
        xa = xs[pl.ds(base, C), :].astype(f32) + jnp.dot(act_a, w2_v[...], preferred_element_type=f32)
        xb = xb + jnp.dot(act_b, w2_v[...], preferred_element_type=f32)
        xs[pl.ds(base, C), :] = xa.astype(bf16)
        xs[pl.ds(base + C, C), :] = xb.astype(bf16)

        @pl.when(item >= NB)
        def _():
            out_copy(blk).start()

        @pl.when(item == NITEM - 1)
        def _():
            for b in range(NB):
                out_copy(b).wait()


@jax.jit
def pallas_interleave_layers__sliding_local_dilated__dense_activation_mish__prompt_kernel(A_x, A_wqkv, A_wo, B_x, B_w1, B_b1, B_w2):
    x = A_x.reshape(S, D)
    b1 = B_b1.reshape(NF, 128)
    out = pl.pallas_call(
        _kernel,
        grid=(2 * NITEM,),
        in_specs=[
            pl.BlockSpec(memory_space=pl.ANY),
            pl.BlockSpec((NF, 128), lambda i: (0, 0)),
            pl.BlockSpec(memory_space=pl.ANY),
            pl.BlockSpec(memory_space=pl.ANY),
            pl.BlockSpec(memory_space=pl.ANY),
            pl.BlockSpec(memory_space=pl.ANY),
        ],
        out_specs=pl.BlockSpec(memory_space=pl.ANY),
        out_shape=jax.ShapeDtypeStruct((S, D), bf16),
        scratch_shapes=[
            pltpu.VMEM((D, 3 * D), bf16), pltpu.VMEM((D // 2, 3 * D), i32),
            pltpu.VMEM((D, D), bf16), pltpu.VMEM((NG, NG * PITCH, 128), f32), pltpu.VMEM((NG, 128, 128), bf16), pltpu.VMEM((D // 2, D), i32),
            pltpu.VMEM((D, F), bf16), pltpu.VMEM((F, D), bf16),
            pltpu.VMEM((S, D), bf16), pltpu.VMEM((C, D), bf16), pltpu.VMEM((SKEW + 1, C, D), bf16),
            pltpu.VMEM((7, NG, C + HALO, 128), f32),
            pltpu.VMEM((C, D), bf16), pltpu.VMEM((C, D), bf16),
            pltpu.VMEM((NG, HALO, 128), f32), pltpu.VMEM((NG, HALO, 128), f32),
            pltpu.SMEM((1,), i32),
            pltpu.SemaphoreType.DMA((NSEM,)),
        ],
        compiler_params=pltpu.CompilerParams(
            dimension_semantics=("arbitrary",), vmem_limit_bytes=100 * 1024 * 1024),
        name="fused",
    )(x, b1, A_wqkv, A_wo, B_w1, B_w2)
    return out.reshape(1, S, D)
```

```python
import functools
import jax
import jax.numpy as jnp
from jax import lax
import jax.experimental.pallas as pl
import jax.experimental.pallas.tpu as pltpu

S, D, F = 2048, 1024, 3584
H, DH, W, DIL = 32, 32, 8, 2
NG = D // 128
NF = F // 128
HALO = 16
T = 256
C = T // 2
R = 8
NCH = C // R
NB = S // T
NITEM = 2 * NB
SKEW = 2
EPS = 1e-5
f32, bf16, i32 = jnp.float32, jnp.bfloat16, jnp.int32
QA, KA, VA, QB, KB, VB, PA, PB, DUMMY, PIN = range(10)
NSLOT = PIN + 1
LA, AA, LB, AB = (7, 16), (23.5, 7.5), (31, 16), (47.5, 7.5)
N1B, N1N, N2A, N2B = (0, 7), (15, 8), (56.5, 8), (1, 20)
LAG = 1.5
AVLAG = 0.15
CLOSE = bool(0)
SPLIT_OUT = bool(1)
AVR = 16
NWCH = 4
SEM_X, SEM_W, SEM_O, SEM_Q, NSEM = 0, NB + 1, NB + 5, NB + 6, NB + 7 + 3 * NWCH
PITCH = 129


def _layernorm(x):
    m = jnp.mean(x, axis=-1, keepdims=True)
    xc = x - m
    v = jnp.mean(xc * xc, axis=-1, keepdims=True)
    return xc * lax.rsqrt(v + EPS)


def _ln_packed(x):
    return pltpu.bitcast(_layernorm(x.astype(f32)).astype(bf16), i32)


def _perm_matrix(j):
    src = lax.broadcasted_iota(i32, (128, 128), 0)
    m = lax.broadcasted_iota(i32, (128, 128), 1)
    jp = (j + 128 - m) & 7
    l = (m + jp) & 127
    want = 32 * ((l >> 3) & 3) + 4 * jp + (l >> 5)
    return jnp.where(src == want, 1.0, 0.0).astype(bf16)


def _exchange_and_roll(mid):
    lane = lax.broadcasted_iota(i32, mid[0].shape, 1)
    for b in (1, 2, 4):
        m = (lane & b) != 0
        mid = [jnp.where(m, mid[(j + b) % 8], mid[j]) for j in range(8)]
    return [g if j == 0 else pltpu.roll(g, j, 1) for j, g in enumerate(mid)]


def _as_bf16(v):
    return v if v.dtype == bf16 else pltpu.bitcast(v, bf16)


def _dot(x, w_ref, n):
    return jnp.dot(x, _as_bf16(w_ref[:, n * 128:(n + 1) * 128]), preferred_element_type=f32)


class _Pacer:
    def __init__(self, att, z):
        self.att, self.z, self.events, self.t, self.now = att, z, [], 0, 0

    def at(self, t, piece):
        self.events.append((t, len(self.events), piece))
        self.events.sort(key=lambda e: e[:2])

    def spread(self, pieces, t0, dur):
        for i, p in enumerate(pieces):
            self.at(t0 + dur * (i + 0.5) / len(pieces), p)

    def later(self, dt, piece):
        self.at(self.now + dt, piece)

    def pin(self, words):
        v = functools.reduce(jnp.bitwise_or, [words[:, j * 128:(j + 1) * 128] for j in range(words.shape[1] // 128)])
        k, self.npin = self.npin, self.npin + 1
        per = (C + HALO) // 8
        self.att[PIN + k // (NG * per), (k // per) % NG, 8 * (k % per):8 * (k % per) + 8, :] = pltpu.bitcast(v, f32)

    def tile(self, r, slot=None, j=None):
        nst = C // 8
        for i in range(nst):
            lim = self.t + (i + 1) / nst
            fence = self.pending or (self.events and self.events[0][0] < lim)
            if slot is not None:
                self.att[slot + self.z if fence else slot, j, HALO + 8 * i:HALO + 8 * i + 8, :] = r[8 * i:8 * i + 8]
            elif fence:
                self.att[DUMMY + self.z, 0, 0:8, :] = r[8 * i:8 * i + 8]
            self.now = lim
            self.pending = False
            while self.events and self.events[0][0] < lim:
                self.events.pop(0)[2]()
                self.pending = CLOSE
        self.t += 1

    pending = False
    npin = 0


def _kernel(x_hbm, b1_hbm, wqkv_hbm, wo_hbm, w1_hbm, w2_hbm, out_hbm,
            wqkv_raw, wqkv_p, wo_raw, wo_stage, pm, wo_p, w1_v, w2_v, b1_v,
            xs, xn_a, xn_b, xn2_a, xn2_b, att, o_a, o_b, hk, hv, zero_ref, sems):
    step = pl.program_id(0)

    def x_copy(k):
        r0, r1 = max(k * T - C, 0), min(k * T + C, S)
        return pltpu.make_async_copy(x_hbm.at[pl.ds(r0, r1 - r0)], xs.at[pl.ds(r0, r1 - r0)], sems.at[SEM_X + k])

    def out_copy(r0):
        return pltpu.make_async_copy(xs.at[pl.ds(r0, C)], out_hbm.at[pl.ds(r0, C)], sems.at[SEM_O])

    rows = D // NWCH

    def q_copy(p, r0, n, k):
        return pltpu.make_async_copy(wqkv_hbm.at[pl.ds(r0, n), pl.ds(p * D, D)],
                                     wqkv_raw.at[p, pl.ds(r0, n)], sems.at[SEM_Q + k])

    wo_cp = pltpu.make_async_copy(wo_hbm, wo_raw, sems.at[SEM_W + 0])
    w1_cp = pltpu.make_async_copy(w1_hbm, w1_v, sems.at[SEM_W + 1])
    w2_cp = pltpu.make_async_copy(w2_hbm, w2_v, sems.at[SEM_W + 2])
    b1_cp = pltpu.make_async_copy(b1_hbm, b1_v, sems.at[SEM_W + 3])

    @pl.when(step == 0)
    def _():
        x_copy(0).start()
        for k in range(3 * NWCH - 1):
            q_copy(k // NWCH, (k % NWCH) * rows, rows, k).start()
            if k == NWCH - 1:
                wo_cp.start()
        for h in range(2):
            q_copy(2, D - rows + h * (rows // 2), rows // 2, 3 * NWCH - 1 + h).start()
        for k in range(1, SKEW + 1):
            x_copy(k).start()
        b1_cp.start()
        w1_cp.start()
        w2_cp.start()
        for k in range(SKEW + 1, NB + 1):
            x_copy(k).start()
        zero_ref[0] = 0
        hk[...] = jnp.zeros(hk.shape, f32)
        hv[...] = jnp.zeros(hv.shape, f32)
        for j in range(NG):
            pm[j] = _perm_matrix(j)
        x_copy(0).wait()
        xn_a[...] = _ln_packed(xs[0:C, :])

        def permute(n, p, r0, k):
            q_copy(0, 0, n, k).wait()
            r0 = pl.multiple_of(r0, n)
            r1 = pl.multiple_of(r0 >> 1, n // 2)
            mid = [pltpu.bitcast(jnp.dot(wqkv_raw[p, pl.ds(r0, n), j * 128:(j + 1) * 128], pm[j],
                                         preferred_element_type=f32).astype(bf16), i32) for j in range(NG)]
            outs = _exchange_and_roll(mid)
            for j in range(NG):
                wqkv_p[p, pl.ds(r1, n // 2), j * 128:(j + 1) * 128] = outs[j]

        def permute_chunks(k0, k1):
            def body(k, c):
                permute(rows, k >> 2, (k & 3) * rows, k)
                return c
            lax.fori_loop(k0, k1, body, 0)

        permute_chunks(0, NWCH)
        xn0 = _as_bf16(xn_a[...])
        for j in range(NG):
            att[QA, j, HALO:HALO + C, :] = _dot(xn0, wqkv_p.at[0], j)

        wo_cp.wait()
        for g in range(NG):
            for j in range(NG):
                wo_stage[g, j * PITCH:j * PITCH + 128, :] = wo_raw[j * 128:(j + 1) * 128, g * 128:(g + 1) * 128].astype(f32)

        def body2(jp, c):
            for t in range(4):
                for a in range(0, 4, 2):
                    for g in range(NG):
                        lo = wo_stage[g, pl.ds(32 * a + 4 * jp + t, 8, stride=PITCH), :]
                        hi = wo_stage[g, pl.ds(32 * (a + 1) + 4 * jp + t, 8, stride=PITCH), :]
                        wo_p[pl.ds(pl.multiple_of(jp * 64 + 16 * t + 4 * a, 8), 8), g * 128:(g + 1) * 128] = pltpu.bitcast(
                            jnp.concatenate([lo, hi], axis=0).astype(bf16), i32)
            return c
        lax.fori_loop(0, NG, body2, 0)
        permute_chunks(NWCH, 3 * NWCH - 1)

        def last(h, c):
            permute(rows // 2, 2, D - rows + h * (rows // 2), 3 * NWCH - 1 + h)
            return c
        lax.fori_loop(0, 2, last, 0)

    u = step - SKEW
    npair = NITEM - SKEW
    is_a = jnp.logical_or(u < 0, jnp.logical_and(u < 2 * npair, (u & 1) == 1))
    item_a = jnp.where(u < 0, step, SKEW + (u >> 1))
    item_b = jnp.where(u < 2 * npair, u >> 1, u - npair)

    @pl.when(is_a)
    def _attention_item():
        item = item_a
        blk = item & (NB - 1)
        nxt = (item + 1) & (NB - 1)
        base = pl.multiple_of(blk * T, T)
        nbase = pl.multiple_of(nxt * T, T)

        @pl.when(item < NB - 1)
        def _():
            pltpu.make_async_copy(x_hbm.at[pl.ds(0, T)], xs.at[pl.ds(0, T)], sems.at[SEM_X + item + 1]).wait()

        @pl.when(item == NB - 1)
        def _():
            x_copy(NB).wait()

        z = zero_ref[0]
        pc = _Pacer(att, z)
        scale = DH ** -0.5
        row = lax.broadcasted_iota(i32, (R, 128), 0) + blk * T

        def logits_pieces(qs, ks, ps, c, first):
            r0 = c * R
            st = {}

            def piece(w):
                if w == 0:
                    st['q'] = att[qs, :, HALO + r0:HALO + r0 + R, :]
                    st['lg'] = []
                kw = att[ks, :, pl.ds(HALO + r0 - DIL * w, R), :]
                p = jnp.sum(st['q'] * kw, axis=0)
                p = p + pltpu.roll(p, 64, 1)
                p = p + pltpu.roll(p, 32, 1)
                if first and r0 < DIL * w:
                    p = jnp.where(row + r0 >= DIL * w, p, -1e9 / scale)
                st['lg'].append(p)

            def softmax():
                lg = st['lg']
                m = functools.reduce(jnp.maximum, lg)
                e = [jnp.exp2((p - m) * (scale * 1.4426950408889634)) for p in lg]
                inv = pl.reciprocal(functools.reduce(jnp.add, e), approx=True)
                for w in range(W):
                    att[ps, w, r0:r0 + R, :] = e[w] * inv
            return [functools.partial(piece, w) for w in range(W)], softmax

        def av_pieces(ps, vs, o_s, c):
            r0 = c * 16
            st = {}

            def piece(j, h):
                q0 = r0 + h * AVR
                if j == 0:
                    st[h] = att[ps, :, q0:q0 + AVR, :]
                a = st[h]
                acc = a[0] * att[vs, j, pl.ds(HALO + q0, AVR), :]
                for w in range(1, W):
                    acc = acc + a[w] * att[vs, j, pl.ds(HALO + q0 - DIL * w, AVR), :]
                if AVR == 8 and h == 0:
                    st['lo'] = acc
                    return
                if AVR == 8:
                    acc = jnp.concatenate([st['lo'], acc], axis=0)
                o = pltpu.bitcast(acc.astype(bf16), i32)
                o_s[r0 // 2:r0 // 2 + 8, j * 128:(j + 1) * 128] = o
                pc.later(AVLAG, lambda: pc.pin(o))
            return [functools.partial(piece, j, h) for j in range(NG) for h in range(16 // AVR)]

        def ln1_piece(row0, dst, c):
            xn = _ln_packed(xs[pl.ds(row0 + c * 16, 16), :])
            dst[8 * c:8 * c + 8, :] = xn
            pc.pin(xn)

        for (qs, ks, ps, first, (t0, n)) in ((QA, KA, PA, True, LA), (QB, KB, PB, False, LB)):
            for c in range(NCH):
                pcs, sm = logits_pieces(qs, ks, ps, c, first)
                pc.spread(pcs, t0 + c * n / NCH, n / NCH)
                pc.at(t0 + (c + 1) * n / NCH + LAG, sm)
        pc.spread([p for c in range(C // 16) for p in av_pieces(PA, VA, o_a, c)], *AA)
        pc.spread([p for c in range(C // 16) for p in av_pieces(PB, VB, o_b, c)], *AB)
        pc.spread([functools.partial(ln1_piece, base + C, xn_b, c) for c in range(C // 16)], *N1B)
        pc.spread([functools.partial(ln1_piece, nbase, xn_a, c) for c in range(C // 16)], *N1N)

        att[KA, :, 0:HALO, :] = hk[...]
        att[VA, :, 0:HALO, :] = hv[...]

        for chain, part in ((0, 1), (0, 2), (1, 0), (1, 1), (1, 2), (0, 0)):
            if (chain, part) in ((0, 1), (1, 0), (0, 0)):
                xn = _as_bf16((xn_b if chain else xn_a)[...])
            for j in range(NG):
                r = _dot(xn, wqkv_p.at[part], j)
                if part > 0:
                    if chain == 0:
                        att[QB + part, j, 0:HALO, :] = r[C - HALO:C]
                    else:
                        (hk if part == 1 else hv)[j] = r[C - HALO:C]
                pc.tile(r, (QB if chain else QA) + part, j)
        for o_s, r0 in ((o_a, base), (o_b, base + C)):
            o = _as_bf16(o_s[...])
            for n in range(NG):
                r = _dot(o, wo_p, n) + xs[pl.ds(r0, C), n * 128:(n + 1) * 128].astype(f32)
                pc.tile(r)
                xs[pl.ds(r0, C), n * 128:(n + 1) * 128] = r.astype(bf16)
        assert not pc.events

    @pl.when(jnp.logical_not(is_a))
    def _mlp_item():
        item = item_b
        blk = item & (NB - 1)
        base = pl.multiple_of(blk * T, T)

        nbase = pl.multiple_of(((item + 1) & (NB - 1)) * T, T)

        @pl.when(item == 0)
        def _():
            xn2_a[...] = _ln_packed(xs[0:C, :])
            b1_cp.wait()
            w1_cp.wait()
            w2_cp.wait()

        pc = _Pacer(att, zero_ref[0])

        def ln_piece(row0, dst, c):
            xn = _ln_packed(xs[pl.ds(row0 + c * 16, 16), :])
            dst[8 * c:8 * c + 8, :] = xn
            pc.pin(xn)

        pc.spread([functools.partial(ln_piece, base + C, xn2_b, c) for c in range(C // 16)], *N2B)
        pc.spread([functools.partial(ln_piece, nbase, xn2_a, c) for c in range(C // 16)], *N2A)

        def mish(h):
            ex = jnp.exp(jnp.minimum(h, 30.0))
            n = ex * (ex + 2.0)
            return (h * n * pl.reciprocal(n + 2.0, approx=True)).astype(bf16)

        def mlp1(xn):
            act = []
            for n in range(NF):
                r = _dot(xn, w1_v, n)
                pc.tile(r)
                act.append(mish(r + b1_v[n:n + 1, :].astype(f32)))
            return jnp.concatenate(act, axis=1)

        act_a = mlp1(_as_bf16(xn2_a[...]))
        act_b = mlp1(_as_bf16(xn2_b[...]))
        for act, r0 in ((act_a, base), (act_b, base + C)):
            for n in range(NG):
                r = _dot(act, w2_v, n) + xs[pl.ds(r0, C), n * 128:(n + 1) * 128].astype(f32)
                pc.tile(r)
                xs[pl.ds(r0, C), n * 128:(n + 1) * 128] = r.astype(bf16)
            if SPLIT_OUT or r0 is not base:
                @pl.when(item >= NITEM - NB)
                def _():
                    if not SPLIT_OUT:
                        out_copy(base).start()
                    out_copy(r0).start()
        assert not pc.events

        @pl.when(item == NITEM - 1)
        def _():
            pltpu.make_async_copy(xs, out_hbm, sems.at[SEM_O]).wait()


@jax.jit
def pallas_interleave_layers__sliding_local_dilated__dense_activation_mish__prompt_kernel(A_x, A_wqkv, A_wo, B_x, B_w1, B_b1, B_w2):
    x = A_x.reshape(S, D)
    b1 = B_b1.reshape(NF, 128)
    out = pl.pallas_call(
        _kernel,
        grid=(2 * NITEM,),
        in_specs=[pl.BlockSpec(memory_space=pl.ANY)] * 6,
        out_specs=pl.BlockSpec(memory_space=pl.ANY),
        out_shape=jax.ShapeDtypeStruct((S, D), bf16),
        scratch_shapes=[
            pltpu.VMEM((3, D, D), bf16), pltpu.VMEM((3, D // 2, D), i32),
            pltpu.VMEM((D, D), bf16), pltpu.VMEM((NG, NG * PITCH, 128), f32), pltpu.VMEM((NG, 128, 128), bf16),
            pltpu.VMEM((D // 2, D), i32),
            pltpu.VMEM((D, F), bf16), pltpu.VMEM((F, D), bf16), pltpu.VMEM((NF, 128), bf16),
            pltpu.VMEM((S, D), bf16), pltpu.VMEM((C // 2, D), i32), pltpu.VMEM((C // 2, D), i32),
            pltpu.VMEM((C // 2, D), i32), pltpu.VMEM((C // 2, D), i32),
            pltpu.VMEM((NSLOT, NG, C + HALO, 128), f32),
            pltpu.VMEM((C // 2, D), i32), pltpu.VMEM((C // 2, D), i32),
            pltpu.VMEM((NG, HALO, 128), f32), pltpu.VMEM((NG, HALO, 128), f32),
            pltpu.SMEM((1,), i32),
            pltpu.SemaphoreType.DMA((NSEM,)),
        ],
        compiler_params=pltpu.CompilerParams(
            dimension_semantics=("arbitrary",), vmem_limit_bytes=100 * 1024 * 1024),
        name="fused",
    )(x, b1, A_wqkv, A_wo, B_w1, B_w2)
    return out.reshape(1, S, D)
```

```python
import functools
import jax
import jax.numpy as jnp
from jax import lax
import jax.experimental.pallas as pl
import jax.experimental.pallas.tpu as pltpu

S, D, F = 2048, 1024, 3584
H, DH, W, DIL = 32, 32, 8, 2
NG = D // 128
NF = F // 128
HALO = 16
T = 256
C = T // 2
R = 8
NCH = C // R
NB = S // T
NITEM = 2 * NB
SKEW = 2
EPS = 1e-5
f32, bf16, i32 = jnp.float32, jnp.bfloat16, jnp.int32
QA, KA, VA, QB, KB, VB, PA, PB, DUMMY, PIN = range(10)
NSLOT = PIN + 1
LA, AA, LB, AB = (7, 16), (23.5, 7.5), (31, 16), (47.5, 7.5)
N1B, N1N, N2A, N2B = (0, 7), (24, 7), (56.5, 8), (1, 20)
LAG = 1.5
AVLAG = 0.15
CLOSE = False
SPLIT_OUT = True
OUT_CUTS = (4, 6, 7, 8)
REL = True
HARD = True
LNLAG = 1.5
AVR = 16
NWCH = 4
SEM_X, SEM_W, SEM_O, SEM_Q, NSEM = 0, NB + 1, NB + 5, NB + 6, NB + 7 + 3 * NWCH
PITCH = 129


def _layernorm(x):
    m = jnp.mean(x, axis=-1, keepdims=True)
    xc = x - m
    v = jnp.mean(xc * xc, axis=-1, keepdims=True)
    return xc * lax.rsqrt(v + EPS)


def _ln_packed(x, zeros=None):
    x = x.astype(f32)
    if zeros is not None:
        x = jnp.concatenate([x[:, 0:128] + jnp.concatenate([zeros, zeros], axis=0), x[:, 128:]], axis=1)
    return pltpu.bitcast(_layernorm(x).astype(bf16), i32)


def _perm_matrix(j):
    src = lax.broadcasted_iota(i32, (128, 128), 0)
    m = lax.broadcasted_iota(i32, (128, 128), 1)
    jp = (j + 128 - m) & 7
    l = (m + jp) & 127
    want = 32 * ((l >> 3) & 3) + 4 * jp + (l >> 5)
    return jnp.where(src == want, 1.0, 0.0).astype(bf16)


def _exchange_and_roll(mid):
    lane = lax.broadcasted_iota(i32, mid[0].shape, 1)
    for b in (1, 2, 4):
        m = (lane & b) != 0
        mid = [jnp.where(m, mid[(j + b) % 8], mid[j]) for j in range(8)]
    return [g if j == 0 else pltpu.roll(g, j, 1) for j, g in enumerate(mid)]


def _as_bf16(v):
    return v if v.dtype == bf16 else pltpu.bitcast(v, bf16)


def _dot(x, w_ref, n):
    return jnp.dot(x, _as_bf16(w_ref[:, n * 128:(n + 1) * 128]), preferred_element_type=f32)


class _Pacer:
    def __init__(self, att, z):
        self.att, self.z, self.events, self.t, self.now = att, z, [], 0, 0

    def at(self, t, piece):
        self.events.append((t, len(self.events), piece))
        self.events.sort(key=lambda e: e[:2])

    def spread(self, pieces, t0, dur):
        for i, p in enumerate(pieces):
            self.at(t0 + dur * (i + 0.5) / len(pieces), p)

    def later(self, dt, piece):
        self.at(self.now + dt, piece)

    def zeros(self):
        return self.att[DUMMY, 1, 0:8, :]

    def tie(self, lhs):
        if not self.tied:
            return lhs
        dep = functools.reduce(jnp.bitwise_or, self.tied) & self.z
        self.tied = []
        a00 = pltpu.bitcast(pltpu.bitcast(lhs[0:16, 0:128], i32) | dep, bf16)
        return jnp.concatenate([jnp.concatenate([a00, lhs[0:16, 128:]], axis=1), lhs[16:]], axis=0)

    def pin(self, words, hard=False):
        v = functools.reduce(jnp.bitwise_or, [words[:, j * 128:(j + 1) * 128] for j in range(words.shape[1] // 128)])
        if hard:
            self.tied = self.tied + [v]
            return
        k, self.npin = self.npin, self.npin + 1
        per = (C + HALO) // 8
        self.att[PIN + k // (NG * per), (k // per) % NG, 8 * (k % per):8 * (k % per) + 8, :] = pltpu.bitcast(v, f32)

    def tile(self, r, slot=None, j=None):
        nst = C // 8
        for i in range(nst):
            lim = self.t + (i + 1) / nst
            fence = self.pending or (self.events and self.events[0][0] < lim)
            if slot is not None:
                self.att[slot + self.z if fence else slot, j, HALO + 8 * i:HALO + 8 * i + 8, :] = r[8 * i:8 * i + 8]
            elif fence:
                self.att[DUMMY + self.z, 0, 0:8, :] = r[8 * i:8 * i + 8]
            self.now = lim
            self.pending = False
            while self.events and self.events[0][0] < lim:
                self.events.pop(0)[2]()
                self.pending = CLOSE
        self.t += 1

    pending = False
    npin = 0
    tied = []


def _kernel(x_hbm, b1_hbm, wqkv_hbm, wo_hbm, w1_hbm, w2_hbm, out_hbm,
            wqkv_raw, wqkv_p, wo_raw, wo_stage, pm, wo_p, w1_v, w2_v, b1_v,
            xs, xn_a, xn_b, xn2_a, xn2_b, att, o_a, o_b, hk, hv, zero_ref, sems):
    step = pl.program_id(0)

    def x_copy(k):
        r0, r1 = max(k * T - C, 0), min(k * T + C, S)
        return pltpu.make_async_copy(x_hbm.at[pl.ds(r0, r1 - r0)], xs.at[pl.ds(r0, r1 - r0)], sems.at[SEM_X + k])

    def out_copy(r0, c0, nc):
        return pltpu.make_async_copy(xs.at[pl.ds(r0, C), pl.ds(c0, nc)], out_hbm.at[pl.ds(r0, C), pl.ds(c0, nc)],
                                     sems.at[SEM_O])

    rows = D // NWCH

    def q_copy(p, r0, n, k):
        return pltpu.make_async_copy(wqkv_hbm.at[pl.ds(r0, n), pl.ds(p * D, D)],
                                     wqkv_raw.at[p, pl.ds(r0, n)], sems.at[SEM_Q + k])

    wo_cp = pltpu.make_async_copy(wo_hbm, wo_raw, sems.at[SEM_W + 0])
    w1_cp = pltpu.make_async_copy(w1_hbm, w1_v, sems.at[SEM_W + 1])
    w2_cp = pltpu.make_async_copy(w2_hbm, w2_v, sems.at[SEM_W + 2])
    b1_cp = pltpu.make_async_copy(b1_hbm, b1_v, sems.at[SEM_W + 3])

    def prologue():
        x_copy(0).start()
        for k in range(3 * NWCH - 1):
            q_copy(k // NWCH, (k % NWCH) * rows, rows, k).start()
            if k == NWCH - 1:
                wo_cp.start()
        for h in range(2):
            q_copy(2, D - rows + h * (rows // 2), rows // 2, 3 * NWCH - 1 + h).start()
        for k in range(1, SKEW + 1):
            x_copy(k).start()
        b1_cp.start()
        w1_cp.start()
        w2_cp.start()
        for k in range(SKEW + 1, NB + 1):
            x_copy(k).start()
        zero_ref[0] = 0
        hk[...] = jnp.zeros(hk.shape, f32)
        att[DUMMY, 1, 0:8, :] = jnp.zeros((8, 128), f32)
        hv[...] = jnp.zeros(hv.shape, f32)
        for j in range(NG):
            pm[j] = _perm_matrix(j)
        x_copy(0).wait()
        xn_a[...] = _ln_packed(xs[0:C, :])

        def permute(n, p, r0, k):
            q_copy(0, 0, n, k).wait()
            r0 = pl.multiple_of(r0, n)
            r1 = pl.multiple_of(r0 >> 1, n // 2)
            mid = [pltpu.bitcast(jnp.dot(wqkv_raw[p, pl.ds(r0, n), j * 128:(j + 1) * 128], pm[j],
                                         preferred_element_type=f32).astype(bf16), i32) for j in range(NG)]
            outs = _exchange_and_roll(mid)
            for j in range(NG):
                wqkv_p[p, pl.ds(r1, n // 2), j * 128:(j + 1) * 128] = outs[j]

        def permute_chunks(k0, k1):
            def body(k, c):
                permute(rows, k >> 2, (k & 3) * rows, k)
                return c
            lax.fori_loop(k0, k1, body, 0)

        permute_chunks(0, NWCH)
        xn0 = _as_bf16(xn_a[...])
        for j in range(NG):
            att[QA, j, HALO:HALO + C, :] = _dot(xn0, wqkv_p.at[0], j)

        wo_cp.wait()
        for g in range(NG):
            for j in range(NG):
                wo_stage[g, j * PITCH:j * PITCH + 128, :] = wo_raw[j * 128:(j + 1) * 128, g * 128:(g + 1) * 128].astype(f32)

        def body2(jp, c):
            for t in range(4):
                for a in range(0, 4, 2):
                    for g in range(NG):
                        lo = wo_stage[g, pl.ds(32 * a + 4 * jp + t, 8, stride=PITCH), :]
                        hi = wo_stage[g, pl.ds(32 * (a + 1) + 4 * jp + t, 8, stride=PITCH), :]
                        wo_p[pl.ds(pl.multiple_of(jp * 64 + 16 * t + 4 * a, 8), 8), g * 128:(g + 1) * 128] = pltpu.bitcast(
                            jnp.concatenate([lo, hi], axis=0).astype(bf16), i32)
            return c
        lax.fori_loop(0, NG, body2, 0)
        permute_chunks(NWCH, 3 * NWCH - 1)

        def last(h, c):
            permute(rows // 2, 2, D - rows + h * (rows // 2), 3 * NWCH - 1 + h)
            return c
        lax.fori_loop(0, 2, last, 0)

    def first_mlp_prep():
        xn2_a[...] = _ln_packed(xs[0:C, :])
        b1_cp.wait()
        w1_cp.wait()
        w2_cp.wait()

    def _attention_item():
        item = step
        blk = item & (NB - 1)
        nxt = (item + 1) & (NB - 1)
        base = pl.multiple_of(blk * T, T)
        nbase = pl.multiple_of(nxt * T, T)

        @pl.when(item < NB - 1)
        def _():
            pltpu.make_async_copy(x_hbm.at[pl.ds(0, T)], xs.at[pl.ds(0, T)], sems.at[SEM_X + item + 1]).wait()

        @pl.when(item == NB - 1)
        def _():
            x_copy(NB).wait()

        z = zero_ref[0]
        pc = _Pacer(att, z)
        scale = DH ** -0.5
        row = lax.broadcasted_iota(i32, (R, 128), 0) + blk * T

        def logits_pieces(qs, ks, ps, c, first):
            r0 = c * R
            st = {}

            def piece(w):
                if w == 0:
                    st['q'] = att[qs, :, HALO + r0:HALO + r0 + R, :]
                    st['lg'] = []
                kw = att[ks, :, pl.ds(HALO + r0 - DIL * w, R), :]
                p = jnp.sum(st['q'] * kw, axis=0)
                p = p + pltpu.roll(p, 64, 1)
                p = p + pltpu.roll(p, 32, 1)
                if first and r0 < DIL * w:
                    p = jnp.where(row + r0 >= DIL * w, p, -1e9 / scale)
                st['lg'].append(p)

            def softmax():
                lg = st['lg']
                m = functools.reduce(jnp.maximum, lg)
                e = [jnp.exp2((p - m) * (scale * 1.4426950408889634)) for p in lg]
                inv = pl.reciprocal(functools.reduce(jnp.add, e), approx=True)
                for w in range(W):
                    att[ps, w, r0:r0 + R, :] = e[w] * inv
            return [functools.partial(piece, w) for w in range(W)], softmax

        def av_pieces(ps, vs, o_s, c):
            r0 = c * 16
            st = {}

            def piece(j, h):
                q0 = r0 + h * AVR
                if j == 0:
                    st[h] = att[ps, :, q0:q0 + AVR, :]
                a = st[h]
                acc = a[0] * att[vs, j, pl.ds(HALO + q0, AVR), :]
                for w in range(1, W):
                    acc = acc + a[w] * att[vs, j, pl.ds(HALO + q0 - DIL * w, AVR), :]
                if AVR == 8 and h == 0:
                    st['lo'] = acc
                    return
                if AVR == 8:
                    acc = jnp.concatenate([st['lo'], acc], axis=0)
                o = pltpu.bitcast(acc.astype(bf16), i32)
                o_s[r0 // 2:r0 // 2 + 8, j * 128:(j + 1) * 128] = o
                pc.later(AVLAG, lambda: pc.pin(o))
            return [functools.partial(piece, j, h) for j in range(NG) for h in range(16 // AVR)]

        def ln1_piece(row0, dst, c):
            xn = _ln_packed(xs[pl.ds(row0 + c * 16, 16), :])
            dst[8 * c:8 * c + 8, :] = xn
            pc.pin(xn, hard=dst is not xn_b)

        for (qs, ks, ps, first, (t0, n)) in ((QA, KA, PA, True, LA), (QB, KB, PB, False, LB)):
            for c in range(NCH):
                pcs, sm = logits_pieces(qs, ks, ps, c, first)
                pc.spread(pcs, t0 + c * n / NCH, n / NCH)
                pc.at(t0 + (c + 1) * n / NCH + LAG, sm)
        pc.spread([p for c in range(C // 16) for p in av_pieces(PA, VA, o_a, c)], *AA)
        pc.spread([p for c in range(C // 16) for p in av_pieces(PB, VB, o_b, c)], *AB)
        pc.spread([functools.partial(ln1_piece, base + C, xn_b, c) for c in range(C // 16)], *N1B)
        pc.spread([functools.partial(ln1_piece, nbase, xn_a, c) for c in range(C // 16)], *N1N)

        att[KA, :, 0:HALO, :] = hk[...]
        att[VA, :, 0:HALO, :] = hv[...]

        for chain, part in ((0, 1), (0, 2), (1, 0), (1, 1), (1, 2), (0, 0)):
            if (chain, part) in ((0, 1), (1, 0), (0, 0)):
                xn = _as_bf16((xn_b if chain else xn_a)[...])
            for j in range(NG):
                r = _dot(pc.tie(xn), wqkv_p.at[part], j)
                if part > 0:
                    if chain == 0:
                        att[QB + part, j, 0:HALO, :] = r[C - HALO:C]
                    else:
                        (hk if part == 1 else hv)[j] = r[C - HALO:C]
                pc.tile(r, (QB if chain else QA) + part, j)
        for o_s, r0 in ((o_a, base), (o_b, base + C)):
            o = _as_bf16(o_s[...])
            for n in range(NG):
                r = _dot(o, wo_p, n) + xs[pl.ds(r0, C), n * 128:(n + 1) * 128].astype(f32)
                pc.tile(r)
                xs[pl.ds(r0, C), n * 128:(n + 1) * 128] = r.astype(bf16)
        assert not pc.events

    def _mlp_item():
        item = step - SKEW
        blk = item & (NB - 1)
        base = pl.multiple_of(blk * T, T)

        nbase = pl.multiple_of(((item + 1) & (NB - 1)) * T, T)

        pc = _Pacer(att, zero_ref[0])

        def ln_piece(row0, dst, c):
            xn = _ln_packed(xs[pl.ds(row0 + c * 16, 16), :])
            dst[8 * c:8 * c + 8, :] = xn
            pc.pin(xn, hard=HARD or dst is xn2_a)

        pc.spread([functools.partial(ln_piece, base + C, xn2_b, c) for c in range(C // 16)], *N2B)
        pc.spread([functools.partial(ln_piece, nbase, xn2_a, c) for c in range(C // 16)], *N2A)

        def mish(h):
            ex = jnp.exp(jnp.minimum(h, 30.0))
            n = ex * (ex + 2.0)
            return (h * n * pl.reciprocal(n + 2.0, approx=True)).astype(bf16)

        def mlp1(xn):
            act = []
            for n in range(NF):
                r = _dot(pc.tie(xn), w1_v, n)
                pc.tile(r)
                act.append(mish(r + b1_v[n:n + 1, :].astype(f32)))
            return jnp.concatenate(act, axis=1)

        act_a = mlp1(_as_bf16(xn2_a[...]))
        act_b = mlp1(_as_bf16(xn2_b[...]))
        for act, r0 in ((act_a, base), (act_b, base + C)):
            for n in range(NG):
                r = _dot(pc.tie(act), w2_v, n) + xs[pl.ds(r0, C), n * 128:(n + 1) * 128].astype(f32)
                pc.tile(r)
                xs[pl.ds(r0, C), n * 128:(n + 1) * 128] = r.astype(bf16)
                cuts = OUT_CUTS if r0 is not base else (NG,)
                if n + 1 in cuts:
                    n0 = ([0] + [c for c in cuts if c <= n])[-1]

                    @pl.when(item >= NITEM - NB)
                    def _():
                        out_copy(r0, n0 * 128, (n + 1 - n0) * 128).start()
        assert not pc.events

        @pl.when(item == NITEM - 1)
        def _():
            pltpu.make_async_copy(xs, out_hbm, sems.at[SEM_O]).wait()

    @pl.when((step == 0) | (step == SKEW))
    def _():
        pl.when(step == 0)(prologue)
        pl.when(step == SKEW)(first_mlp_prep)

    pl.when(step >= SKEW)(_mlp_item)
    pl.when(step < NITEM)(_attention_item)


@jax.jit
def pallas_interleave_layers__sliding_local_dilated__dense_activation_mish__prompt_kernel(A_x, A_wqkv, A_wo, B_x, B_w1, B_b1, B_w2):
    x = A_x.reshape(S, D)
    b1 = B_b1.reshape(NF, 128)
    out = pl.pallas_call(
        _kernel,
        grid=(NITEM + SKEW,),
        in_specs=[pl.BlockSpec(memory_space=pl.ANY)] * 6,
        out_specs=pl.BlockSpec(memory_space=pl.ANY),
        out_shape=jax.ShapeDtypeStruct((S, D), bf16),
        scratch_shapes=[
            pltpu.VMEM((3, D, D), bf16), pltpu.VMEM((3, D // 2, D), i32),
            pltpu.VMEM((D, D), bf16), pltpu.VMEM((NG, NG * PITCH, 128), f32), pltpu.VMEM((NG, 128, 128), bf16),
            pltpu.VMEM((D // 2, D), i32),
            pltpu.VMEM((D, F), bf16), pltpu.VMEM((F, D), bf16), pltpu.VMEM((NF, 128), bf16),
            pltpu.VMEM((S, D), bf16), pltpu.VMEM((C // 2, D), i32), pltpu.VMEM((C // 2, D), i32),
            pltpu.VMEM((C // 2, D), i32), pltpu.VMEM((C // 2, D), i32),
            pltpu.VMEM((NSLOT, NG, C + HALO, 128), f32),
            pltpu.VMEM((C // 2, D), i32), pltpu.VMEM((C // 2, D), i32),
            pltpu.VMEM((NG, HALO, 128), f32), pltpu.VMEM((NG, HALO, 128), f32),
            pltpu.SMEM((1,), i32),
            pltpu.SemaphoreType.DMA((NSEM,)),
        ],
        compiler_params=pltpu.CompilerParams(
            dimension_semantics=("arbitrary",), vmem_limit_bytes=100 * 1024 * 1024),
        name="fused",
    )(x, b1, A_wqkv, A_wo, B_w1, B_w2)
    return out.reshape(1, S, D)
```

```python
import functools
import jax
import jax.numpy as jnp
from jax import lax
import jax.experimental.pallas as pl
import jax.experimental.pallas.tpu as pltpu

S, D, F = 2048, 1024, 3584
H, DH, W, DIL = 32, 32, 8, 2
NG = D // 128
NF = F // 128
HALO = 16
T = 256
C = T // 2
R = 8
NCH = C // R
NB = S // T
NITEM = 2 * NB
SKEW = 2
EPS = 1e-5
f32, bf16, i32 = jnp.float32, jnp.bfloat16, jnp.int32
QA, KA, VA, QB, KB, VB, PA, PB, DUMMY, PIN = range(10)
NSLOT = PIN + 1
LA, AA, LB, AB = (8, 15.5), (23.5, 7.5), (31, 16), (47.5, 7.5)
N1B, N1N, N2A, N2B = (0, 4), (4, 4), (56.5, 8), (1, 20)
LAG = 1.5
AVLAG = 0.2
CLOSE = False
SPLIT_OUT = True
OUT_CUTS = (4, 6, 7, 8)
REL = True
HARD = True
LNLAG = 1.5
QRE = 8
HARD1 = False
AVR = 16
NWCH = 4
SEM_X, SEM_W, SEM_O, SEM_Q, NSEM = 0, NB + 1, NB + 5, NB + 6, NB + 7 + 3 * NWCH
PITCH = 129


def _layernorm(x):
    m = jnp.mean(x, axis=-1, keepdims=True)
    xc = x - m
    v = jnp.mean(xc * xc, axis=-1, keepdims=True)
    return xc * lax.rsqrt(v + EPS)


def _ln_packed(x, zeros=None):
    x = x.astype(f32)
    if zeros is not None:
        x = jnp.concatenate([x[:, 0:128] + jnp.concatenate([zeros, zeros], axis=0), x[:, 128:]], axis=1)
    return pltpu.bitcast(_layernorm(x).astype(bf16), i32)


def _perm_matrix(j):
    src = lax.broadcasted_iota(i32, (128, 128), 0)
    m = lax.broadcasted_iota(i32, (128, 128), 1)
    jp = (j + 128 - m) & 7
    l = (m + jp) & 127
    want = 32 * ((l >> 3) & 3) + 4 * jp + (l >> 5)
    return jnp.where(src == want, 1.0, 0.0).astype(bf16)


def _exchange_and_roll(mid):
    lane = lax.broadcasted_iota(i32, mid[0].shape, 1)
    for b in (1, 2, 4):
        m = (lane & b) != 0
        mid = [jnp.where(m, mid[(j + b) % 8], mid[j]) for j in range(8)]
    return [g if j == 0 else pltpu.roll(g, j, 1) for j, g in enumerate(mid)]


def _as_bf16(v):
    return v if v.dtype == bf16 else pltpu.bitcast(v, bf16)


def _dot(x, w_ref, n):
    return jnp.dot(x, _as_bf16(w_ref[:, n * 128:(n + 1) * 128]), preferred_element_type=f32)


class _Pacer:
    def __init__(self, att, z):
        self.att, self.z, self.events, self.t, self.now = att, z, [], 0, 0

    def at(self, t, piece):
        self.events.append((t, len(self.events), piece))
        self.events.sort(key=lambda e: e[:2])

    def spread(self, pieces, t0, dur):
        for i, p in enumerate(pieces):
            self.at(t0 + dur * (i + 0.5) / len(pieces), p)

    def later(self, dt, piece):
        self.at(self.now + dt, piece)

    def zeros(self):
        return self.att[DUMMY, 1, 0:8, :]

    def tie(self, lhs):
        if not self.tied:
            return lhs
        dep = functools.reduce(jnp.bitwise_or, self.tied) & self.z
        self.tied = []
        a00 = pltpu.bitcast(pltpu.bitcast(lhs[0:16, 0:128], i32) | dep, bf16)
        return jnp.concatenate([jnp.concatenate([a00, lhs[0:16, 128:]], axis=1), lhs[16:]], axis=0)

    def pin(self, words, hard=False):
        v = functools.reduce(jnp.bitwise_or, [words[:, j * 128:(j + 1) * 128] for j in range(words.shape[1] // 128)])
        if hard:
            self.tied = self.tied + [v]
            return
        k, self.npin = self.npin, self.npin + 1
        per = (C + HALO) // 8
        self.att[PIN + k // (NG * per), (k // per) % NG, 8 * (k % per):8 * (k % per) + 8, :] = pltpu.bitcast(v, f32)

    def tile(self, r, slot=None, j=None):
        nst = C // 8
        for i in range(nst):
            lim = self.t + (i + 1) / nst
            fence = self.pending or (self.events and self.events[0][0] < lim)
            if slot is not None:
                self.att[slot + self.z if fence else slot, j, HALO + 8 * i:HALO + 8 * i + 8, :] = r[8 * i:8 * i + 8]
            elif fence:
                self.att[DUMMY + self.z, 0, 0:8, :] = r[8 * i:8 * i + 8]
            self.now = lim
            self.pending = False
            while self.events and self.events[0][0] < lim:
                self.events.pop(0)[2]()
                self.pending = CLOSE
        self.t += 1

    pending = False
    npin = 0
    tied = []


def _kernel(x_hbm, b1_hbm, wqkv_hbm, wo_hbm, w1_hbm, w2_hbm, out_hbm,
            wqkv_raw, wqkv_p, wo_raw, wo_stage, pm, wo_p, w1_v, w2_v, b1_v,
            xs, xn_a, xn_b, xn_n, xn2_a, xn2_b, att, o_a, o_b, hk, hv, zero_ref, sems):
    step = pl.program_id(0)

    def x_copy(k):
        r0, r1 = max(k * T - C, 0), min(k * T + C, S)
        return pltpu.make_async_copy(x_hbm.at[pl.ds(r0, r1 - r0)], xs.at[pl.ds(r0, r1 - r0)], sems.at[SEM_X + k])

    def out_copy(r0, c0, nc):
        return pltpu.make_async_copy(xs.at[pl.ds(r0, C), pl.ds(c0, nc)], out_hbm.at[pl.ds(r0, C), pl.ds(c0, nc)],
                                     sems.at[SEM_O])

    rows = D // NWCH

    def q_copy(p, r0, n, k):
        return pltpu.make_async_copy(wqkv_hbm.at[pl.ds(r0, n), pl.ds(p * D, D)],
                                     wqkv_raw.at[p, pl.ds(r0, n)], sems.at[SEM_Q + k])

    wo_cp = pltpu.make_async_copy(wo_hbm, wo_raw, sems.at[SEM_W + 0])
    w1_cp = pltpu.make_async_copy(w1_hbm, w1_v, sems.at[SEM_W + 1])
    w2_cp = pltpu.make_async_copy(w2_hbm, w2_v, sems.at[SEM_W + 2])
    b1_cp = pltpu.make_async_copy(b1_hbm, b1_v, sems.at[SEM_W + 3])

    def prologue():
        x_copy(0).start()
        for k in range(3 * NWCH - 1):
            q_copy(k // NWCH, (k % NWCH) * rows, rows, k).start()
            if k == NWCH - 1:
                wo_cp.start()
        for h in range(2):
            q_copy(2, D - rows + h * (rows // 2), rows // 2, 3 * NWCH - 1 + h).start()
        for k in range(1, SKEW + 1):
            x_copy(k).start()
        b1_cp.start()
        w1_cp.start()
        w2_cp.start()
        for k in range(SKEW + 1, NB + 1):
            x_copy(k).start()
        zero_ref[0] = 0
        hk[...] = jnp.zeros(hk.shape, f32)
        att[DUMMY, 1, 0:8, :] = jnp.zeros((8, 128), f32)
        hv[...] = jnp.zeros(hv.shape, f32)
        for j in range(NG):
            pm[j] = _perm_matrix(j)
        x_copy(0).wait()
        xn_a[...] = _ln_packed(xs[0:C, :])

        def permute(n, p, r0, k):
            q_copy(0, 0, n, k).wait()
            r0 = pl.multiple_of(r0, n)
            r1 = pl.multiple_of(r0 >> 1, n // 2)
            mid = [pltpu.bitcast(jnp.dot(wqkv_raw[p, pl.ds(r0, n), j * 128:(j + 1) * 128], pm[j],
                                         preferred_element_type=f32).astype(bf16), i32) for j in range(NG)]
            outs = _exchange_and_roll(mid)
            for j in range(NG):
                wqkv_p[p, pl.ds(r1, n // 2), j * 128:(j + 1) * 128] = outs[j]

        def permute_chunks(k0, k1):
            def body(k, c):
                permute(rows, k >> 2, (k & 3) * rows, k)
                return c
            lax.fori_loop(k0, k1, body, 0)

        permute_chunks(0, NWCH)
        xn0 = _as_bf16(xn_a[...])
        for j in range(NG):
            att[QA, j, HALO:HALO + C, :] = _dot(xn0, wqkv_p.at[0], j)

        wo_cp.wait()
        for g in range(NG):
            for j in range(NG):
                wo_stage[g, j * PITCH:j * PITCH + 128, :] = wo_raw[j * 128:(j + 1) * 128, g * 128:(g + 1) * 128].astype(f32)

        def body2(jp, c):
            for t in range(4):
                for a in range(0, 4, 2):
                    for g in range(NG):
                        lo = wo_stage[g, pl.ds(32 * a + 4 * jp + t, 8, stride=PITCH), :]
                        hi = wo_stage[g, pl.ds(32 * (a + 1) + 4 * jp + t, 8, stride=PITCH), :]
                        wo_p[pl.ds(pl.multiple_of(jp * 64 + 16 * t + 4 * a, 8), 8), g * 128:(g + 1) * 128] = pltpu.bitcast(
                            jnp.concatenate([lo, hi], axis=0).astype(bf16), i32)
            return c
        lax.fori_loop(0, NG, body2, 0)
        permute_chunks(NWCH, 3 * NWCH - 1)

        def last(h, c):
            permute(rows // 2, 2, D - rows + h * (rows // 2), 3 * NWCH - 1 + h)
            return c
        lax.fori_loop(0, 2, last, 0)

    def first_mlp_prep():
        xn2_a[...] = _ln_packed(xs[0:C, :])
        b1_cp.wait()
        w1_cp.wait()
        w2_cp.wait()

    def _attention_item():
        item = step
        blk = item & (NB - 1)
        nxt = (item + 1) & (NB - 1)
        base = pl.multiple_of(blk * T, T)
        nbase = pl.multiple_of(nxt * T, T)

        z = zero_ref[0]
        pc = _Pacer(att, z)
        scale = DH ** -0.5
        row = lax.broadcasted_iota(i32, (R, 128), 0) + blk * T

        def logits_pieces(qs, ks, ps, c, first):
            r0 = c * R
            st = {}

            def piece(w):
                if w % QRE == 0:
                    st['q'] = att[qs, :, HALO + r0:HALO + r0 + R, :]
                if w == 0:
                    st['lg'] = []
                kw = att[ks, :, pl.ds(HALO + r0 - DIL * w, R), :]
                p = jnp.sum(st['q'] * kw, axis=0)
                p = p + pltpu.roll(p, 64, 1)
                p = p + pltpu.roll(p, 32, 1)
                if first and r0 < DIL * w:
                    p = jnp.where(row + r0 >= DIL * w, p, -1e9 / scale)
                st['lg'].append(p)

            def softmax():
                lg = st['lg']
                m = functools.reduce(jnp.maximum, lg)
                e = [jnp.exp2((p - m) * (scale * 1.4426950408889634)) for p in lg]
                inv = pl.reciprocal(functools.reduce(jnp.add, e), approx=True)
                for w in range(W):
                    att[ps, w, r0:r0 + R, :] = e[w] * inv
            return [functools.partial(piece, w) for w in range(W)], softmax

        def av_pieces(ps, vs, o_s, c):
            r0 = c * 16
            st = {}

            def piece(j, h):
                q0 = r0 + h * AVR
                if j == 0:
                    st[h] = att[ps, :, q0:q0 + AVR, :]
                a = st[h]
                acc = a[0] * att[vs, j, pl.ds(HALO + q0, AVR), :]
                for w in range(1, W):
                    acc = acc + a[w] * att[vs, j, pl.ds(HALO + q0 - DIL * w, AVR), :]
                if AVR == 8 and h == 0:
                    st['lo'] = acc
                    return
                if AVR == 8:
                    acc = jnp.concatenate([st['lo'], acc], axis=0)
                o = pltpu.bitcast(acc.astype(bf16), i32)
                o_s[r0 // 2:r0 // 2 + 8, j * 128:(j + 1) * 128] = o
                pc.later(AVLAG, lambda: pc.pin(o))
            return [functools.partial(piece, j, h) for j in range(NG) for h in range(16 // AVR)]

        def ln1_piece(row0, dst, c):
            xn = _ln_packed(xs[pl.ds(row0 + c * 16, 16), :])
            dst[8 * c:8 * c + 8, :] = xn
            pc.pin(xn, hard=HARD1 and dst is not xn_b)

        for (qs, ks, ps, first, (t0, n)) in ((QA, KA, PA, True, LA), (QB, KB, PB, False, LB)):
            for c in range(NCH):
                pcs, sm = logits_pieces(qs, ks, ps, c, first)
                pc.spread(pcs, t0 + c * n / NCH, n / NCH)
                pc.at(t0 + (c + 1) * n / NCH + LAG, sm)
        pc.spread([p for c in range(C // 16) for p in av_pieces(PA, VA, o_a, c)], *AA)
        pc.spread([p for c in range(C // 16) for p in av_pieces(PB, VB, o_b, c)], *AB)
        pc.spread([functools.partial(ln1_piece, base + C, xn_b, c) for c in range(C // 16)], *N1B)
        pc.spread([functools.partial(ln1_piece, nbase, xn_n, c) for c in range(C // 16)], *N1N)

        att[KA, :, 0:HALO, :] = hk[...]
        att[VA, :, 0:HALO, :] = hv[...]

        for chain, part in ((0, 1), (0, 2), (1, 0), (1, 1), (1, 2), (0, 0)):
            if (chain, part) in ((0, 1), (1, 0), (0, 0)):
                xn = _as_bf16((xn_b if chain else (xn_a if part else xn_n))[...])
            for j in range(NG):
                r = _dot(pc.tie(xn), wqkv_p.at[part], j)
                if part > 0:
                    if chain == 0:
                        att[QB + part, j, 0:HALO, :] = r[C - HALO:C]
                    else:
                        (hk if part == 1 else hv)[j] = r[C - HALO:C]
                pc.tile(r, (QB if chain else QA) + part, j)
        for o_s, r0 in ((o_a, base), (o_b, base + C)):
            if o_s is o_b:
                xn_a[...] = xn_n[...]
            o = _as_bf16(o_s[...])
            for n in range(NG):
                r = _dot(o, wo_p, n) + xs[pl.ds(r0, C), n * 128:(n + 1) * 128].astype(f32)
                pc.tile(r)
                xs[pl.ds(r0, C), n * 128:(n + 1) * 128] = r.astype(bf16)
        assert not pc.events

    def _mlp_item():
        item = step - SKEW
        blk = item & (NB - 1)
        base = pl.multiple_of(blk * T, T)

        nbase = pl.multiple_of(((item + 1) & (NB - 1)) * T, T)

        pc = _Pacer(att, zero_ref[0])

        def ln_piece(row0, dst, c):
            xn = _ln_packed(xs[pl.ds(row0 + c * 16, 16), :])
            dst[8 * c:8 * c + 8, :] = xn
            pc.pin(xn, hard=HARD or dst is xn2_a)

        pc.spread([functools.partial(ln_piece, base + C, xn2_b, c) for c in range(C // 16)], *N2B)
        pc.spread([functools.partial(ln_piece, nbase, xn2_a, c) for c in range(C // 16)], *N2A)

        def mish(h):
            ex = jnp.exp(jnp.minimum(h, 30.0))
            n = ex * (ex + 2.0)
            return (h * n * pl.reciprocal(n + 2.0, approx=True)).astype(bf16)

        def mlp1(xn):
            act = []
            for n in range(NF):
                r = _dot(pc.tie(xn), w1_v, n)
                pc.tile(r)
                act.append(mish(r + b1_v[n:n + 1, :].astype(f32)))
            return jnp.concatenate(act, axis=1)

        act_a = mlp1(_as_bf16(xn2_a[...]))
        act_b = mlp1(_as_bf16(xn2_b[...]))
        for act, r0 in ((act_a, base), (act_b, base + C)):
            for n in range(NG):
                r = _dot(pc.tie(act), w2_v, n) + xs[pl.ds(r0, C), n * 128:(n + 1) * 128].astype(f32)
                pc.tile(r)
                xs[pl.ds(r0, C), n * 128:(n + 1) * 128] = r.astype(bf16)
                cuts = OUT_CUTS if r0 is not base else (NG,)
                if n + 1 in cuts:
                    n0 = ([0] + [c for c in cuts if c <= n])[-1]

                    @pl.when(item >= NITEM - NB)
                    def _():
                        out_copy(r0, n0 * 128, (n + 1 - n0) * 128).start()
        assert not pc.events

        @pl.when(item == NITEM - 1)
        def _():
            pltpu.make_async_copy(xs, out_hbm, sems.at[SEM_O]).wait()

    @pl.when(step <= SKEW + 1)
    def _():
        pl.when(step == 0)(prologue)
        pl.when(step == SKEW)(first_mlp_prep)
        for k in range(SKEW + 1):
            pl.when(step == k)(x_copy(k + 1).wait)

        @pl.when(step == SKEW + 1)
        def _():
            for k in range(SKEW + 2, NB + 1):
                x_copy(k).wait()

    pl.when(step >= SKEW)(_mlp_item)
    pl.when(step < NITEM)(_attention_item)


@jax.jit
def pallas_interleave_layers__sliding_local_dilated__dense_activation_mish__prompt_kernel(A_x, A_wqkv, A_wo, B_x, B_w1, B_b1, B_w2):
    x = A_x.reshape(S, D)
    b1 = B_b1.reshape(NF, 128)
    out = pl.pallas_call(
        _kernel,
        grid=(NITEM + SKEW,),
        in_specs=[pl.BlockSpec(memory_space=pl.ANY)] * 6,
        out_specs=pl.BlockSpec(memory_space=pl.ANY),
        out_shape=jax.ShapeDtypeStruct((S, D), bf16),
        scratch_shapes=[
            pltpu.VMEM((3, D, D), bf16), pltpu.VMEM((3, D // 2, D), i32),
            pltpu.VMEM((D, D), bf16), pltpu.VMEM((NG, NG * PITCH, 128), f32), pltpu.VMEM((NG, 128, 128), bf16),
            pltpu.VMEM((D // 2, D), i32),
            pltpu.VMEM((D, F), bf16), pltpu.VMEM((F, D), bf16), pltpu.VMEM((NF, 128), bf16),
            pltpu.VMEM((S, D), bf16), pltpu.VMEM((C // 2, D), i32), pltpu.VMEM((C // 2, D), i32), pltpu.VMEM((C // 2, D), i32),
            pltpu.VMEM((C // 2, D), i32), pltpu.VMEM((C // 2, D), i32),
            pltpu.VMEM((NSLOT, NG, C + HALO, 128), f32),
            pltpu.VMEM((C // 2, D), i32), pltpu.VMEM((C // 2, D), i32),
            pltpu.VMEM((NG, HALO, 128), f32), pltpu.VMEM((NG, HALO, 128), f32),
            pltpu.SMEM((1,), i32),
            pltpu.SemaphoreType.DMA((NSEM,)),
        ],
        compiler_params=pltpu.CompilerParams(
            dimension_semantics=("arbitrary",), vmem_limit_bytes=100 * 1024 * 1024),
        name="fused",
    )(x, b1, A_wqkv, A_wo, B_w1, B_w2)
    return out.reshape(1, S, D)
```

```python
import functools
import jax
import jax.numpy as jnp
from jax import lax
import jax.experimental.pallas as pl
import jax.experimental.pallas.tpu as pltpu

S, D, F = 2048, 1024, 3584
H, DH, W, DIL = 32, 32, 8, 2
NG = D // 128
NF = F // 128
HALO = 16
T = 256
C = T // 2
R = 8
NCH = C // R
NB = S // T
NITEM = 2 * NB
SKEW = 3
EPS = 1e-5
f32, bf16, i32 = jnp.float32, jnp.bfloat16, jnp.int32
QA, KA, VA, QB, KB, VB, PA, PB, DUMMY, PIN = range(10)
NSLOT = PIN + 1
LA, AA, LB, AB = (15, 16), (55.3, 7.2), (39, 16), (0.3, 7.5)
N1B, N1N, N2A, N2B = (8, 7), (32, 5), (56.5, 8), (1, 20)
FLA, FAA, FLB = (31, 12), (55.3, 7.2), (43, 12)
FN1 = (0, 6.5)
LAG = 1.5
AVLAG = 0.2
OUT_CUTS = (4, 6, 7, 8)
LNLAG = 1.2
NWCH = 4
SEM_X, SEM_W, SEM_O, SEM_Q, NSEM = 0, NB + 1, NB + 5, NB + 6, NB + 8 + NWCH
PITCH = 129


def _layernorm(x):
    m = jnp.mean(x, axis=-1, keepdims=True)
    xc = x - m
    v = jnp.mean(xc * xc, axis=-1, keepdims=True)
    return xc * lax.rsqrt(v + EPS)


def _ln_packed(x, zeros=None):
    x = x.astype(f32)
    if zeros is not None:
        x = jnp.concatenate([x[:, 0:128] + jnp.concatenate([zeros, zeros], axis=0), x[:, 128:]], axis=1)
    return pltpu.bitcast(_layernorm(x).astype(bf16), i32)


def _perm_matrix(j):
    src = lax.broadcasted_iota(i32, (128, 128), 0)
    m = lax.broadcasted_iota(i32, (128, 128), 1)
    jp = (j + 128 - m) & 7
    l = (m + jp) & 127
    want = 32 * ((l >> 3) & 3) + 4 * jp + (l >> 5)
    return jnp.where(src == want, 1.0, 0.0).astype(bf16)


def _exchange_and_roll(mid):
    lane = lax.broadcasted_iota(i32, mid[0].shape, 1)
    for b in (1, 2, 4):
        m = (lane & b) != 0
        mid = [jnp.where(m, mid[(j + b) % 8], mid[j]) for j in range(8)]
    return [g if j == 0 else pltpu.roll(g, j, 1) for j, g in enumerate(mid)]


def _as_bf16(v):
    return v if v.dtype == bf16 else pltpu.bitcast(v, bf16)


def _dot(x, w_ref, n):
    return jnp.dot(x, _as_bf16(w_ref[:, n * 128:(n + 1) * 128]), preferred_element_type=f32)


class _Pacer:
    def __init__(self, att, z):
        self.att, self.z, self.events, self.t, self.now = att, z, [], 0, 0

    def at(self, t, piece):
        self.events.append((t, len(self.events), piece))
        self.events.sort(key=lambda e: e[:2])

    def spread(self, pieces, t0, dur):
        for i, p in enumerate(pieces):
            self.at(t0 + dur * (i + 0.5) / len(pieces), p)

    def later(self, dt, piece):
        self.at(self.now + dt, piece)

    def tie(self, lhs):
        if not self.tied:
            return lhs
        dep = functools.reduce(jnp.bitwise_or, self.tied) & self.z
        self.tied = []
        a00 = pltpu.bitcast(pltpu.bitcast(lhs[0:16, 0:128], i32) | dep, bf16)
        return jnp.concatenate([jnp.concatenate([a00, lhs[0:16, 128:]], axis=1), lhs[16:]], axis=0)

    def pin(self, words, hard=False):
        v = functools.reduce(jnp.bitwise_or, [words[:, j * 128:(j + 1) * 128] for j in range(words.shape[1] // 128)])
        if hard:
            self.tied = self.tied + [v]
            return
        k, self.npin = self.npin, self.npin + 1
        per = (C + HALO) // 8
        self.att[PIN + k // (NG * per), (k // per) % NG, 8 * (k % per):8 * (k % per) + 8, :] = pltpu.bitcast(v, f32)

    def tile(self, r, slot=None, j=None):
        nst = C // 8
        for i in range(nst):
            lim = self.t + (i + 1) / nst
            fence = self.events and self.events[0][0] < lim
            if slot is not None:
                self.att[slot + self.z if fence else slot, j, HALO + 8 * i:HALO + 8 * i + 8, :] = r[8 * i:8 * i + 8]
            elif fence:
                self.att[DUMMY + self.z, 0, 0:8, :] = r[8 * i:8 * i + 8]
            self.now = lim
            while self.events and self.events[0][0] < lim:
                self.events.pop(0)[2]()
        self.t += 1

    npin = 0
    tied = []


def _kernel(x_hbm, b1_hbm, wqkv_hbm, wo_hbm, w1_hbm, w2_hbm, out_hbm,
            wqkv_raw, wqkv_p, wo_raw, wo_stage, pm, wo_p, w1_v, w2_v, b1_v,
            xs, xn1, xn2_a, xn2_b, att, o_a, o_b, hk, hv, zero_ref, sems):
    step = pl.program_id(0)
    xn_a, xn_b, xn_n = xn1.at[0], xn1.at[1], xn1.at[2]

    def x_copy(k):
        r0, r1 = max(k * T - C, 0), min(k * T + C, S)
        return pltpu.make_async_copy(x_hbm.at[pl.ds(r0, r1 - r0)], xs.at[pl.ds(r0, r1 - r0)], sems.at[SEM_X + k])

    def out_copy(r0, c0, nc):
        return pltpu.make_async_copy(xs.at[pl.ds(r0, C), pl.ds(c0, nc)], out_hbm.at[pl.ds(r0, C), pl.ds(c0, nc)],
                                     sems.at[SEM_O])

    rows = D // NWCH

    def q_copy(p, r0, n, k):
        return pltpu.make_async_copy(wqkv_hbm.at[pl.ds(r0, n), pl.ds(p * D, D)],
                                     wqkv_raw.at[p, pl.ds(r0, n)], sems.at[SEM_Q + k])

    wk_cp = q_copy(1, 0, D, NWCH)
    wv_cp = q_copy(2, 0, D, NWCH + 1)
    wo_cp = pltpu.make_async_copy(wo_hbm, wo_raw, sems.at[SEM_W + 0])
    w1_cp = pltpu.make_async_copy(w1_hbm, w1_v, sems.at[SEM_W + 1])
    w2_cp = pltpu.make_async_copy(w2_hbm, w2_v, sems.at[SEM_W + 2])
    b1_cp = pltpu.make_async_copy(b1_hbm, b1_v, sems.at[SEM_W + 3])

    def permute(p, r0, pc=None):
        r1 = r0 // 2 if isinstance(r0, int) else pl.multiple_of(r0 >> 1, rows // 2)
        mid = []
        for j in range(NG):
            r = jnp.dot(wqkv_raw[p, pl.ds(r0, rows), j * 128:(j + 1) * 128], pm[j], preferred_element_type=f32)
            if pc is not None and j % 4 == 3:
                pc.tile(r[rows - C:rows])
            mid.append(pltpu.bitcast(r.astype(bf16), i32))
        outs = _exchange_and_roll(mid)
        for j in range(NG):
            wqkv_p[p, pl.ds(r1, rows // 2), j * 128:(j + 1) * 128] = outs[j]

    def prologue():
        x_copy(0).start()
        for k in range(NWCH):
            q_copy(0, k * rows, rows, k).start()
        x_copy(1).start()
        wk_cp.start()
        wv_cp.start()
        wo_cp.start()
        for k in range(2, SKEW + 1):
            x_copy(k).start()
        b1_cp.start()
        w1_cp.start()
        w2_cp.start()
        for k in range(SKEW + 1, NB + 1):
            x_copy(k).start()
        zero_ref[0] = 0
        hk[...] = jnp.zeros(hk.shape, f32)
        att[DUMMY, 1, 0:8, :] = jnp.zeros((8, 128), f32)
        hv[...] = jnp.zeros(hv.shape, f32)
        for j in range(NG):
            pm[j] = _perm_matrix(j)
        x_copy(0).wait()
        xn_a[...] = _ln_packed(xs[0:C, :])

        def body(k, c):
            r0 = pl.multiple_of(k * rows, rows)
            q_copy(0, r0, rows, k).wait()
            permute(0, r0)
            return c
        lax.fori_loop(0, NWCH, body, 0)
        x_copy(1).wait()

        def qbody(c, carry):
            pc = _Pacer(att, zero_ref[0])

            def ln_piece(k):
                xn = _ln_packed(xs[pl.ds(pl.multiple_of((c + 1) * C + k * 16, 16), 16), :])
                xn1[c + 1, 8 * k:8 * k + 8, :] = xn
                pc.pin(xn)
            pc.spread([functools.partial(ln_piece, k) for k in range(C // 16)], *FN1)
            xn = _as_bf16(xn1[c])
            for j in range(NG):
                pc.tile(_dot(xn, wqkv_p.at[0], j), QA + (QB - QA) * c, j)
            return carry
        lax.fori_loop(0, 2, qbody, 0)
        attention('first')

    def permute_wo():
        wo_cp.wait()
        def body1(j, c):
            blk = wo_raw[pl.ds(pl.multiple_of(j * 128, 128), 128), :].astype(f32)
            for g in range(NG):
                wo_stage[g, pl.ds(j * PITCH, 128), :] = blk[:, g * 128:(g + 1) * 128]
            return c
        lax.fori_loop(0, NG, body1, 0)

        def body2(jp, c):
            for t in range(4):
                for a in range(0, 4, 2):
                    for g in range(NG):
                        lo = wo_stage[g, pl.ds(32 * a + 4 * jp + t, 8, stride=PITCH), :]
                        hi = wo_stage[g, pl.ds(32 * (a + 1) + 4 * jp + t, 8, stride=PITCH), :]
                        wo_p[pl.ds(pl.multiple_of(jp * 64 + 16 * t + 4 * a, 8), 8), g * 128:(g + 1) * 128] = pltpu.bitcast(
                            jnp.concatenate([lo, hi], axis=0).astype(bf16), i32)
            return c
        lax.fori_loop(0, NG, body2, 0)

    def first_mlp_prep():
        xn2_a[...] = _ln_packed(xs[0:C, :])
        b1_cp.wait()
        w1_cp.wait()
        w2_cp.wait()

    def attention(kind):
        if kind == 'mid':
            blk = step & (NB - 1)
            base = pl.multiple_of(blk * T, T)
            nbase = pl.multiple_of(((step + 1) & (NB - 1)) * T, T)
            pbase = pl.multiple_of(((step - 1) & (NB - 1)) * T, T)
        elif kind == 'first':
            blk = 0
        else:
            pbase = S - T

        pc = _Pacer(att, zero_ref[0])
        scale = DH ** -0.5

        def logits_pieces(qs, ks, ps, c, first):
            r0 = c * R
            st = {}

            def piece(w):
                if w == 0:
                    st['q'] = att[qs, :, HALO + r0:HALO + r0 + R, :]
                    st['lg'] = []
                kw = att[ks, :, pl.ds(HALO + r0 - DIL * w, R), :]
                p = jnp.sum(st['q'] * kw, axis=0)
                p = p + pltpu.roll(p, 64, 1)
                p = p + pltpu.roll(p, 32, 1)
                if first and r0 < DIL * w:
                    row = lax.broadcasted_iota(i32, (R, 128), 0) + blk * T
                    p = jnp.where(row + r0 >= DIL * w, p, -1e9 / scale)
                st['lg'].append(p)

            def softmax():
                lg = st['lg']
                m = functools.reduce(jnp.maximum, lg)
                e = [jnp.exp2((p - m) * (scale * 1.4426950408889634)) for p in lg]
                inv = pl.reciprocal(functools.reduce(jnp.add, e), approx=True)
                for w in range(W):
                    att[ps, w, r0:r0 + R, :] = e[w] * inv
            return [functools.partial(piece, w) for w in range(W)], softmax

        def av_pieces(ps, vs, o_s, c):
            r0 = c * 16
            st = {}

            def piece(j):
                if j == 0:
                    st['a'] = att[ps, :, r0:r0 + 16, :]
                a = st['a']
                acc = a[0] * att[vs, j, pl.ds(HALO + r0, 16), :]
                for w in range(1, W):
                    acc = acc + a[w] * att[vs, j, pl.ds(HALO + r0 - DIL * w, 16), :]
                o = pltpu.bitcast(acc.astype(bf16), i32)
                o_s[r0 // 2:r0 // 2 + 8, j * 128:(j + 1) * 128] = o
                pc.later(AVLAG, lambda: pc.pin(o))
            return [functools.partial(piece, j) for j in range(NG)]

        def ln1_piece(row0, dst, c):
            rel = dst is xn_n
            xn = _ln_packed(xs[pl.ds(row0 + c * 16, 16), :], att[DUMMY, 1, 0:8, :] if rel else None)
            dst[8 * c:8 * c + 8, :] = xn
            if rel:
                pc.later(LNLAG, lambda: pc.pin(xn))
            else:
                pc.pin(xn)

        if kind != 'last':
            la, lb, aa = (LA, LB, AA) if kind == 'mid' else (FLA, FLB, FAA)
            for (qs, ks, ps, first, (t0, n)) in ((QA, KA, PA, True, la), (QB, KB, PB, False, lb)):
                for c in range(NCH):
                    pcs, sm = logits_pieces(qs, ks, ps, c, first)
                    pc.spread(pcs, t0 + c * n / NCH, n / NCH)
                    pc.at(t0 + (c + 1) * n / NCH + LAG, sm)
            pc.spread([p for c in range(C // 16) for p in av_pieces(PA, VA, o_a, c)], *aa)
            if kind == 'mid':
                pc.spread([functools.partial(ln1_piece, base + C, xn_b, c) for c in range(C // 16)], *N1B)
                pc.spread([functools.partial(ln1_piece, nbase, xn_n, c) for c in range(C // 16)], *N1N)
            att[KA, :, 0:HALO, :] = hk[...]
            att[VA, :, 0:HALO, :] = hv[...]
        if kind != 'first':
            pc.spread([p for c in range(C // 16) for p in av_pieces(PB, VB, o_b, c)], *AB)

        def proj(chain, part):
            xn = _as_bf16((xn_b if chain else xn_a)[...])
            for j in range(NG):
                r = _dot(xn, wqkv_p.at[part], j)
                if part > 0:
                    if chain == 0:
                        att[QB + part, j, 0:HALO, :] = r[C - HALO:C]
                    else:
                        (hk if part == 1 else hv)[j] = r[C - HALO:C]
                pc.tile(r, (QB if chain else QA) + part, j)

        def out_proj(chain):
            r0 = pbase + chain * C
            o = _as_bf16((o_b if chain else o_a)[...])
            for n in range(NG):
                r = _dot(o, wo_p, n) + xs[pl.ds(r0, C), n * 128:(n + 1) * 128].astype(f32)
                pc.tile(r)
                xs[pl.ds(r0, C), n * 128:(n + 1) * 128] = r.astype(bf16)

        if kind == 'mid':
            proj(0, 0), proj(0, 1), out_proj(0), proj(1, 0), proj(1, 1), proj(0, 2), out_proj(1)
        elif kind == 'first':
            pc.t = 2 * NG
            wk_cp.wait()
            for k in range(NWCH):
                permute(1, k * rows, pc)
            proj(0, 1), proj(1, 1)
            wv_cp.wait()
            for k in range(NWCH):
                permute(2, k * rows, pc)
            proj(0, 2)
        else:
            out_proj(0), out_proj(1)
        if kind != 'last':
            xn_a[...] = xn_n[...]
            proj(1, 2)
        assert not pc.events

    def _mlp_item():
        item = step - SKEW
        blk = item & (NB - 1)
        base = pl.multiple_of(blk * T, T)

        nbase = pl.multiple_of(((item + 1) & (NB - 1)) * T, T)

        pc = _Pacer(att, zero_ref[0])

        def ln_piece(row0, dst, c):
            xn = _ln_packed(xs[pl.ds(row0 + c * 16, 16), :])
            dst[8 * c:8 * c + 8, :] = xn
            pc.pin(xn, hard=True)

        pc.spread([functools.partial(ln_piece, base + C, xn2_b, c) for c in range(C // 16)], *N2B)
        pc.spread([functools.partial(ln_piece, nbase, xn2_a, c) for c in range(C // 16)], *N2A)

        def mish(h):
            ex = jnp.exp(jnp.minimum(h, 30.0))
            n = ex * (ex + 2.0)
            return (h * n * pl.reciprocal(n + 2.0, approx=True)).astype(bf16)

        def mlp1(xn):
            act = []
            for n in range(NF):
                r = _dot(pc.tie(xn), w1_v, n)
                pc.tile(r)
                act.append(mish(r + b1_v[n:n + 1, :].astype(f32)))
            return jnp.concatenate(act, axis=1)

        act_a = mlp1(_as_bf16(xn2_a[...]))
        act_b = mlp1(_as_bf16(xn2_b[...]))
        for act, r0 in ((act_a, base), (act_b, base + C)):
            for n in range(NG):
                r = _dot(pc.tie(act), w2_v, n) + xs[pl.ds(r0, C), n * 128:(n + 1) * 128].astype(f32)
                pc.tile(r)
                xs[pl.ds(r0, C), n * 128:(n + 1) * 128] = r.astype(bf16)
                cuts = OUT_CUTS if r0 is not base else (NG,)
                if n + 1 in cuts:
                    n0 = ([0] + [c for c in cuts if c <= n])[-1]

                    @pl.when(item >= NITEM - NB)
                    def _():
                        out_copy(r0, n0 * 128, (n + 1 - n0) * 128).start()
        assert not pc.events

        @pl.when(item == NITEM - 1)
        def _():
            pltpu.make_async_copy(xs, out_hbm, sems.at[SEM_O]).wait()

    @pl.when((step <= SKEW + 1) | (step == NITEM + 1))
    def _():
        pl.when(step == 0)(prologue)
        pl.when(step == 1)(permute_wo)
        pl.when(step == SKEW)(first_mlp_prep)
        for k in range(1, SKEW + 1):
            pl.when(step == k)(x_copy(k + 1).wait)

        @pl.when(step == SKEW + 1)
        def _():
            for k in range(SKEW + 2, NB + 1):
                x_copy(k).wait()

        pl.when(step == NITEM + 1)(functools.partial(attention, 'last'))

    pl.when(step >= SKEW)(_mlp_item)
    pl.when((step >= 1) & (step < NITEM))(functools.partial(attention, 'mid'))


@jax.jit
def pallas_interleave_layers__sliding_local_dilated__dense_activation_mish__prompt_kernel(A_x, A_wqkv, A_wo, B_x, B_w1, B_b1, B_w2):
    x = A_x.reshape(S, D)
    b1 = B_b1.reshape(NF, 128)
    out = pl.pallas_call(
        _kernel,
        grid=(NITEM + SKEW,),
        in_specs=[pl.BlockSpec(memory_space=pl.ANY)] * 6,
        out_specs=pl.BlockSpec(memory_space=pl.ANY),
        out_shape=jax.ShapeDtypeStruct((S, D), bf16),
        scratch_shapes=[
            pltpu.VMEM((3, D, D), bf16), pltpu.VMEM((3, D // 2, D), i32),
            pltpu.VMEM((D, D), bf16), pltpu.VMEM((NG, NG * PITCH, 128), f32), pltpu.VMEM((NG, 128, 128), bf16),
            pltpu.VMEM((D // 2, D), i32),
            pltpu.VMEM((D, F), bf16), pltpu.VMEM((F, D), bf16), pltpu.VMEM((NF, 128), bf16),
            pltpu.VMEM((S, D), bf16), pltpu.VMEM((3, C // 2, D), i32),
            pltpu.VMEM((C // 2, D), i32), pltpu.VMEM((C // 2, D), i32),
            pltpu.VMEM((NSLOT, NG, C + HALO, 128), f32),
            pltpu.VMEM((C // 2, D), i32), pltpu.VMEM((C // 2, D), i32),
            pltpu.VMEM((NG, HALO, 128), f32), pltpu.VMEM((NG, HALO, 128), f32),
            pltpu.SMEM((1,), i32),
            pltpu.SemaphoreType.DMA((NSEM,)),
        ],
        compiler_params=pltpu.CompilerParams(
            dimension_semantics=("arbitrary",), vmem_limit_bytes=100 * 1024 * 1024),
        name="fused",
    )(x, b1, A_wqkv, A_wo, B_w1, B_w2)
    return out.reshape(1, S, D)
```

```python
import functools
import jax
import jax.numpy as jnp
from jax import lax
import jax.experimental.pallas as pl
import jax.experimental.pallas.tpu as pltpu

S, D, F = 2048, 1024, 3584
H, DH, W, DIL = 32, 32, 8, 2
NG = D // 128
NF = F // 128
HALO = 16
T = 256
C = T // 2
R = 8
NCH = C // R
NB = S // T
NITEM = 2 * NB
SKEW = 3
EPS = 1e-5
f32, bf16, i32 = jnp.float32, jnp.bfloat16, jnp.int32
QA, KA, VA, QB, KB, VB, PA, PB, DUMMY, PIN = range(10)
NSLOT = PIN + 2
LA, AA, LB, AB = (15, 16), (55.3, 7.2), (39, 16), (0.3, 7.5)
N1B, N1N, N2A, N2B = (8, 7), (32, 5), (56.5, 8), (1, 20)
FLA, FAA, FLB = (31, 12), (57.5, 5.5), (48, 8)
FN1 = (0, 6.5)
LAG = 1.5
AVLAG = 0.2
OUT_CUTS = (4, 6, 7, 8)
LNLAG = 1.2
WOPIN = 2
WOS, WOG = (48, 9), (57, 5.8)
NWCH = 4
SEM_X, SEM_W, SEM_O, SEM_Q, NSEM = 0, NB + 1, NB + 5, NB + 6, NB + 8 + NWCH
PITCH = 129


def _layernorm(x):
    m = jnp.mean(x, axis=-1, keepdims=True)
    xc = x - m
    v = jnp.mean(xc * xc, axis=-1, keepdims=True)
    return xc * lax.rsqrt(v + EPS)


def _ln_packed(x, zeros=None):
    x = x.astype(f32)
    if zeros is not None:
        x = jnp.concatenate([x[:, 0:128] + jnp.concatenate([zeros, zeros], axis=0), x[:, 128:]], axis=1)
    return pltpu.bitcast(_layernorm(x).astype(bf16), i32)


def _perm_matrix(j):
    src = lax.broadcasted_iota(i32, (128, 128), 0)
    m = lax.broadcasted_iota(i32, (128, 128), 1)
    jp = (j + 128 - m) & 7
    l = (m + jp) & 127
    want = 32 * ((l >> 3) & 3) + 4 * jp + (l >> 5)
    return jnp.where(src == want, 1.0, 0.0).astype(bf16)


def _exchange_and_roll(mid):
    lane = lax.broadcasted_iota(i32, mid[0].shape, 1)
    for b in (1, 2, 4):
        m = (lane & b) != 0
        mid = [jnp.where(m, mid[(j + b) % 8], mid[j]) for j in range(8)]
    return [g if j == 0 else pltpu.roll(g, j, 1) for j, g in enumerate(mid)]


def _as_bf16(v):
    return v if v.dtype == bf16 else pltpu.bitcast(v, bf16)


def _dot(x, w_ref, n):
    return jnp.dot(x, _as_bf16(w_ref[:, n * 128:(n + 1) * 128]), preferred_element_type=f32)


class _Pacer:
    def __init__(self, att, z):
        self.att, self.z, self.events, self.t, self.now = att, z, [], 0, 0

    def at(self, t, piece):
        self.events.append((t, len(self.events), piece))
        self.events.sort(key=lambda e: e[:2])

    def spread(self, pieces, t0, dur):
        for i, p in enumerate(pieces):
            self.at(t0 + dur * (i + 0.5) / len(pieces), p)

    def later(self, dt, piece):
        self.at(self.now + dt, piece)

    def tie(self, lhs):
        if not self.tied:
            return lhs
        dep = functools.reduce(jnp.bitwise_or, self.tied) & self.z
        self.tied = []
        a00 = pltpu.bitcast(pltpu.bitcast(lhs[0:16, 0:128], i32) | dep, bf16)
        return jnp.concatenate([jnp.concatenate([a00, lhs[0:16, 128:]], axis=1), lhs[16:]], axis=0)

    def pin(self, words, hard=False):
        v = functools.reduce(jnp.bitwise_or, [words[:, j * 128:(j + 1) * 128] for j in range(words.shape[1] // 128)])
        if hard:
            self.tied = self.tied + [v]
            return
        k, self.npin = self.npin, self.npin + 1
        per = (C + HALO) // 8
        self.att[PIN + k // (NG * per), (k // per) % NG, 8 * (k % per):8 * (k % per) + 8, :] = pltpu.bitcast(v, f32)

    def tile(self, r, slot=None, j=None):
        nst = C // 8
        for i in range(nst):
            lim = self.t + (i + 1) / nst
            fence = self.events and self.events[0][0] < lim
            if slot is not None:
                self.att[slot + self.z if fence else slot, j, HALO + 8 * i:HALO + 8 * i + 8, :] = r[8 * i:8 * i + 8]
            elif fence:
                self.att[DUMMY + self.z, 0, 0:8, :] = r[8 * i:8 * i + 8]
            self.now = lim
            while self.events and self.events[0][0] < lim:
                self.events.pop(0)[2]()
        self.t += 1

    npin = 0
    tied = []


def _kernel(x_hbm, b1_hbm, wqkv_hbm, wo_hbm, w1_hbm, w2_hbm, out_hbm,
            wqkv_raw, wqkv_p, wo_raw, wo_stage, pm, wo_p, w1_v, w2_v, b1_v,
            xs, xn1, xn2_a, xn2_b, att, o_a, o_b, hk, hv, zero_ref, sems):
    step = pl.program_id(0)
    xn_a, xn_b, xn_n = xn1.at[0], xn1.at[1], xn1.at[2]

    def x_copy(k):
        r0, r1 = max(k * T - C, 0), min(k * T + C, S)
        return pltpu.make_async_copy(x_hbm.at[pl.ds(r0, r1 - r0)], xs.at[pl.ds(r0, r1 - r0)], sems.at[SEM_X + k])

    def out_copy(r0, c0, nc):
        return pltpu.make_async_copy(xs.at[pl.ds(r0, C), pl.ds(c0, nc)], out_hbm.at[pl.ds(r0, C), pl.ds(c0, nc)],
                                     sems.at[SEM_O])

    rows = D // NWCH

    def q_copy(p, r0, n, k):
        return pltpu.make_async_copy(wqkv_hbm.at[pl.ds(r0, n), pl.ds(p * D, D)],
                                     wqkv_raw.at[p, pl.ds(r0, n)], sems.at[SEM_Q + k])

    wk_cp = q_copy(1, 0, D, NWCH)
    wv_cp = q_copy(2, 0, D, NWCH + 1)
    wo_cp = pltpu.make_async_copy(wo_hbm, wo_raw, sems.at[SEM_W + 0])
    w1_cp = pltpu.make_async_copy(w1_hbm, w1_v, sems.at[SEM_W + 1])
    w2_cp = pltpu.make_async_copy(w2_hbm, w2_v, sems.at[SEM_W + 2])
    b1_cp = pltpu.make_async_copy(b1_hbm, b1_v, sems.at[SEM_W + 3])

    def permute(p, r0, pc=None):
        r1 = r0 // 2 if isinstance(r0, int) else pl.multiple_of(r0 >> 1, rows // 2)
        mid = []
        for j in range(NG):
            r = jnp.dot(wqkv_raw[p, pl.ds(r0, rows), j * 128:(j + 1) * 128], pm[j], preferred_element_type=f32)
            if pc is not None and j % 4 == 3:
                pc.tile(r[rows - C:rows])
            mid.append(pltpu.bitcast(r.astype(bf16), i32))
        outs = _exchange_and_roll(mid)
        for j in range(NG):
            wqkv_p[p, pl.ds(r1, rows // 2), j * 128:(j + 1) * 128] = outs[j]

    def prologue():
        x_copy(0).start()
        for k in range(NWCH):
            q_copy(0, k * rows, rows, k).start()
        x_copy(1).start()
        wk_cp.start()
        wv_cp.start()
        wo_cp.start()
        for k in range(2, SKEW + 1):
            x_copy(k).start()
        b1_cp.start()
        w1_cp.start()
        w2_cp.start()
        for k in range(SKEW + 1, NB + 1):
            x_copy(k).start()
        zero_ref[0] = 0
        hk[...] = jnp.zeros(hk.shape, f32)
        att[DUMMY, 1, 0:8, :] = jnp.zeros((8, 128), f32)
        hv[...] = jnp.zeros(hv.shape, f32)
        for j in range(NG):
            pm[j] = _perm_matrix(j)
        x_copy(0).wait()
        xn_a[...] = _ln_packed(xs[0:C, :])

        def body(k, c):
            r0 = pl.multiple_of(k * rows, rows)
            q_copy(0, r0, rows, k).wait()
            permute(0, r0)
            return c
        lax.fori_loop(0, NWCH, body, 0)
        x_copy(1).wait()

        def qbody(c, carry):
            pc = _Pacer(att, zero_ref[0])

            def ln_piece(k):
                xn = _ln_packed(xs[pl.ds(pl.multiple_of((c + 1) * C + k * 16, 16), 16), :])
                xn1[c + 1, 8 * k:8 * k + 8, :] = xn
                pc.pin(xn)
            pc.spread([functools.partial(ln_piece, k) for k in range(C // 16)], *FN1)
            xn = _as_bf16(xn1[c])
            for j in range(NG):
                pc.tile(_dot(xn, wqkv_p.at[0], j), QA + (QB - QA) * c, j)
            return carry
        lax.fori_loop(0, 2, qbody, 0)
        attention('first')

    def wo_stage_piece(j, g0, g1, pc):
        blk = wo_raw[j * 128:(j + 1) * 128, g0 * 128:g1 * 128].astype(f32)
        for g in range(g0, g1):
            wo_stage[g, j * PITCH:j * PITCH + 128, :] = blk[:, (g - g0) * 128:(g - g0 + 1) * 128]
        if WOPIN:
            pc.pin(pltpu.bitcast(blk[120:128, (g1 - g0 - 1) * 128:], i32), hard=WOPIN == 2)

    def wo_gather_piece(jp, t, a, pc):
        for g in range(NG):
            lo = wo_stage[g, pl.ds(32 * a + 4 * jp + t, 8, stride=PITCH), :]
            hi = wo_stage[g, pl.ds(32 * (a + 1) + 4 * jp + t, 8, stride=PITCH), :]
            v = pltpu.bitcast(jnp.concatenate([lo, hi], axis=0).astype(bf16), i32)
            wo_p[jp * 64 + 16 * t + 4 * a:jp * 64 + 16 * t + 4 * a + 8, g * 128:(g + 1) * 128] = v
        if WOPIN:
            pc.pin(v, hard=WOPIN == 2)

    def first_mlp_prep():
        xn2_a[...] = _ln_packed(xs[0:C, :])
        b1_cp.wait()
        w1_cp.wait()
        w2_cp.wait()

    def attention(kind):
        if kind == 'mid':
            blk = step & (NB - 1)
            base = pl.multiple_of(blk * T, T)
            nbase = pl.multiple_of(((step + 1) & (NB - 1)) * T, T)
            pbase = pl.multiple_of(((step - 1) & (NB - 1)) * T, T)
        elif kind == 'first':
            blk = 0
        else:
            pbase = S - T

        pc = _Pacer(att, zero_ref[0])
        scale = DH ** -0.5

        def logits_pieces(qs, ks, ps, c, first):
            r0 = c * R
            st = {}

            def piece(w):
                if w == 0:
                    st['q'] = att[qs, :, HALO + r0:HALO + r0 + R, :]
                    st['lg'] = []
                kw = att[ks, :, pl.ds(HALO + r0 - DIL * w, R), :]
                p = jnp.sum(st['q'] * kw, axis=0)
                p = p + pltpu.roll(p, 64, 1)
                p = p + pltpu.roll(p, 32, 1)
                if first and r0 < DIL * w:
                    row = lax.broadcasted_iota(i32, (R, 128), 0) + blk * T
                    p = jnp.where(row + r0 >= DIL * w, p, -1e9 / scale)
                st['lg'].append(p)

            def softmax():
                lg = st['lg']
                m = functools.reduce(jnp.maximum, lg)
                e = [jnp.exp2((p - m) * (scale * 1.4426950408889634)) for p in lg]
                inv = pl.reciprocal(functools.reduce(jnp.add, e), approx=True)
                for w in range(W):
                    att[ps, w, r0:r0 + R, :] = e[w] * inv
            return [functools.partial(piece, w) for w in range(W)], softmax

        def av_pieces(ps, vs, o_s, c):
            r0 = c * 16
            st = {}

            def piece(j):
                if j == 0:
                    st['a'] = att[ps, :, r0:r0 + 16, :]
                a = st['a']
                acc = a[0] * att[vs, j, pl.ds(HALO + r0, 16), :]
                for w in range(1, W):
                    acc = acc + a[w] * att[vs, j, pl.ds(HALO + r0 - DIL * w, 16), :]
                o = pltpu.bitcast(acc.astype(bf16), i32)
                o_s[r0 // 2:r0 // 2 + 8, j * 128:(j + 1) * 128] = o
                pc.later(AVLAG, lambda: pc.pin(o))
            return [functools.partial(piece, j) for j in range(NG)]

        def ln1_piece(row0, dst, c):
            rel = dst is xn_n
            xn = _ln_packed(xs[pl.ds(row0 + c * 16, 16), :], att[DUMMY, 1, 0:8, :] if rel else None)
            dst[8 * c:8 * c + 8, :] = xn
            if rel:
                pc.later(LNLAG, lambda: pc.pin(xn))
            else:
                pc.pin(xn)

        if kind != 'last':
            la, lb, aa = (LA, LB, AA) if kind == 'mid' else (FLA, FLB, FAA)
            for (qs, ks, ps, first, (t0, n)) in ((QA, KA, PA, True, la), (QB, KB, PB, False, lb)):
                for c in range(NCH):
                    pcs, sm = logits_pieces(qs, ks, ps, c, first)
                    pc.spread(pcs, t0 + c * n / NCH, n / NCH)
                    pc.at(t0 + (c + 1) * n / NCH + LAG, sm)
            pc.spread([p for c in range(C // 16) for p in av_pieces(PA, VA, o_a, c)], *aa)
            if kind == 'mid':
                pc.spread([functools.partial(ln1_piece, base + C, xn_b, c) for c in range(C // 16)], *N1B)
                pc.spread([functools.partial(ln1_piece, nbase, xn_n, c) for c in range(C // 16)], *N1N)
            att[KA, :, 0:HALO, :] = hk[...]
            att[VA, :, 0:HALO, :] = hv[...]
        if kind != 'first':
            pc.spread([p for c in range(C // 16) for p in av_pieces(PB, VB, o_b, c)], *AB)

        def proj(chain, part):
            xn = _as_bf16((xn_b if chain else xn_a)[...])
            for j in range(NG):
                r = _dot(pc.tie(xn), wqkv_p.at[part], j)
                if part > 0:
                    if chain == 0:
                        att[QB + part, j, 0:HALO, :] = r[C - HALO:C]
                    else:
                        (hk if part == 1 else hv)[j] = r[C - HALO:C]
                pc.tile(r, (QB if chain else QA) + part, j)

        def out_proj(chain):
            r0 = pbase + chain * C
            o = _as_bf16((o_b if chain else o_a)[...])
            for n in range(NG):
                r = _dot(o, wo_p, n) + xs[pl.ds(r0, C), n * 128:(n + 1) * 128].astype(f32)
                pc.tile(r)
                xs[pl.ds(r0, C), n * 128:(n + 1) * 128] = r.astype(bf16)

        if kind == 'mid':
            proj(0, 0), proj(0, 1), out_proj(0), proj(1, 0), proj(1, 1), proj(0, 2), out_proj(1)
        elif kind == 'first':
            pc.t = 2 * NG
            wk_cp.wait()
            for k in range(NWCH):
                permute(1, k * rows, pc)
            proj(0, 1), proj(1, 1)
            wv_cp.wait()
            for k in range(NWCH):
                permute(2, k * rows, pc)
            wo_cp.wait()
            pc.spread([functools.partial(wo_stage_piece, j, g, g + 2, pc) for j in range(NG) for g in range(0, NG, 2)], *WOS)
            pc.spread([functools.partial(wo_gather_piece, jp, t, a, pc)
                       for jp in range(NG) for t in range(4) for a in (0, 2)], *WOG)
            proj(0, 2)
        else:
            out_proj(0), out_proj(1)
        if kind != 'last':
            xn_a[...] = xn_n[...]
            proj(1, 2)
        assert not pc.events

    def _mlp_item():
        item = step - SKEW
        blk = item & (NB - 1)
        base = pl.multiple_of(blk * T, T)

        nbase = pl.multiple_of(((item + 1) & (NB - 1)) * T, T)

        pc = _Pacer(att, zero_ref[0])

        def ln_piece(row0, dst, c):
            xn = _ln_packed(xs[pl.ds(row0 + c * 16, 16), :])
            dst[8 * c:8 * c + 8, :] = xn
            pc.pin(xn, hard=True)

        pc.spread([functools.partial(ln_piece, base + C, xn2_b, c) for c in range(C // 16)], *N2B)
        pc.spread([functools.partial(ln_piece, nbase, xn2_a, c) for c in range(C // 16)], *N2A)

        def mish(h):
            ex = jnp.exp(jnp.minimum(h, 30.0))
            n = ex * (ex + 2.0)
            return (h * n * pl.reciprocal(n + 2.0, approx=True)).astype(bf16)

        def mlp1(xn):
            act = []
            for n in range(NF):
                r = _dot(pc.tie(xn), w1_v, n)
                pc.tile(r)
                act.append(mish(r + b1_v[n:n + 1, :].astype(f32)))
            return jnp.concatenate(act, axis=1)

        act_a = mlp1(_as_bf16(xn2_a[...]))
        act_b = mlp1(_as_bf16(xn2_b[...]))
        for act, r0 in ((act_a, base), (act_b, base + C)):
            for n in range(NG):
                r = _dot(pc.tie(act), w2_v, n) + xs[pl.ds(r0, C), n * 128:(n + 1) * 128].astype(f32)
                pc.tile(r)
                xs[pl.ds(r0, C), n * 128:(n + 1) * 128] = r.astype(bf16)
                cuts = OUT_CUTS if r0 is not base else (NG,)
                if n + 1 in cuts:
                    n0 = ([0] + [c for c in cuts if c <= n])[-1]

                    @pl.when(item >= NITEM - NB)
                    def _():
                        out_copy(r0, n0 * 128, (n + 1 - n0) * 128).start()
        assert not pc.events

        @pl.when(item == NITEM - 1)
        def _():
            pltpu.make_async_copy(xs, out_hbm, sems.at[SEM_O]).wait()

    @pl.when((step <= SKEW + 1) | (step == NITEM + 1))
    def _():
        pl.when(step == 0)(prologue)
        pl.when(step == SKEW)(first_mlp_prep)
        for k in range(1, SKEW + 1):
            pl.when(step == k)(x_copy(k + 1).wait)

        @pl.when(step == SKEW + 1)
        def _():
            for k in range(SKEW + 2, NB + 1):
                x_copy(k).wait()

        pl.when(step == NITEM + 1)(functools.partial(attention, 'last'))

    pl.when(step >= SKEW)(_mlp_item)
    pl.when((step >= 1) & (step < NITEM))(functools.partial(attention, 'mid'))


@jax.jit
def pallas_interleave_layers__sliding_local_dilated__dense_activation_mish__prompt_kernel(A_x, A_wqkv, A_wo, B_x, B_w1, B_b1, B_w2):
    x = A_x.reshape(S, D)
    b1 = B_b1.reshape(NF, 128)
    out = pl.pallas_call(
        _kernel,
        grid=(NITEM + SKEW,),
        in_specs=[pl.BlockSpec(memory_space=pl.ANY)] * 6,
        out_specs=pl.BlockSpec(memory_space=pl.ANY),
        out_shape=jax.ShapeDtypeStruct((S, D), bf16),
        scratch_shapes=[
            pltpu.VMEM((3, D, D), bf16), pltpu.VMEM((3, D // 2, D), i32),
            pltpu.VMEM((D, D), bf16), pltpu.VMEM((NG, NG * PITCH, 128), f32), pltpu.VMEM((NG, 128, 128), bf16),
            pltpu.VMEM((D // 2, D), i32),
            pltpu.VMEM((D, F), bf16), pltpu.VMEM((F, D), bf16), pltpu.VMEM((NF, 128), bf16),
            pltpu.VMEM((S, D), bf16), pltpu.VMEM((3, C // 2, D), i32),
            pltpu.VMEM((C // 2, D), i32), pltpu.VMEM((C // 2, D), i32),
            pltpu.VMEM((NSLOT, NG, C + HALO, 128), f32),
            pltpu.VMEM((C // 2, D), i32), pltpu.VMEM((C // 2, D), i32),
            pltpu.VMEM((NG, HALO, 128), f32), pltpu.VMEM((NG, HALO, 128), f32),
            pltpu.SMEM((1,), i32),
            pltpu.SemaphoreType.DMA((NSEM,)),
        ],
        compiler_params=pltpu.CompilerParams(
            dimension_semantics=("arbitrary",), vmem_limit_bytes=100 * 1024 * 1024),
        name="fused",
    )(x, b1, A_wqkv, A_wo, B_w1, B_w2)
    return out.reshape(1, S, D)
```

```python
import functools
import jax
import jax.numpy as jnp
from jax import lax
import jax.experimental.pallas as pl
import jax.experimental.pallas.tpu as pltpu

S, D, F = 2048, 1024, 3584
H, DH, W, DIL = 32, 32, 8, 2
NG = D // 128
NF = F // 128
HALO = 16
T = 256
C = T // 2
R = 8
NCH = C // R
NB = S // T
NITEM = 2 * NB
SKEW = 3
EPS = 1e-5
f32, bf16, i32 = jnp.float32, jnp.bfloat16, jnp.int32
QA, KA, VA, QB, KB, VB, PA, PB, DUMMY, PIN = range(10)
NSLOT = PIN + 2
LA, AA, LB, AB = (15, 16), (55.3, 7.2), (39, 16), (0.3, 7.5)
N1B, N1N, N2A, N2B = (8, 7), (32, 5), (56.5, 8), (1, 20)
FAA = (48.3, 3.5)
FN1B, FN1N = (0, 3.5), (3.5, 3)
LAG = 1.5
AVLAG = 0.2
OUT_CUTS = (4, 6, 7, 8)
LNLAG = 1.2
WOS, WOG = (44, 4), (48, 3.8)
FT = [(t0 + i * dt, dt) for t0, dt, n in ((28, 0.6, 5), (32, 0.55, 21), (44, 0.6, 6)) for i in range(n)]
NWCH = 4
SEM_X, SEM_W, SEM_O, SEM_Q, NSEM = 0, NB + 1, NB + 5, NB + 6, NB + 10 + NWCH
PITCH = 129


def _layernorm(x):
    m = jnp.mean(x, axis=-1, keepdims=True)
    xc = x - m
    v = jnp.mean(xc * xc, axis=-1, keepdims=True)
    return xc * lax.rsqrt(v + EPS)


def _ln_packed(x, zeros=None):
    x = x.astype(f32)
    if zeros is not None:
        x = jnp.concatenate([x[:, 0:128] + jnp.concatenate([zeros, zeros], axis=0), x[:, 128:]], axis=1)
    return pltpu.bitcast(_layernorm(x).astype(bf16), i32)


def _perm_matrix(j):
    src = lax.broadcasted_iota(i32, (128, 128), 0)
    m = lax.broadcasted_iota(i32, (128, 128), 1)
    jp = (j + 128 - m) & 7
    l = (m + jp) & 127
    want = 32 * ((l >> 3) & 3) + 4 * jp + (l >> 5)
    return jnp.where(src == want, 1.0, 0.0).astype(bf16)


def _perm_pattern(j, r):
    m = lax.broadcasted_iota(i32, (r, 128), 1)
    jp = (j + 128 - m) & 7
    l = (m + jp) & 127
    return 32 * ((l >> 3) & 3) + 4 * jp + (l >> 5)


def _exchange_and_roll(mid):
    lane = lax.broadcasted_iota(i32, mid[0].shape, 1)
    for b in (1, 2, 4):
        m = (lane & b) != 0
        mid = [jnp.where(m, mid[(j + b) % 8], mid[j]) for j in range(8)]
    return [g if j == 0 else pltpu.roll(g, j, 1) for j, g in enumerate(mid)]


def _as_bf16(v):
    return v if v.dtype == bf16 else pltpu.bitcast(v, bf16)


def _dot(x, w_ref, n):
    return jnp.dot(x, _as_bf16(w_ref[:, n * 128:(n + 1) * 128]), preferred_element_type=f32)


class _Pacer:
    def __init__(self, att, z):
        self.att, self.z, self.events, self.t, self.now = att, z, [], 0, 0

    def at(self, t, piece):
        self.events.append((t, len(self.events), piece))
        self.events.sort(key=lambda e: e[:2])

    def spread(self, pieces, t0, dur):
        for i, p in enumerate(pieces):
            self.at(t0 + dur * (i + 0.5) / len(pieces), p)

    def later(self, dt, piece):
        self.at(self.now + dt, piece)

    def tie(self, lhs):
        if not self.tied:
            return lhs
        dep = functools.reduce(jnp.bitwise_or, self.tied) & self.z
        self.tied = []
        a00 = pltpu.bitcast(pltpu.bitcast(lhs[0:16, 0:128], i32) | dep, bf16)
        return jnp.concatenate([jnp.concatenate([a00, lhs[0:16, 128:]], axis=1), lhs[16:]], axis=0)

    def pin(self, words, hard=False):
        v = functools.reduce(jnp.bitwise_or, [words[:, j * 128:(j + 1) * 128] for j in range(words.shape[1] // 128)])
        if hard:
            self.tied = self.tied + [v]
            return
        k, self.npin = self.npin, self.npin + 1
        per = (C + HALO) // 8
        self.att[PIN + k // (NG * per), (k // per) % NG, 8 * (k % per):8 * (k % per) + 8, :] = pltpu.bitcast(v, f32)

    def tile(self, r, slot=None, j=None, dur=1):
        nst = C // 8
        for i in range(nst):
            lim = self.t + dur * (i + 1) / nst
            fence = self.events and self.events[0][0] < lim
            if slot is not None:
                self.att[slot + self.z if fence else slot, j, HALO + 8 * i:HALO + 8 * i + 8, :] = r[8 * i:8 * i + 8]
            elif fence:
                self.att[DUMMY + self.z, 0, 0:8, :] = r[8 * i:8 * i + 8]
            self.now = lim
            while self.events and self.events[0][0] < lim:
                self.events.pop(0)[2]()
        self.t += dur

    npin = 0
    tied = []


def _kernel(x_hbm, b1_hbm, wqkv_hbm, wo_hbm, w1_hbm, w2_hbm, out_hbm,
            wqkv_raw, wqkv_p, wo_raw, wo_stage, pm, wo_p, w1_v, w2_v, b1_v,
            xs, xn1, xn2_a, xn2_b, att, o_a, o_b, hk, hv, zero_ref, sems):
    step = pl.program_id(0)
    xn_a, xn_b, xn_n = xn1.at[0], xn1.at[1], xn1.at[2]

    def x_copy(k):
        r0, r1 = max(k * T - C, 0), min(k * T + C, S)
        return pltpu.make_async_copy(x_hbm.at[pl.ds(r0, r1 - r0)], xs.at[pl.ds(r0, r1 - r0)], sems.at[SEM_X + k])

    def out_copy(r0, c0, nc):
        return pltpu.make_async_copy(xs.at[pl.ds(r0, C), pl.ds(c0, nc)], out_hbm.at[pl.ds(r0, C), pl.ds(c0, nc)],
                                     sems.at[SEM_O])

    rows = D // NWCH

    def q_copy(p, r0, n, k):
        return pltpu.make_async_copy(wqkv_hbm.at[pl.ds(r0, n), pl.ds(p * D, D)],
                                     wqkv_raw.at[p, pl.ds(r0, n)], sems.at[SEM_Q + k])

    kv_cps = [[q_copy(p, h * (D // 2), D // 2, NWCH + 2 * (p - 1) + h) for h in range(2)] for p in (1, 2)]
    wo_cp = pltpu.make_async_copy(wo_hbm, wo_raw, sems.at[SEM_W + 0])
    w1_cp = pltpu.make_async_copy(w1_hbm, w1_v, sems.at[SEM_W + 1])
    w2_cp = pltpu.make_async_copy(w2_hbm, w2_v, sems.at[SEM_W + 2])
    b1_cp = pltpu.make_async_copy(b1_hbm, b1_v, sems.at[SEM_W + 3])

    def permute(p, r0, pc=None):
        r1 = r0 // 2 if isinstance(r0, int) else pl.multiple_of(r0 >> 1, rows // 2)
        mid = []
        for j in range(NG):
            r = jnp.dot(wqkv_raw[p, pl.ds(r0, rows), j * 128:(j + 1) * 128], pm[j], preferred_element_type=f32)
            if pc is not None and j % 4 == 3:
                pc.tile(r[rows - C:rows])
            mid.append(pltpu.bitcast(r.astype(bf16), i32))
        outs = _exchange_and_roll(mid)
        for j in range(NG):
            wqkv_p[p, pl.ds(r1, rows // 2), j * 128:(j + 1) * 128] = outs[j]

    def permute_xlu(p, r0, n):
        w0, w1 = r0 // 2, (r0 + n) // 2
        for j in range(NG):
            words = pltpu.bitcast(wqkv_raw[p, r0:r0 + n, j * 128:(j + 1) * 128], i32)
            wqkv_p[p, w0:w1, j * 128:(j + 1) * 128] = jnp.take_along_axis(
                words, _perm_pattern(j, n // 2), axis=1, mode="promise_in_bounds")
        for w in range(w0, w1, 8):
            outs = _exchange_and_roll([wqkv_p[p, w:w + 8, j * 128:(j + 1) * 128] for j in range(NG)])
            for j in range(NG):
                wqkv_p[p, w:w + 8, j * 128:(j + 1) * 128] = outs[j]

    def prologue():
        x_copy(0).start()
        for k in range(NWCH):
            q_copy(0, k * rows, rows, k).start()
        x_copy(1).start()
        for cp in kv_cps[0] + kv_cps[1]:
            cp.start()
        wo_cp.start()
        for k in range(2, SKEW + 1):
            x_copy(k).start()
        b1_cp.start()
        w1_cp.start()
        w2_cp.start()
        for k in range(SKEW + 1, NB + 1):
            x_copy(k).start()
        zero_ref[0] = 0
        hk[...] = jnp.zeros(hk.shape, f32)
        att[DUMMY, 1, 0:8, :] = jnp.zeros((8, 128), f32)
        hv[...] = jnp.zeros(hv.shape, f32)
        for j in range(NG):
            pm[j] = _perm_matrix(j)
        x_copy(0).wait()
        xn_a[...] = _ln_packed(xs[0:C, :])

        def body(k, c):
            r0 = pl.multiple_of(k * rows, rows)
            q_copy(0, r0, rows, k).wait()
            permute(0, r0)
            return c
        lax.fori_loop(0, NWCH, body, 0)
        x_copy(1).wait()

        attention('first')

    def wo_stage_piece(j, g0, g1, pc):
        blk = wo_raw[j * 128:(j + 1) * 128, g0 * 128:g1 * 128].astype(f32)
        for g in range(g0, g1):
            wo_stage[g, j * PITCH:j * PITCH + 128, :] = blk[:, (g - g0) * 128:(g - g0 + 1) * 128]
        pc.pin(pltpu.bitcast(blk[120:128, (g1 - g0 - 1) * 128:], i32), hard=True)

    def wo_gather_piece(jp, t, a, pc):
        for g in range(NG):
            lo = wo_stage[g, pl.ds(32 * a + 4 * jp + t, 8, stride=PITCH), :]
            hi = wo_stage[g, pl.ds(32 * (a + 1) + 4 * jp + t, 8, stride=PITCH), :]
            v = pltpu.bitcast(jnp.concatenate([lo, hi], axis=0).astype(bf16), i32)
            wo_p[jp * 64 + 16 * t + 4 * a:jp * 64 + 16 * t + 4 * a + 8, g * 128:(g + 1) * 128] = v
        pc.pin(v, hard=True)

    def first_mlp_prep():
        xn2_a[...] = _ln_packed(xs[0:C, :])
        b1_cp.wait()
        w1_cp.wait()
        w2_cp.wait()

    def attention(kind):
        if kind == 'mid':
            blk = step & (NB - 1)
            base = pl.multiple_of(blk * T, T)
            nbase = pl.multiple_of(((step + 1) & (NB - 1)) * T, T)
            pbase = pl.multiple_of(((step - 1) & (NB - 1)) * T, T)
        elif kind == 'first':
            blk, base, nbase = 0, 0, T
        else:
            pbase = S - T

        pc = _Pacer(att, zero_ref[0])
        scale = DH ** -0.5

        def logits_pieces(qs, ks, ps, c, first):
            r0 = c * R
            st = {}

            def piece(w):
                if w == 0:
                    st['q'] = att[qs, :, HALO + r0:HALO + r0 + R, :]
                    st['lg'] = []
                kw = att[ks, :, pl.ds(HALO + r0 - DIL * w, R), :]
                p = jnp.sum(st['q'] * kw, axis=0)
                p = p + pltpu.roll(p, 64, 1)
                p = p + pltpu.roll(p, 32, 1)
                if first and r0 < DIL * w:
                    row = lax.broadcasted_iota(i32, (R, 128), 0) + blk * T
                    p = jnp.where(row + r0 >= DIL * w, p, -1e9 / scale)
                st['lg'].append(p)

            def softmax():
                lg = st['lg']
                m = functools.reduce(jnp.maximum, lg)
                e = [jnp.exp2((p - m) * (scale * 1.4426950408889634)) for p in lg]
                inv = pl.reciprocal(functools.reduce(jnp.add, e), approx=True)
                for w in range(W):
                    att[ps, w, r0:r0 + R, :] = e[w] * inv
            return [functools.partial(piece, w) for w in range(W)], softmax

        def av_pieces(ps, vs, o_s, c):
            r0 = c * 16
            st = {}

            def piece(j):
                if j == 0:
                    st['a'] = att[ps, :, r0:r0 + 16, :]
                a = st['a']
                acc = a[0] * att[vs, j, pl.ds(HALO + r0, 16), :]
                for w in range(1, W):
                    acc = acc + a[w] * att[vs, j, pl.ds(HALO + r0 - DIL * w, 16), :]
                o = pltpu.bitcast(acc.astype(bf16), i32)
                o_s[r0 // 2:r0 // 2 + 8, j * 128:(j + 1) * 128] = o
                pc.later(AVLAG, lambda: pc.pin(o))
            return [functools.partial(piece, j) for j in range(NG)]

        def ln1_piece(row0, dst, c):
            rel = kind == 'mid' and dst is xn_n
            xn = _ln_packed(xs[pl.ds(row0 + c * 16, 16), :], att[DUMMY, 1, 0:8, :] if rel else None)
            dst[8 * c:8 * c + 8, :] = xn
            if rel:
                pc.later(LNLAG, lambda: pc.pin(xn))
            else:
                pc.pin(xn)

        if kind != 'last':
            aa = AA if kind == 'mid' else FAA
            for (qs, ks, ps, first, (t0, n)) in ((QA, KA, PA, True, LA), (QB, KB, PB, False, LB)):
                for c in range(NCH):
                    pcs, sm = logits_pieces(qs, ks, ps, c, first)
                    ts, dt = (t0 + c * n / NCH, n / NCH) if kind == 'mid' else FT[(0 if first else NCH) + c]
                    pc.spread(pcs, ts, dt)
                    pc.at(ts + dt + LAG, sm)
            pc.spread([p for c in range(C // 16) for p in av_pieces(PA, VA, o_a, c)], *aa)
            n1b, n1n = (N1B, N1N) if kind == 'mid' else (FN1B, FN1N)
            pc.spread([functools.partial(ln1_piece, base + C, xn_b, c) for c in range(C // 16)], *n1b)
            pc.spread([functools.partial(ln1_piece, nbase, xn_n, c) for c in range(C // 16)], *n1n)
            att[KA, :, 0:HALO, :] = hk[...]
            att[VA, :, 0:HALO, :] = hv[...]
        if kind != 'first':
            pc.spread([p for c in range(C // 16) for p in av_pieces(PB, VB, o_b, c)], *AB)

        def proj(chain, part, half=None):
            slot = (QB if chain else QA) + part
            src = xn_b if chain else xn_a
            if half is None:
                xn, w_ref = _as_bf16(src[...]), wqkv_p.at[part]
            else:
                xn = _as_bf16(src[:, half * (D // 2):(half + 1) * (D // 2)])
                w_ref = wqkv_p.at[part, half * (D // 4):(half + 1) * (D // 4)]
            for j in range(NG):
                r = _dot(pc.tie(xn), w_ref, j)
                if half == 1:
                    r = r + att[slot, j, HALO:HALO + C, :]
                if part > 0 and half != 0:
                    if chain == 0:
                        att[QB + part, j, 0:HALO, :] = r[C - HALO:C]
                    else:
                        (hk if part == 1 else hv)[j] = r[C - HALO:C]
                pc.tile(r, slot, j, dur=1 if half is None else 0.5)

        def out_proj(chain):
            r0 = pbase + chain * C
            o = _as_bf16((o_b if chain else o_a)[...])
            for n in range(NG):
                r = _dot(o, wo_p, n) + xs[pl.ds(r0, C), n * 128:(n + 1) * 128].astype(f32)
                pc.tile(r)
                xs[pl.ds(r0, C), n * 128:(n + 1) * 128] = r.astype(bf16)

        if kind == 'mid':
            proj(0, 0), proj(0, 1), out_proj(0), proj(1, 0), proj(1, 1), proj(0, 2), out_proj(1)
            xn_a[...] = xn_n[...]
            proj(1, 2)
        elif kind == 'first':
            proj(0, 0)
            kv_cps[0][0].wait()
            permute_xlu(1, 0, D // 2)
            proj(1, 0)
            kv_cps[0][1].wait()
            permute_xlu(1, D // 2, D // 2)
            proj(0, 1, 0), proj(1, 1, 0)
            kv_cps[1][0].wait()
            permute_xlu(2, 0, D // 2)
            proj(0, 1, 1), proj(1, 1, 1)
            kv_cps[1][1].wait()
            permute(2, 2 * rows, pc), permute(2, 3 * rows, pc)
            proj(0, 2, 0), proj(1, 2, 0)
            wo_cp.wait()
            pc.spread([functools.partial(wo_stage_piece, j, g, g + 2, pc)
                       for j in range(NG) for g in range(0, NG, 2)], *WOS)
            pc.spread([functools.partial(wo_gather_piece, jp, t, a, pc)
                       for jp in range(NG) for t in range(4) for a in (0, 2)], *WOG)
            proj(0, 2, 1)
            xn_a[...] = xn_n[...]
            proj(1, 2, 1)
        else:
            out_proj(0), out_proj(1)
        assert not pc.events

    def _mlp_item():
        item = step - SKEW
        blk = item & (NB - 1)
        base = pl.multiple_of(blk * T, T)

        nbase = pl.multiple_of(((item + 1) & (NB - 1)) * T, T)

        pc = _Pacer(att, zero_ref[0])

        def ln_piece(row0, dst, c):
            xn = _ln_packed(xs[pl.ds(row0 + c * 16, 16), :])
            dst[8 * c:8 * c + 8, :] = xn
            pc.pin(xn, hard=True)

        pc.spread([functools.partial(ln_piece, base + C, xn2_b, c) for c in range(C // 16)], *N2B)
        pc.spread([functools.partial(ln_piece, nbase, xn2_a, c) for c in range(C // 16)], *N2A)

        def mish(h):
            ex = jnp.exp(jnp.minimum(h, 30.0))
            n = ex * (ex + 2.0)
            return (h * n * pl.reciprocal(n + 2.0, approx=True)).astype(bf16)

        def mlp1(xn):
            act = []
            for n in range(NF):
                r = _dot(pc.tie(xn), w1_v, n)
                pc.tile(r)
                act.append(mish(r + b1_v[n:n + 1, :].astype(f32)))
            return jnp.concatenate(act, axis=1)

        act_a = mlp1(_as_bf16(xn2_a[...]))
        act_b = mlp1(_as_bf16(xn2_b[...]))
        for act, r0 in ((act_a, base), (act_b, base + C)):
            for n in range(NG):
                r = _dot(pc.tie(act), w2_v, n) + xs[pl.ds(r0, C), n * 128:(n + 1) * 128].astype(f32)
                pc.tile(r)
                xs[pl.ds(r0, C), n * 128:(n + 1) * 128] = r.astype(bf16)
                cuts = OUT_CUTS if r0 is not base else (NG,)
                if n + 1 in cuts:
                    n0 = ([0] + [c for c in cuts if c <= n])[-1]

                    @pl.when(item >= NITEM - NB)
                    def _():
                        out_copy(r0, n0 * 128, (n + 1 - n0) * 128).start()
        assert not pc.events

        @pl.when(item == NITEM - 1)
        def _():
            pltpu.make_async_copy(xs, out_hbm, sems.at[SEM_O]).wait()

    @pl.when((step <= SKEW + 1) | (step == NITEM + 1))
    def _():
        pl.when(step == 0)(prologue)
        pl.when(step == SKEW)(first_mlp_prep)
        for k in range(1, SKEW + 1):
            pl.when(step == k)(x_copy(k + 1).wait)

        @pl.when(step == SKEW + 1)
        def _():
            for k in range(SKEW + 2, NB + 1):
                x_copy(k).wait()

        pl.when(step == NITEM + 1)(functools.partial(attention, 'last'))

    pl.when(step >= SKEW)(_mlp_item)
    pl.when((step >= 1) & (step < NITEM))(functools.partial(attention, 'mid'))


@jax.jit
def pallas_interleave_layers__sliding_local_dilated__dense_activation_mish__prompt_kernel(A_x, A_wqkv, A_wo, B_x, B_w1, B_b1, B_w2):
    x = A_x.reshape(S, D)
    b1 = B_b1.reshape(NF, 128)
    out = pl.pallas_call(
        _kernel,
        grid=(NITEM + SKEW,),
        in_specs=[pl.BlockSpec(memory_space=pl.ANY)] * 6,
        out_specs=pl.BlockSpec(memory_space=pl.ANY),
        out_shape=jax.ShapeDtypeStruct((S, D), bf16),
        scratch_shapes=[
            pltpu.VMEM((3, D, D), bf16), pltpu.VMEM((3, D // 2, D), i32),
            pltpu.VMEM((D, D), bf16), pltpu.VMEM((NG, NG * PITCH, 128), f32), pltpu.VMEM((NG, 128, 128), bf16),
            pltpu.VMEM((D // 2, D), i32),
            pltpu.VMEM((D, F), bf16), pltpu.VMEM((F, D), bf16), pltpu.VMEM((NF, 128), bf16),
            pltpu.VMEM((S, D), bf16), pltpu.VMEM((3, C // 2, D), i32),
            pltpu.VMEM((C // 2, D), i32), pltpu.VMEM((C // 2, D), i32),
            pltpu.VMEM((NSLOT, NG, C + HALO, 128), f32),
            pltpu.VMEM((C // 2, D), i32), pltpu.VMEM((C // 2, D), i32),
            pltpu.VMEM((NG, HALO, 128), f32), pltpu.VMEM((NG, HALO, 128), f32),
            pltpu.SMEM((1,), i32),
            pltpu.SemaphoreType.DMA((NSEM,)),
        ],
        compiler_params=pltpu.CompilerParams(
            dimension_semantics=("arbitrary",), vmem_limit_bytes=100 * 1024 * 1024),
        name="fused",
    )(x, b1, A_wqkv, A_wo, B_w1, B_w2)
    return out.reshape(1, S, D)
```

```python
import functools
import jax
import jax.numpy as jnp
from jax import lax
import jax.experimental.pallas as pl
import jax.experimental.pallas.tpu as pltpu

S, D, F = 2048, 1024, 3584
H, DH, W, DIL = 32, 32, 8, 2
NG = D // 128
NF = F // 128
HALO = 16
T = 256
C = T // 2
R = 8
NCH = C // R
NB = S // T
NITEM = 2 * NB
SKEW = 3
EPS = 1e-5
f32, bf16, i32 = jnp.float32, jnp.bfloat16, jnp.int32
QA, KA, VA, QB, KB, VB, PA, PB, DUMMY, PIN = range(10)
NSLOT = PIN + 2
LA, AA, LB, AB = (15, 16), (55.3, 7.2), (39, 16), (0.3, 7.5)
N1B, N1N, N2A, N2B = (8, 7), (32, 5), (56.5, 8), (1, 20)
FAA = (48.3, 3.5)
FN1B, FN1N = (0, 3.5), (3.5, 3)
LAG = 1.5
AVLAG = 0.2
OUT_CUTS = (4, 6, 7, 8)
LNLAG = 1.2
WOS, WOG = (44, 3), (47, 4.8)
FT = [(t0 + i * dt, dt) for t0, dt, n in ((28, 0.6, 5), (32, 0.6, 19), (44, 0.5, 8)) for i in range(n)]
NWCH = 4
SEM_X, SEM_W, SEM_O, SEM_Q, NSEM = 0, NB + 1, NB + 5, NB + 6, NB + 10 + NWCH
PITCH = 65


def _layernorm(x):
    m = jnp.mean(x, axis=-1, keepdims=True)
    xc = x - m
    v = jnp.mean(xc * xc, axis=-1, keepdims=True)
    return xc * lax.rsqrt(v + EPS)


def _ln_packed(x, zeros=None):
    x = x.astype(f32)
    if zeros is not None:
        x = jnp.concatenate([x[:, 0:128] + jnp.concatenate([zeros, zeros], axis=0), x[:, 128:]], axis=1)
    return pltpu.bitcast(_layernorm(x).astype(bf16), i32)


def _perm_matrix(j):
    src = lax.broadcasted_iota(i32, (128, 128), 0)
    m = lax.broadcasted_iota(i32, (128, 128), 1)
    jp = (j + 128 - m) & 7
    l = (m + jp) & 127
    want = 32 * ((l >> 3) & 3) + 4 * jp + (l >> 5)
    return jnp.where(src == want, 1.0, 0.0).astype(bf16)


def _perm_pattern(j, r):
    m = lax.broadcasted_iota(i32, (r, 128), 1)
    jp = (j + 128 - m) & 7
    l = (m + jp) & 127
    return 32 * ((l >> 3) & 3) + 4 * jp + (l >> 5)


def _exchange_and_roll(mid):
    lane = lax.broadcasted_iota(i32, mid[0].shape, 1)
    for b in (1, 2, 4):
        m = (lane & b) != 0
        mid = [jnp.where(m, mid[(j + b) % 8], mid[j]) for j in range(8)]
    return [g if j == 0 else pltpu.roll(g, j, 1) for j, g in enumerate(mid)]


def _as_bf16(v):
    return v if v.dtype == bf16 else pltpu.bitcast(v, bf16)


def _dot(x, w_ref, n):
    return jnp.dot(x, _as_bf16(w_ref[:, n * 128:(n + 1) * 128]), preferred_element_type=f32)


class _Pacer:
    def __init__(self, att, z):
        self.att, self.z, self.events, self.t, self.now = att, z, [], 0, 0

    def at(self, t, piece):
        self.events.append((t, len(self.events), piece))
        self.events.sort(key=lambda e: e[:2])

    def spread(self, pieces, t0, dur):
        for i, p in enumerate(pieces):
            self.at(t0 + dur * (i + 0.5) / len(pieces), p)

    def later(self, dt, piece):
        self.at(self.now + dt, piece)

    def tie(self, lhs):
        if not self.tied:
            return lhs
        dep = functools.reduce(jnp.bitwise_or, self.tied) & self.z
        self.tied = []
        a00 = pltpu.bitcast(pltpu.bitcast(lhs[0:16, 0:128], i32) | dep, bf16)
        return jnp.concatenate([jnp.concatenate([a00, lhs[0:16, 128:]], axis=1), lhs[16:]], axis=0)

    def pin(self, words, hard=False):
        v = functools.reduce(jnp.bitwise_or, [words[:, j * 128:(j + 1) * 128] for j in range(words.shape[1] // 128)])
        if hard:
            self.tied = self.tied + [v]
            return
        k, self.npin = self.npin, self.npin + 1
        per = (C + HALO) // 8
        self.att[PIN + k // (NG * per), (k // per) % NG, 8 * (k % per):8 * (k % per) + 8, :] = pltpu.bitcast(v, f32)

    def tile(self, r, slot=None, j=None, dur=1):
        nst = C // 8
        for i in range(nst):
            lim = self.t + dur * (i + 1) / nst
            fence = self.events and self.events[0][0] < lim
            if slot is not None:
                self.att[slot + self.z if fence else slot, j, HALO + 8 * i:HALO + 8 * i + 8, :] = r[8 * i:8 * i + 8]
            elif fence:
                self.att[DUMMY + self.z, 0, 0:8, :] = r[8 * i:8 * i + 8]
            self.now = lim
            while self.events and self.events[0][0] < lim:
                self.events.pop(0)[2]()
        self.t += dur

    npin = 0
    tied = []


def _kernel(x_hbm, b1_hbm, wqkv_hbm, wo_hbm, w1_hbm, w2_hbm, out_hbm,
            wqkv_raw, wqkv_p, wo_raw, wo_stage, pm, wo_p, w1_v, w2_v, b1_v,
            xs, xn1, xn2_a, xn2_b, att, o_a, o_b, hk, hv, zero_ref, sems):
    step = pl.program_id(0)
    xn_a, xn_b, xn_n = xn1.at[0], xn1.at[1], xn1.at[2]

    def x_copy(k):
        r0, r1 = max(k * T - C, 0), min(k * T + C, S)
        return pltpu.make_async_copy(x_hbm.at[pl.ds(r0, r1 - r0)], xs.at[pl.ds(r0, r1 - r0)], sems.at[SEM_X + k])

    def out_copy(r0, c0, nc):
        return pltpu.make_async_copy(xs.at[pl.ds(r0, C), pl.ds(c0, nc)], out_hbm.at[pl.ds(r0, C), pl.ds(c0, nc)],
                                     sems.at[SEM_O])

    rows = D // NWCH

    def q_copy(p, r0, n, k):
        return pltpu.make_async_copy(wqkv_hbm.at[pl.ds(r0, n), pl.ds(p * D, D)],
                                     wqkv_raw.at[p, pl.ds(r0, n)], sems.at[SEM_Q + k])

    kv_cps = [[q_copy(p, h * (D // 2), D // 2, NWCH + 2 * (p - 1) + h) for h in range(2)] for p in (1, 2)]
    wo_cp = pltpu.make_async_copy(wo_hbm, wo_raw, sems.at[SEM_W + 0])
    w1_cp = pltpu.make_async_copy(w1_hbm, w1_v, sems.at[SEM_W + 1])
    w2_cp = pltpu.make_async_copy(w2_hbm, w2_v, sems.at[SEM_W + 2])
    b1_cp = pltpu.make_async_copy(b1_hbm, b1_v, sems.at[SEM_W + 3])

    def permute(p, r0, pc=None):
        r1 = r0 // 2 if isinstance(r0, int) else pl.multiple_of(r0 >> 1, rows // 2)
        mid = []
        for j in range(NG):
            r = jnp.dot(wqkv_raw[p, pl.ds(r0, rows), j * 128:(j + 1) * 128], pm[j], preferred_element_type=f32)
            if pc is not None and j % 4 == 3:
                pc.tile(r[rows - C:rows])
            mid.append(pltpu.bitcast(r.astype(bf16), i32))
        outs = _exchange_and_roll(mid)
        for j in range(NG):
            wqkv_p[p, pl.ds(r1, rows // 2), j * 128:(j + 1) * 128] = outs[j]

    def permute_xlu(p, r0, n):
        w0, w1 = r0 // 2, (r0 + n) // 2
        for j in range(NG):
            words = pltpu.bitcast(wqkv_raw[p, r0:r0 + n, j * 128:(j + 1) * 128], i32)
            wqkv_p[p, w0:w1, j * 128:(j + 1) * 128] = jnp.take_along_axis(
                words, _perm_pattern(j, n // 2), axis=1, mode="promise_in_bounds")
        for w in range(w0, w1, 8):
            outs = _exchange_and_roll([wqkv_p[p, w:w + 8, j * 128:(j + 1) * 128] for j in range(NG)])
            for j in range(NG):
                wqkv_p[p, w:w + 8, j * 128:(j + 1) * 128] = outs[j]

    def prologue():
        x_copy(0).start()
        for k in range(NWCH):
            q_copy(0, k * rows, rows, k).start()
        x_copy(1).start()
        for cp in kv_cps[0] + kv_cps[1]:
            cp.start()
        wo_cp.start()
        for k in range(2, SKEW + 1):
            x_copy(k).start()
        b1_cp.start()
        w1_cp.start()
        w2_cp.start()
        for k in range(SKEW + 1, NB + 1):
            x_copy(k).start()
        zero_ref[0] = 0
        hk[...] = jnp.zeros(hk.shape, f32)
        att[DUMMY, 1, 0:8, :] = jnp.zeros((8, 128), f32)
        hv[...] = jnp.zeros(hv.shape, f32)
        for j in range(NG):
            pm[j] = _perm_matrix(j)
        x_copy(0).wait()
        xn_a[...] = _ln_packed(xs[0:C, :])

        def body(k, c):
            r0 = pl.multiple_of(k * rows, rows)
            q_copy(0, r0, rows, k).wait()
            permute(0, r0)
            return c
        lax.fori_loop(0, NWCH, body, 0)
        x_copy(1).wait()

        attention('first')

    def wo_stage_piece(j, g0, g1, pc):
        words = pltpu.bitcast(wo_raw[j * 128:(j + 1) * 128, g0 * 128:g1 * 128], i32)
        for g in range(g0, g1):
            for a in range(4):
                r0 = PITCH * (j // 2 + 4 * (a % 2)) + 32 * (j % 2) + 16 * (a // 2)
                wo_stage[g, r0:r0 + 16, :] = words[16 * a:16 * a + 16, (g - g0) * 128:(g - g0 + 1) * 128]
        pc.pin(words[56:64, (g1 - g0 - 1) * 128:], hard=True)

    def wo_gather_piece(jp, th, ah, pc):
        for g in range(NG):
            ev = wo_stage[g, pl.ds(16 * ah + 2 * jp + th, 8, stride=PITCH), :]
            od = wo_stage[g, pl.ds(32 + 16 * ah + 2 * jp + th, 8, stride=PITCH), :]
            lo = (ev & 0xFFFF) | lax.shift_left(od, 16)
            hi = lax.shift_right_logical(ev, 16) | (od & -0x10000)
            for t, v in ((2 * th, lo), (2 * th + 1, hi)):
                w0 = jp * 64 + 16 * t + 8 * ah
                wo_p[w0:w0 + 8, g * 128:(g + 1) * 128] = v
        pc.pin(lo | hi, hard=True)

    def first_mlp_prep():
        xn2_a[...] = _ln_packed(xs[0:C, :])
        b1_cp.wait()
        w1_cp.wait()
        w2_cp.wait()

    def attention(kind):
        if kind == 'mid':
            blk = step & (NB - 1)
            base = pl.multiple_of(blk * T, T)
            nbase = pl.multiple_of(((step + 1) & (NB - 1)) * T, T)
            pbase = pl.multiple_of(((step - 1) & (NB - 1)) * T, T)
        elif kind == 'first':
            blk, base, nbase = 0, 0, T
        else:
            pbase = S - T

        pc = _Pacer(att, zero_ref[0])
        scale = DH ** -0.5

        def logits_pieces(qs, ks, ps, c, first):
            r0 = c * R
            st = {}

            def piece(w):
                if w == 0:
                    st['q'] = att[qs, :, HALO + r0:HALO + r0 + R, :]
                    st['lg'] = []
                kw = att[ks, :, pl.ds(HALO + r0 - DIL * w, R), :]
                p = jnp.sum(st['q'] * kw, axis=0)
                p = p + pltpu.roll(p, 64, 1)
                p = p + pltpu.roll(p, 32, 1)
                if first and r0 < DIL * w:
                    row = lax.broadcasted_iota(i32, (R, 128), 0) + blk * T
                    p = jnp.where(row + r0 >= DIL * w, p, -1e9 / scale)
                st['lg'].append(p)

            def softmax():
                lg = st['lg']
                m = functools.reduce(jnp.maximum, lg)
                e = [jnp.exp2((p - m) * (scale * 1.4426950408889634)) for p in lg]
                inv = pl.reciprocal(functools.reduce(jnp.add, e), approx=True)
                for w in range(W):
                    att[ps, w, r0:r0 + R, :] = e[w] * inv
            return [functools.partial(piece, w) for w in range(W)], softmax

        def av_pieces(ps, vs, o_s, c):
            r0 = c * 16
            st = {}

            def piece(j):
                if j == 0:
                    st['a'] = att[ps, :, r0:r0 + 16, :]
                a = st['a']
                acc = a[0] * att[vs, j, pl.ds(HALO + r0, 16), :]
                for w in range(1, W):
                    acc = acc + a[w] * att[vs, j, pl.ds(HALO + r0 - DIL * w, 16), :]
                o = pltpu.bitcast(acc.astype(bf16), i32)
                o_s[r0 // 2:r0 // 2 + 8, j * 128:(j + 1) * 128] = o
                pc.later(AVLAG, lambda: pc.pin(o))
            return [functools.partial(piece, j) for j in range(NG)]

        def ln1_piece(row0, dst, c):
            rel = kind == 'mid' and dst is xn_n
            xn = _ln_packed(xs[pl.ds(row0 + c * 16, 16), :], att[DUMMY, 1, 0:8, :] if rel else None)
            dst[8 * c:8 * c + 8, :] = xn
            if rel:
                pc.later(LNLAG, lambda: pc.pin(xn))
            else:
                pc.pin(xn)

        if kind != 'last':
            aa = AA if kind == 'mid' else FAA
            for (qs, ks, ps, first, (t0, n)) in ((QA, KA, PA, True, LA), (QB, KB, PB, False, LB)):
                for c in range(NCH):
                    pcs, sm = logits_pieces(qs, ks, ps, c, first)
                    ts, dt = (t0 + c * n / NCH, n / NCH) if kind == 'mid' else FT[(0 if first else NCH) + c]
                    pc.spread(pcs, ts, dt)
                    pc.at(ts + dt + LAG, sm)
            pc.spread([p for c in range(C // 16) for p in av_pieces(PA, VA, o_a, c)], *aa)
            n1b, n1n = (N1B, N1N) if kind == 'mid' else (FN1B, FN1N)
            pc.spread([functools.partial(ln1_piece, base + C, xn_b, c) for c in range(C // 16)], *n1b)
            pc.spread([functools.partial(ln1_piece, nbase, xn_n, c) for c in range(C // 16)], *n1n)
            att[KA, :, 0:HALO, :] = hk[...]
            att[VA, :, 0:HALO, :] = hv[...]
        if kind != 'first':
            pc.spread([p for c in range(C // 16) for p in av_pieces(PB, VB, o_b, c)], *AB)

        def proj(chain, part, half=None):
            slot = (QB if chain else QA) + part
            src = xn_b if chain else xn_a
            if half is None:
                xn, w_ref = _as_bf16(src[...]), wqkv_p.at[part]
            else:
                xn = _as_bf16(src[:, half * (D // 2):(half + 1) * (D // 2)])
                w_ref = wqkv_p.at[part, half * (D // 4):(half + 1) * (D // 4)]
            for j in range(NG):
                r = _dot(pc.tie(xn), w_ref, j)
                if half == 1:
                    r = r + att[slot, j, HALO:HALO + C, :]
                if part > 0 and half != 0:
                    if chain == 0:
                        att[QB + part, j, 0:HALO, :] = r[C - HALO:C]
                    else:
                        (hk if part == 1 else hv)[j] = r[C - HALO:C]
                pc.tile(r, slot, j, dur=1 if half is None else 0.5)

        def out_proj(chain):
            r0 = pbase + chain * C
            o = _as_bf16((o_b if chain else o_a)[...])
            for n in range(NG):
                r = _dot(o, wo_p, n) + xs[pl.ds(r0, C), n * 128:(n + 1) * 128].astype(f32)
                pc.tile(r)
                xs[pl.ds(r0, C), n * 128:(n + 1) * 128] = r.astype(bf16)

        if kind == 'mid':
            proj(0, 0), proj(0, 1), out_proj(0), proj(1, 0), proj(1, 1), proj(0, 2), out_proj(1)
            xn_a[...] = xn_n[...]
            proj(1, 2)
        elif kind == 'first':
            proj(0, 0)
            kv_cps[0][0].wait()
            permute_xlu(1, 0, D // 2)
            proj(1, 0)
            kv_cps[0][1].wait()
            permute_xlu(1, D // 2, D // 2)
            proj(0, 1, 0), proj(1, 1, 0)
            kv_cps[1][0].wait()
            permute_xlu(2, 0, D // 2)
            proj(0, 1, 1), proj(1, 1, 1)
            kv_cps[1][1].wait()
            permute(2, 2 * rows, pc), permute(2, 3 * rows, pc)
            proj(0, 2, 0), proj(1, 2, 0)
            wo_cp.wait()
            pc.spread([functools.partial(wo_stage_piece, j, g, g + 2, pc)
                       for j in range(NG) for g in range(0, NG, 2)], *WOS)
            pc.spread([functools.partial(wo_gather_piece, jp, th, ah, pc)
                       for jp in range(NG) for th in range(2) for ah in range(2)], *WOG)
            proj(0, 2, 1)
            xn_a[...] = xn_n[...]
            proj(1, 2, 1)
        else:
            out_proj(0), out_proj(1)
        assert not pc.events

    def _mlp_item():
        item = step - SKEW
        blk = item & (NB - 1)
        base = pl.multiple_of(blk * T, T)

        nbase = pl.multiple_of(((item + 1) & (NB - 1)) * T, T)

        pc = _Pacer(att, zero_ref[0])

        def ln_piece(row0, dst, c):
            xn = _ln_packed(xs[pl.ds(row0 + c * 16, 16), :])
            dst[8 * c:8 * c + 8, :] = xn
            pc.pin(xn, hard=True)

        pc.spread([functools.partial(ln_piece, base + C, xn2_b, c) for c in range(C // 16)], *N2B)
        pc.spread([functools.partial(ln_piece, nbase, xn2_a, c) for c in range(C // 16)], *N2A)

        def mish(h):
            ex = jnp.exp(jnp.minimum(h, 30.0))
            n = ex * (ex + 2.0)
            return (h * n * pl.reciprocal(n + 2.0, approx=True)).astype(bf16)

        def mlp1(xn):
            act = []
            for n in range(NF):
                r = _dot(pc.tie(xn), w1_v, n)
                pc.tile(r)
                act.append(mish(r + b1_v[n:n + 1, :].astype(f32)))
            return jnp.concatenate(act, axis=1)

        act_a = mlp1(_as_bf16(xn2_a[...]))
        act_b = mlp1(_as_bf16(xn2_b[...]))
        for act, r0 in ((act_a, base), (act_b, base + C)):
            for n in range(NG):
                r = _dot(pc.tie(act), w2_v, n) + xs[pl.ds(r0, C), n * 128:(n + 1) * 128].astype(f32)
                pc.tile(r)
                xs[pl.ds(r0, C), n * 128:(n + 1) * 128] = r.astype(bf16)
                cuts = OUT_CUTS if r0 is not base else (NG,)
                if n + 1 in cuts:
                    n0 = ([0] + [c for c in cuts if c <= n])[-1]

                    @pl.when(item >= NITEM - NB)
                    def _():
                        out_copy(r0, n0 * 128, (n + 1 - n0) * 128).start()
        assert not pc.events

        @pl.when(item == NITEM - 1)
        def _():
            pltpu.make_async_copy(xs, out_hbm, sems.at[SEM_O]).wait()

    @pl.when((step <= SKEW + 1) | (step == NITEM + 1))
    def _():
        pl.when(step == 0)(prologue)
        pl.when(step == SKEW)(first_mlp_prep)
        for k in range(1, SKEW + 1):
            pl.when(step == k)(x_copy(k + 1).wait)

        @pl.when(step == SKEW + 1)
        def _():
            for k in range(SKEW + 2, NB + 1):
                x_copy(k).wait()

        pl.when(step == NITEM + 1)(functools.partial(attention, 'last'))

    pl.when(step >= SKEW)(_mlp_item)
    pl.when((step >= 1) & (step < NITEM))(functools.partial(attention, 'mid'))


@jax.jit
def pallas_interleave_layers__sliding_local_dilated__dense_activation_mish__prompt_kernel(A_x, A_wqkv, A_wo, B_x, B_w1, B_b1, B_w2):
    x = A_x.reshape(S, D)
    b1 = B_b1.reshape(NF, 128)
    out = pl.pallas_call(
        _kernel,
        grid=(NITEM + SKEW,),
        in_specs=[pl.BlockSpec(memory_space=pl.ANY)] * 6,
        out_specs=pl.BlockSpec(memory_space=pl.ANY),
        out_shape=jax.ShapeDtypeStruct((S, D), bf16),
        scratch_shapes=[
            pltpu.VMEM((3, D, D), bf16), pltpu.VMEM((3, D // 2, D), i32),
            pltpu.VMEM((D, D), bf16), pltpu.VMEM((NG, NG * PITCH, 128), i32), pltpu.VMEM((NG, 128, 128), bf16),
            pltpu.VMEM((D // 2, D), i32),
            pltpu.VMEM((D, F), bf16), pltpu.VMEM((F, D), bf16), pltpu.VMEM((NF, 128), bf16),
            pltpu.VMEM((S, D), bf16), pltpu.VMEM((3, C // 2, D), i32),
            pltpu.VMEM((C // 2, D), i32), pltpu.VMEM((C // 2, D), i32),
            pltpu.VMEM((NSLOT, NG, C + HALO, 128), f32),
            pltpu.VMEM((C // 2, D), i32), pltpu.VMEM((C // 2, D), i32),
            pltpu.VMEM((NG, HALO, 128), f32), pltpu.VMEM((NG, HALO, 128), f32),
            pltpu.SMEM((1,), i32),
            pltpu.SemaphoreType.DMA((NSEM,)),
        ],
        compiler_params=pltpu.CompilerParams(
            dimension_semantics=("arbitrary",), vmem_limit_bytes=100 * 1024 * 1024),
        name="fused",
    )(x, b1, A_wqkv, A_wo, B_w1, B_w2)
    return out.reshape(1, S, D)
```

```python
import functools
import jax
import jax.numpy as jnp
from jax import lax
import jax.experimental.pallas as pl
import jax.experimental.pallas.tpu as pltpu

S, D, F = 2048, 1024, 3584
H, DH, W, DIL = 32, 32, 8, 2
NG = D // 128
NF = F // 128
HALO = 16
T = 256
C = T // 2
R = 8
NCH = C // R
NB = S // T
NITEM = 2 * NB
SKEW = 3
EPS = 1e-5
f32, bf16, i32 = jnp.float32, jnp.bfloat16, jnp.int32
QA, KA, VA, QB, KB, VB, PA, PB, DUMMY, PIN = range(10)
NSLOT = PIN + 1
LA, AA, LB, AB = (15, 16), (55.3, 7.2), (39, 16), (0.3, 7.5)
N1B, N1N, N2A, N2B = (8, 7), (32, 5), (56.5, 8), (1, 20)
FAA = (48.3, 3.5)
FN1B, FN1N = (0, 3.5), (3.5, 3)
LAG = 1.5
AVLAG = 0.2
OUT_CUTS = (4, 6, 7, 8)
LNLAG = 1.2
WOS, WOG = (44, 4), (48, 3.8)
FT = [(t0 + i * dt, dt) for t0, dt, n in ((28, 0.5, 6), (32, 0.56, 20), (44, 0.6, 6)) for i in range(n)]
FLAG = 1.7
NWCH = 4
SEM_X, SEM_W, SEM_O, SEM_Q, NSEM = 0, NB + 1, NB + 5, NB + 6, NB + 10 + NWCH
PITCH = 65


def _layernorm(x):
    m = jnp.mean(x, axis=-1, keepdims=True)
    xc = x - m
    v = jnp.mean(xc * xc, axis=-1, keepdims=True)
    return xc * lax.rsqrt(v + EPS)


def _ln_packed(x, zeros=None):
    x = x.astype(f32)
    if zeros is not None:
        x = jnp.concatenate([x[:, 0:128] + jnp.concatenate([zeros, zeros], axis=0), x[:, 128:]], axis=1)
    return pltpu.bitcast(_layernorm(x).astype(bf16), i32)


def _perm_matrix(j):
    src = lax.broadcasted_iota(i32, (128, 128), 0)
    m = lax.broadcasted_iota(i32, (128, 128), 1)
    jp = (j + 128 - m) & 7
    l = (m + jp) & 127
    want = 32 * ((l >> 3) & 3) + 4 * jp + (l >> 5)
    return jnp.where(src == want, 1.0, 0.0).astype(bf16)


def _perm_pattern(j, r):
    m = lax.broadcasted_iota(i32, (r, 128), 1)
    jp = (j + 128 - m) & 7
    l = (m + jp) & 127
    return 32 * ((l >> 3) & 3) + 4 * jp + (l >> 5)


def _exchange_and_roll(mid):
    lane = lax.broadcasted_iota(i32, mid[0].shape, 1)
    for b in (1, 2, 4):
        m = (lane & b) != 0
        mid = [jnp.where(m, mid[(j + b) % 8], mid[j]) for j in range(8)]
    return [g if j == 0 else pltpu.roll(g, j, 1) for j, g in enumerate(mid)]


def _as_bf16(v):
    return v if v.dtype == bf16 else pltpu.bitcast(v, bf16)


def _dot(x, w_ref, n):
    return jnp.dot(x, _as_bf16(w_ref[:, n * 128:(n + 1) * 128]), preferred_element_type=f32)


class _Pacer:
    def __init__(self, att, z):
        self.att, self.z, self.events, self.t, self.now = att, z, [], 0, 0

    def at(self, t, piece):
        self.events.append((t, len(self.events), piece))
        self.events.sort(key=lambda e: e[:2])

    def spread(self, pieces, t0, dur):
        for i, p in enumerate(pieces):
            self.at(t0 + dur * (i + 0.5) / len(pieces), p)

    def later(self, dt, piece):
        self.at(self.now + dt, piece)

    def tie(self, lhs):
        if not self.tied:
            return lhs
        dep = functools.reduce(jnp.bitwise_or, self.tied) & self.z
        self.tied = []
        a00 = pltpu.bitcast(pltpu.bitcast(lhs[0:16, 0:128], i32) | dep, bf16)
        return jnp.concatenate([jnp.concatenate([a00, lhs[0:16, 128:]], axis=1), lhs[16:]], axis=0)

    def pin(self, words, hard=False):
        v = functools.reduce(jnp.bitwise_or, [words[:, j * 128:(j + 1) * 128] for j in range(words.shape[1] // 128)])
        if hard:
            self.tied = self.tied + [v]
            return
        k, self.npin = self.npin, self.npin + 1
        per = (C + HALO) // 8
        self.att[PIN + k // (NG * per), (k // per) % NG, 8 * (k % per):8 * (k % per) + 8, :] = pltpu.bitcast(v, f32)

    def tile(self, r, slot=None, j=None, dur=1):
        nst = C // 8
        for i in range(nst):
            lim = self.t + dur * (i + 1) / nst
            fence = self.events and self.events[0][0] < lim
            if slot is not None:
                self.att[slot + self.z if fence else slot, j, HALO + 8 * i:HALO + 8 * i + 8, :] = r[8 * i:8 * i + 8]
            elif fence:
                self.att[DUMMY + self.z, 0, 0:8, :] = r[8 * i:8 * i + 8]
            if fence and self.aux is not None:
                n = self.aux.shape[1]
                self.aux[self.z, n - 8:n, :] = pltpu.bitcast(r[8 * i:8 * i + 8], i32)
            self.now = lim
            while self.events and self.events[0][0] < lim:
                self.events.pop(0)[2]()
        self.t += dur

    npin = 0
    aux = None
    tied = []


def _kernel(x_hbm, b1_hbm, wqkv_hbm, wo_hbm, w1_hbm, w2_hbm, out_hbm,
            wqkv_raw, wqkv_p, wo_raw, wo_stage, pm, wo_p, w1_v, w2_v, b1_v,
            xs, xn1, xn2_a, xn2_b, att, o_a, o_b, hk, hv, zero_ref, sems):
    step = pl.program_id(0)
    xn_a, xn_b, xn_n = xn1.at[0], xn1.at[1], xn1.at[2]

    def x_copy(k):
        r0, r1 = max(k * T - C, 0), min(k * T + C, S)
        return pltpu.make_async_copy(x_hbm.at[pl.ds(r0, r1 - r0)], xs.at[pl.ds(r0, r1 - r0)], sems.at[SEM_X + k])

    def out_copy(r0, c0, nc):
        return pltpu.make_async_copy(xs.at[pl.ds(r0, C), pl.ds(c0, nc)], out_hbm.at[pl.ds(r0, C), pl.ds(c0, nc)],
                                     sems.at[SEM_O])

    rows = D // NWCH

    def q_copy(p, r0, n, k):
        return pltpu.make_async_copy(wqkv_hbm.at[pl.ds(r0, n), pl.ds(p * D, D)],
                                     wqkv_raw.at[p, pl.ds(r0, n)], sems.at[SEM_Q + k])

    kv_cps = [[q_copy(p, h * (D // 2), D // 2, NWCH + 2 * (p - 1) + h) for h in range(2)] for p in (1, 2)]
    wo_cp = pltpu.make_async_copy(wo_hbm, wo_raw, sems.at[SEM_W + 0])
    w1_cp = pltpu.make_async_copy(w1_hbm, w1_v, sems.at[SEM_W + 1])
    w2_cp = pltpu.make_async_copy(w2_hbm, w2_v, sems.at[SEM_W + 2])
    b1_cp = pltpu.make_async_copy(b1_hbm, b1_v, sems.at[SEM_W + 3])

    def permute(p, r0, pc=None):
        r1 = r0 // 2 if isinstance(r0, int) else pl.multiple_of(r0 >> 1, rows // 2)
        mid = []
        for j in range(NG):
            r = jnp.dot(wqkv_raw[p, pl.ds(r0, rows), j * 128:(j + 1) * 128], pm[j], preferred_element_type=f32)
            if pc is not None and j % 4 == 3:
                pc.tile(r[rows - C:rows])
            mid.append(pltpu.bitcast(r.astype(bf16), i32))
        outs = _exchange_and_roll(mid)
        for j in range(NG):
            wqkv_p[p, pl.ds(r1, rows // 2), j * 128:(j + 1) * 128] = outs[j]

    def permute_xlu(p, r0, n):
        w0, w1 = r0 // 2, (r0 + n) // 2
        for j in range(NG):
            words = pltpu.bitcast(wqkv_raw[p, r0:r0 + n, j * 128:(j + 1) * 128], i32)
            wqkv_p[p, w0:w1, j * 128:(j + 1) * 128] = jnp.take_along_axis(
                words, _perm_pattern(j, n // 2), axis=1, mode="promise_in_bounds")
        for w in range(w0, w1, 8):
            outs = _exchange_and_roll([wqkv_p[p, w:w + 8, j * 128:(j + 1) * 128] for j in range(NG)])
            for j in range(NG):
                wqkv_p[p, w:w + 8, j * 128:(j + 1) * 128] = outs[j]

    def prologue():
        x_copy(0).start()
        for k in range(NWCH):
            q_copy(0, k * rows, rows, k).start()
        x_copy(1).start()
        for cp in kv_cps[0] + kv_cps[1]:
            cp.start()
        wo_cp.start()
        for k in range(2, SKEW + 1):
            x_copy(k).start()
        b1_cp.start()
        w1_cp.start()
        w2_cp.start()
        for k in range(SKEW + 1, NB + 1):
            x_copy(k).start()
        zero_ref[0] = 0
        hk[...] = jnp.zeros(hk.shape, f32)
        att[DUMMY, 1, 0:8, :] = jnp.zeros((8, 128), f32)
        hv[...] = jnp.zeros(hv.shape, f32)
        for j in range(NG):
            pm[j] = _perm_matrix(j)
        x_copy(0).wait()
        xn_a[...] = _ln_packed(xs[0:C, :])

        def body(k, c):
            r0 = pl.multiple_of(k * rows, rows)
            q_copy(0, r0, rows, k).wait()
            permute(0, r0)
            return c
        lax.fori_loop(0, NWCH, body, 0)
        x_copy(1).wait()

        attention('first')

    def wo_stage_piece(j, g0, g1):
        words = pltpu.bitcast(wo_raw[j * 128:(j + 1) * 128, g0 * 128:g1 * 128], i32)
        for g in range(g0, g1):
            for a in range(4):
                r0 = PITCH * (j // 2 + 4 * (a % 2)) + 32 * (j % 2) + 16 * (a // 2)
                wo_stage[g, r0:r0 + 16, :] = words[16 * a:16 * a + 16, (g - g0) * 128:(g - g0 + 1) * 128]

    def wo_gather_piece(jp, th, ah):
        for g in range(NG):
            ev = wo_stage[g, pl.ds(16 * ah + 2 * jp + th, 8, stride=PITCH), :]
            od = wo_stage[g, pl.ds(32 + 16 * ah + 2 * jp + th, 8, stride=PITCH), :]
            lo = (ev & 0xFFFF) | lax.shift_left(od, 16)
            hi = lax.shift_right_logical(ev, 16) | (od & -0x10000)
            for t, v in ((2 * th, lo), (2 * th + 1, hi)):
                w0 = jp * 64 + 16 * t + 8 * ah
                wo_p[w0:w0 + 8, g * 128:(g + 1) * 128] = v

    def first_mlp_prep():
        xn2_a[...] = _ln_packed(xs[0:C, :])
        b1_cp.wait()
        w1_cp.wait()
        w2_cp.wait()

    def attention(kind):
        if kind == 'mid':
            blk = step & (NB - 1)
            base = pl.multiple_of(blk * T, T)
            nbase = pl.multiple_of(((step + 1) & (NB - 1)) * T, T)
            pbase = pl.multiple_of(((step - 1) & (NB - 1)) * T, T)
        elif kind == 'first':
            blk, base, nbase = 0, 0, T
        else:
            pbase = S - T

        pc = _Pacer(att, zero_ref[0])
        scale = DH ** -0.5

        def logits_pieces(qs, ks, ps, c, first):
            r0 = c * R
            st = {}

            def piece(w):
                if w == 0:
                    st['q'] = att[qs, :, HALO + r0:HALO + r0 + R, :]
                    st['lg'] = []
                kw = att[ks, :, pl.ds(HALO + r0 - DIL * w, R), :]
                p = jnp.sum(st['q'] * kw, axis=0)
                p = p + pltpu.roll(p, 64, 1)
                p = p + pltpu.roll(p, 32, 1)
                if first and r0 < DIL * w:
                    row = lax.broadcasted_iota(i32, (R, 128), 0) + blk * T
                    p = jnp.where(row + r0 >= DIL * w, p, -1e9 / scale)
                st['lg'].append(p)

            def softmax():
                lg = st['lg']
                m = functools.reduce(jnp.maximum, lg)
                e = [jnp.exp2((p - m) * (scale * 1.4426950408889634)) for p in lg]
                inv = pl.reciprocal(functools.reduce(jnp.add, e), approx=True)
                for w in range(W):
                    att[ps, w, r0:r0 + R, :] = e[w] * inv
            return [functools.partial(piece, w) for w in range(W)], softmax

        def av_pieces(ps, vs, o_s, c):
            r0 = c * 16
            st = {}

            def piece(j):
                if j == 0:
                    st['a'] = att[ps, :, r0:r0 + 16, :]
                a = st['a']
                acc = a[0] * att[vs, j, pl.ds(HALO + r0, 16), :]
                for w in range(1, W):
                    acc = acc + a[w] * att[vs, j, pl.ds(HALO + r0 - DIL * w, 16), :]
                o = pltpu.bitcast(acc.astype(bf16), i32)
                o_s[r0 // 2:r0 // 2 + 8, j * 128:(j + 1) * 128] = o
                pc.later(AVLAG, lambda: pc.pin(o))
            return [functools.partial(piece, j) for j in range(NG)]

        def ln1_piece(row0, dst, c):
            rel = kind == 'mid' and dst is xn_n
            xn = _ln_packed(xs[pl.ds(row0 + c * 16, 16), :], att[DUMMY, 1, 0:8, :] if rel else None)
            dst[8 * c:8 * c + 8, :] = xn
            if rel:
                pc.later(LNLAG, lambda: pc.pin(xn))
            else:
                pc.pin(xn)

        if kind != 'last':
            aa = AA if kind == 'mid' else FAA
            for (qs, ks, ps, first, (t0, n)) in ((QA, KA, PA, True, LA), (QB, KB, PB, False, LB)):
                for c in range(NCH):
                    pcs, sm = logits_pieces(qs, ks, ps, c, first)
                    ts, dt = (t0 + c * n / NCH, n / NCH) if kind == 'mid' else FT[(0 if first else NCH) + c]
                    pc.spread(pcs, ts, dt)
                    pc.at(ts + dt + (LAG if kind == 'mid' else FLAG), sm)
            pc.spread([p for c in range(C // 16) for p in av_pieces(PA, VA, o_a, c)], *aa)
            n1b, n1n = (N1B, N1N) if kind == 'mid' else (FN1B, FN1N)
            pc.spread([functools.partial(ln1_piece, base + C, xn_b, c) for c in range(C // 16)], *n1b)
            pc.spread([functools.partial(ln1_piece, nbase, xn_n, c) for c in range(C // 16)], *n1n)
            att[KA, :, 0:HALO, :] = hk[...]
            att[VA, :, 0:HALO, :] = hv[...]
        if kind != 'first':
            pc.spread([p for c in range(C // 16) for p in av_pieces(PB, VB, o_b, c)], *AB)

        def proj(chain, part, half=None):
            slot = (QB if chain else QA) + part
            src = xn_b if chain else xn_a
            if half is None:
                xn, w_ref = _as_bf16(src[...]), wqkv_p.at[part]
            else:
                xn = _as_bf16(src[:, half * (D // 2):(half + 1) * (D // 2)])
                w_ref = wqkv_p.at[part, half * (D // 4):(half + 1) * (D // 4)]
            for j in range(NG):
                r = _dot(xn, w_ref, j)
                if half == 1:
                    r = r + att[slot, j, HALO:HALO + C, :]
                if part > 0 and half != 0:
                    if chain == 0:
                        att[QB + part, j, 0:HALO, :] = r[C - HALO:C]
                    else:
                        (hk if part == 1 else hv)[j] = r[C - HALO:C]
                pc.tile(r, slot, j, dur=1 if half is None else 0.5)

        def out_proj(chain):
            r0 = pbase + chain * C
            o = _as_bf16((o_b if chain else o_a)[...])
            for n in range(NG):
                r = _dot(o, wo_p, n) + xs[pl.ds(r0, C), n * 128:(n + 1) * 128].astype(f32)
                pc.tile(r)
                xs[pl.ds(r0, C), n * 128:(n + 1) * 128] = r.astype(bf16)

        if kind == 'mid':
            proj(0, 0), proj(0, 1), out_proj(0), proj(1, 0), proj(1, 1), proj(0, 2), out_proj(1)
            xn_a[...] = xn_n[...]
            proj(1, 2)
        elif kind == 'first':
            proj(0, 0)
            kv_cps[0][0].wait()
            permute_xlu(1, 0, D // 2)
            proj(1, 0)
            kv_cps[0][1].wait()
            permute_xlu(1, D // 2, D // 2)
            proj(0, 1, 0), proj(1, 1, 0)
            kv_cps[1][0].wait()
            permute_xlu(2, 0, D // 2)
            proj(0, 1, 1), proj(1, 1, 1)
            kv_cps[1][1].wait()
            permute(2, 2 * rows, pc), permute(2, 3 * rows, pc)
            proj(0, 2, 0), proj(1, 2, 0)
            wo_cp.wait()
            pc.aux = wo_stage
            pc.spread([functools.partial(wo_stage_piece, j, g, g + 2)
                       for j in range(NG) for g in range(0, NG, 2)], *WOS)
            pc.spread([functools.partial(wo_gather_piece, jp, th, ah)
                       for jp in range(NG) for th in range(2) for ah in range(2)], *WOG)
            proj(0, 2, 1)
            xn_a[...] = xn_n[...]
            proj(1, 2, 1)
        else:
            out_proj(0), out_proj(1)
        assert not pc.events

    def _mlp_item():
        item = step - SKEW
        blk = item & (NB - 1)
        base = pl.multiple_of(blk * T, T)
        nbase = pl.multiple_of(((item + 1) & (NB - 1)) * T, T)

        pc = _Pacer(att, zero_ref[0])

        def ln_piece(row0, dst, c):
            xn = _ln_packed(xs[pl.ds(row0 + c * 16, 16), :])
            dst[8 * c:8 * c + 8, :] = xn
            pc.pin(xn, hard=True)

        pc.spread([functools.partial(ln_piece, base + C, xn2_b, c) for c in range(C // 16)], *N2B)
        pc.spread([functools.partial(ln_piece, nbase, xn2_a, c) for c in range(C // 16)], *N2A)

        def mish(h):
            ex = jnp.exp(jnp.minimum(h, 30.0))
            n = ex * (ex + 2.0)
            return (h * n * pl.reciprocal(n + 2.0, approx=True)).astype(bf16)

        def mlp1(xn):
            act = []
            for n in range(NF):
                r = _dot(pc.tie(xn), w1_v, n)
                pc.tile(r)
                act.append(mish(r + b1_v[n:n + 1, :].astype(f32)))
            return jnp.concatenate(act, axis=1)

        act_a = mlp1(_as_bf16(xn2_a[...]))
        act_b = mlp1(_as_bf16(xn2_b[...]))
        for act, r0 in ((act_a, base), (act_b, base + C)):
            for n in range(NG):
                r = _dot(pc.tie(act), w2_v, n) + xs[pl.ds(r0, C), n * 128:(n + 1) * 128].astype(f32)
                pc.tile(r)
                xs[pl.ds(r0, C), n * 128:(n + 1) * 128] = r.astype(bf16)
                cuts = OUT_CUTS if r0 is not base else (NG,)
                if n + 1 in cuts:
                    n0 = ([0] + [c for c in cuts if c <= n])[-1]

                    @pl.when(item >= NITEM - NB)
                    def _():
                        out_copy(r0, n0 * 128, (n + 1 - n0) * 128).start()
        assert not pc.events

        @pl.when(item == NITEM - 1)
        def _():
            pltpu.make_async_copy(xs, out_hbm, sems.at[SEM_O]).wait()

    @pl.when((step <= SKEW + 1) | (step == NITEM + 1))
    def _():
        pl.when(step == 0)(prologue)
        pl.when(step == SKEW)(first_mlp_prep)
        for k in range(1, SKEW + 1):
            pl.when(step == k)(x_copy(k + 1).wait)

        @pl.when(step == SKEW + 1)
        def _():
            for k in range(SKEW + 2, NB + 1):
                x_copy(k).wait()

        pl.when(step == NITEM + 1)(functools.partial(attention, 'last'))

    pl.when(step >= SKEW)(_mlp_item)
    pl.when((step >= 1) & (step < NITEM))(functools.partial(attention, 'mid'))


@jax.jit
def pallas_interleave_layers__sliding_local_dilated__dense_activation_mish__prompt_kernel(A_x, A_wqkv, A_wo, B_x, B_w1, B_b1, B_w2):
    x = A_x.reshape(S, D)
    b1 = B_b1.reshape(NF, 128)
    out = pl.pallas_call(
        _kernel,
        grid=(NITEM + SKEW,),
        in_specs=[pl.BlockSpec(memory_space=pl.ANY)] * 6,
        out_specs=pl.BlockSpec(memory_space=pl.ANY),
        out_shape=jax.ShapeDtypeStruct((S, D), bf16),
        scratch_shapes=[
            pltpu.VMEM((3, D, D), bf16), pltpu.VMEM((3, D // 2, D), i32),
            pltpu.VMEM((D, D), bf16), pltpu.VMEM((NG, NG * PITCH + 8, 128), i32), pltpu.VMEM((NG, 128, 128), bf16),
            pltpu.VMEM((D // 2, D), i32),
            pltpu.VMEM((D, F), bf16), pltpu.VMEM((F, D), bf16), pltpu.VMEM((NF, 128), bf16),
            pltpu.VMEM((S, D), bf16), pltpu.VMEM((3, C // 2, D), i32),
            pltpu.VMEM((C // 2, D), i32), pltpu.VMEM((C // 2, D), i32),
            pltpu.VMEM((NSLOT, NG, C + HALO, 128), f32),
            pltpu.VMEM((C // 2, D), i32), pltpu.VMEM((C // 2, D), i32),
            pltpu.VMEM((NG, HALO, 128), f32), pltpu.VMEM((NG, HALO, 128), f32),
            pltpu.SMEM((1,), i32),
            pltpu.SemaphoreType.DMA((NSEM,)),
        ],
        compiler_params=pltpu.CompilerParams(
            dimension_semantics=("arbitrary",), vmem_limit_bytes=100 * 1024 * 1024),
        name="fused",
    )(x, b1, A_wqkv, A_wo, B_w1, B_w2)
    return out.reshape(1, S, D)
```

```python
import functools
import jax
import jax.numpy as jnp
from jax import lax
import jax.experimental.pallas as pl
import jax.experimental.pallas.tpu as pltpu

S, D, F = 2048, 1024, 3584
H, DH, W, DIL = 32, 32, 8, 2
NG = D // 128
NF = F // 128
HALO = 16
T = 256
C = T // 2
R = 8
NCH = C // R
NB = S // T
NITEM = 2 * NB
SKEW = 3
EPS = 1e-5
f32, bf16, i32 = jnp.float32, jnp.bfloat16, jnp.int32
QA, KA, VA, QB, KB, VB, PA, PB, DUMMY, PIN = range(10)
NSLOT = PIN + 1
LA, AA, LB, AB = (15, 16), (55.3, 7.2), (39, 16), (0.3, 7.5)
N1B, N1N, N2A, N2B = (8, 7), (32, 5), (57, 8), (2, 22)
FAA = (48.3, 3.5)
FN1B, FN1N = (0, 3.5), (3.5, 3)
LAG = 1.5
AVLAG = 0.2
OUT_CUTS = (4, 6, 7, 8)
LNLAG = 1.0
WOS, WOG = (44, 4), (48, 3.8)
FT = [(t0 + i * dt, dt) for t0, dt, n in ((28, 0.5, 6), (32, 0.56, 20), (44, 0.6, 6)) for i in range(n)]
FLAG = 1.4
AROWS = C + HALO + 8
NWCH = 4
SEM_X, SEM_W, SEM_O, SEM_Q, NSEM = 0, NB + 1, NB + 5, NB + 6, NB + 10 + NWCH
PITCH = 65


def _layernorm(x):
    m = jnp.mean(x, axis=-1, keepdims=True)
    xc = x - m
    v = jnp.mean(xc * xc, axis=-1, keepdims=True)
    return xc * lax.rsqrt(v + EPS)


def _ln_packed(x, zeros=None):
    x = x.astype(f32)
    if zeros is not None:
        x = jnp.concatenate([x[:, 0:128] + jnp.concatenate([zeros, zeros], axis=0), x[:, 128:]], axis=1)
    return pltpu.bitcast(_layernorm(x).astype(bf16), i32)


def _perm_matrix(j):
    src = lax.broadcasted_iota(i32, (128, 128), 0)
    m = lax.broadcasted_iota(i32, (128, 128), 1)
    jp = (j + 128 - m) & 7
    l = (m + jp) & 127
    want = 32 * ((l >> 3) & 3) + 4 * jp + (l >> 5)
    return jnp.where(src == want, 1.0, 0.0).astype(bf16)


def _perm_pattern(j, r):
    m = lax.broadcasted_iota(i32, (r, 128), 1)
    jp = (j + 128 - m) & 7
    l = (m + jp) & 127
    return 32 * ((l >> 3) & 3) + 4 * jp + (l >> 5)


def _exchange_and_roll(mid):
    lane = lax.broadcasted_iota(i32, mid[0].shape, 1)
    for b in (1, 2, 4):
        m = (lane & b) != 0
        mid = [jnp.where(m, mid[(j + b) % 8], mid[j]) for j in range(8)]
    return [g if j == 0 else pltpu.roll(g, j, 1) for j, g in enumerate(mid)]


def _as_bf16(v):
    return v if v.dtype == bf16 else pltpu.bitcast(v, bf16)


def _dot(x, w_ref, n):
    return jnp.dot(x, _as_bf16(w_ref[:, n * 128:(n + 1) * 128]), preferred_element_type=f32)


class _Pacer:
    def __init__(self, att, z):
        self.att, self.z, self.events, self.t, self.now = att, z, [], 0, 0

    def at(self, t, piece):
        self.events.append((t, len(self.events), piece))
        self.events.sort(key=lambda e: e[:2])

    def spread(self, pieces, t0, dur):
        for i, p in enumerate(pieces):
            self.at(t0 + dur * (i + 0.5) / len(pieces), p)

    def later(self, dt, piece):
        self.at(self.now + dt, piece)

    def tie(self, lhs):
        if not self.tied:
            return lhs
        dep = functools.reduce(jnp.bitwise_or, self.tied) & self.z
        self.tied = []
        a00 = pltpu.bitcast(pltpu.bitcast(lhs[0:16, 0:128], i32) | dep, bf16)
        return jnp.concatenate([jnp.concatenate([a00, lhs[0:16, 128:]], axis=1), lhs[16:]], axis=0)

    def pin(self, words, hard=False):
        v = functools.reduce(jnp.bitwise_or, [words[:, j * 128:(j + 1) * 128] for j in range(words.shape[1] // 128)])
        if hard:
            self.tied = self.tied + [v]
            return
        k, self.npin = self.npin, self.npin + 1
        per = (C + HALO) // 8
        self.att[PIN + k // (NG * per), (k // per) % NG, 8 * (k % per):8 * (k % per) + 8, :] = pltpu.bitcast(v, f32)

    def tile(self, r, slot=None, j=None, dur=1):
        nst = C // 8
        for i in range(nst):
            lim = self.t + dur * (i + 1) / nst
            fence = self.events and self.events[0][0] < lim
            if slot is not None:
                self.att[slot + self.z if fence else slot, j, HALO + 8 * i:HALO + 8 * i + 8, :] = r[8 * i:8 * i + 8]
            elif fence:
                self.att[DUMMY + self.z, 0, 0:8, :] = r[8 * i:8 * i + 8]
            if fence and self.aux is not None:
                n = self.aux.shape[1]
                self.aux[self.z, n - 8:n, :] = pltpu.bitcast(r[8 * i:8 * i + 8], i32)
            self.now = lim
            while self.events and self.events[0][0] < lim:
                self.events.pop(0)[2]()
        self.t += dur

    npin = 0
    aux = None
    tied = []


def _kernel(x_hbm, b1_hbm, wqkv_hbm, wo_hbm, w1_hbm, w2_hbm, out_hbm,
            wqkv_raw, wqkv_p, wo_raw, wo_stage, pm, wo_p, w1_v, w2_v, b1_v,
            xs, xn1, xn2_a, xn2_b, att, o_a, o_b, hk, hv, zero_ref, sems):
    step = pl.program_id(0)
    xn_a, xn_b, xn_n = xn1.at[0], xn1.at[1], xn1.at[2]

    def x_copy(k):
        r0, r1 = max(k * T - C, 0), min(k * T + C, S)
        return pltpu.make_async_copy(x_hbm.at[pl.ds(r0, r1 - r0)], xs.at[pl.ds(r0, r1 - r0)], sems.at[SEM_X + k])

    def out_copy(r0, c0, nc):
        return pltpu.make_async_copy(xs.at[pl.ds(r0, C), pl.ds(c0, nc)], out_hbm.at[pl.ds(r0, C), pl.ds(c0, nc)],
                                     sems.at[SEM_O])

    rows = D // NWCH

    def q_copy(p, r0, n, k):
        return pltpu.make_async_copy(wqkv_hbm.at[pl.ds(r0, n), pl.ds(p * D, D)],
                                     wqkv_raw.at[p, pl.ds(r0, n)], sems.at[SEM_Q + k])

    kv_cps = [[q_copy(p, h * (D // 2), D // 2, NWCH + 2 * (p - 1) + h) for h in range(2)] for p in (1, 2)]
    wo_cp = pltpu.make_async_copy(wo_hbm, wo_raw, sems.at[SEM_W + 0])
    w1_cp = pltpu.make_async_copy(w1_hbm, w1_v, sems.at[SEM_W + 1])
    w2_cp = pltpu.make_async_copy(w2_hbm, w2_v, sems.at[SEM_W + 2])
    b1_cp = pltpu.make_async_copy(b1_hbm, b1_v, sems.at[SEM_W + 3])

    def permute(p, r0, pc=None):
        r1 = r0 // 2 if isinstance(r0, int) else pl.multiple_of(r0 >> 1, rows // 2)
        mid = []
        for j in range(NG):
            r = jnp.dot(wqkv_raw[p, pl.ds(r0, rows), j * 128:(j + 1) * 128], pm[j], preferred_element_type=f32)
            if pc is not None and j % 4 == 3:
                pc.tile(r[rows - C:rows])
            mid.append(pltpu.bitcast(r.astype(bf16), i32))
        outs = _exchange_and_roll(mid)
        for j in range(NG):
            wqkv_p[p, pl.ds(r1, rows // 2), j * 128:(j + 1) * 128] = outs[j]

    def permute_xlu(p, r0, n):
        w0, w1 = r0 // 2, (r0 + n) // 2
        for j in range(NG):
            words = pltpu.bitcast(wqkv_raw[p, r0:r0 + n, j * 128:(j + 1) * 128], i32)
            wqkv_p[p, w0:w1, j * 128:(j + 1) * 128] = jnp.take_along_axis(
                words, _perm_pattern(j, n // 2), axis=1, mode="promise_in_bounds")
        for w in range(w0, w1, 8):
            outs = _exchange_and_roll([wqkv_p[p, w:w + 8, j * 128:(j + 1) * 128] for j in range(NG)])
            for j in range(NG):
                wqkv_p[p, w:w + 8, j * 128:(j + 1) * 128] = outs[j]

    def prologue():
        x_copy(0).start()
        for k in range(NWCH):
            q_copy(0, k * rows, rows, k).start()
        x_copy(1).start()
        for cp in kv_cps[0] + kv_cps[1]:
            cp.start()
        wo_cp.start()
        for k in range(2, SKEW + 1):
            x_copy(k).start()
        b1_cp.start()
        w1_cp.start()
        w2_cp.start()
        for k in range(SKEW + 1, NB + 1):
            x_copy(k).start()
        zero_ref[0] = 0
        hk[...] = jnp.zeros(hk.shape, f32)
        att[DUMMY, 1, 0:8, :] = jnp.zeros((8, 128), f32)
        hv[...] = jnp.zeros(hv.shape, f32)
        for j in range(NG):
            pm[j] = _perm_matrix(j)
        x_copy(0).wait()
        xn_a[...] = _ln_packed(xs[0:C, :])

        def body(k, c):
            r0 = pl.multiple_of(k * rows, rows)
            q_copy(0, r0, rows, k).wait()
            permute(0, r0)
            return c
        lax.fori_loop(0, NWCH, body, 0)
        x_copy(1).wait()

        attention('first')

    def wo_stage_piece(j, g0, g1):
        words = pltpu.bitcast(wo_raw[j * 128:(j + 1) * 128, g0 * 128:g1 * 128], i32)
        for g in range(g0, g1):
            for a in range(4):
                r0 = PITCH * (j // 2 + 4 * (a % 2)) + 32 * (j % 2) + 16 * (a // 2)
                wo_stage[g, r0:r0 + 16, :] = words[16 * a:16 * a + 16, (g - g0) * 128:(g - g0 + 1) * 128]

    def wo_gather_piece(jp, th, ah):
        for g in range(NG):
            ev = wo_stage[g, pl.ds(16 * ah + 2 * jp + th, 8, stride=PITCH), :]
            od = wo_stage[g, pl.ds(32 + 16 * ah + 2 * jp + th, 8, stride=PITCH), :]
            lo = (ev & 0xFFFF) | lax.shift_left(od, 16)
            hi = lax.shift_right_logical(ev, 16) | (od & -0x10000)
            for t, v in ((2 * th, lo), (2 * th + 1, hi)):
                w0 = jp * 64 + 16 * t + 8 * ah
                wo_p[w0:w0 + 8, g * 128:(g + 1) * 128] = v

    def first_mlp_prep():
        xn2_a[...] = _ln_packed(xs[0:C, :])
        b1_cp.wait()
        w1_cp.wait()
        w2_cp.wait()

    def attention(kind):
        if kind == 'mid':
            blk = step & (NB - 1)
            base = pl.multiple_of(blk * T, T)
            nbase = pl.multiple_of(((step + 1) & (NB - 1)) * T, T)
            pbase = pl.multiple_of(((step - 1) & (NB - 1)) * T, T)
        elif kind == 'first':
            blk, base, nbase = 0, 0, T
        else:
            pbase = S - T

        pc = _Pacer(att, zero_ref[0])
        scale = DH ** -0.5

        def logits_pieces(qs, ks, ps, c, first):
            r0 = c * R
            st = {}

            def piece(w):
                if w == 0:
                    st['q'] = att[qs, :, HALO + r0:HALO + r0 + R, :]
                    st['lg'] = []
                kw = att[ks, :, pl.ds(HALO + r0 - DIL * w, R), :]
                p = jnp.sum(st['q'] * kw, axis=0)
                p = p + pltpu.roll(p, 64, 1)
                p = p + pltpu.roll(p, 32, 1)
                if first and r0 < DIL * w:
                    row = lax.broadcasted_iota(i32, (R, 128), 0) + blk * T
                    p = jnp.where(row + r0 >= DIL * w, p, -1e9 / scale)
                st['lg'].append(p)

            def softmax():
                lg = st['lg']
                m = functools.reduce(jnp.maximum, lg)
                e = [jnp.exp2((p - m) * (scale * 1.4426950408889634)) for p in lg]
                inv = pl.reciprocal(functools.reduce(jnp.add, e), approx=True)
                for w in range(W):
                    att[ps, w, r0:r0 + R, :] = e[w] * inv
            return [functools.partial(piece, w) for w in range(W)], softmax

        def av_pieces(ps, vs, o_s, c):
            r0 = c * 16
            st = {}

            def piece(j):
                if j == 0:
                    st['a'] = att[ps, :, r0:r0 + 16, :]
                a = st['a']
                acc = a[0] * att[vs, j, pl.ds(HALO + r0, 16), :]
                for w in range(1, W):
                    acc = acc + a[w] * att[vs, j, pl.ds(HALO + r0 - DIL * w, 16), :]
                o = pltpu.bitcast(acc.astype(bf16), i32)
                o_s[r0 // 2:r0 // 2 + 8, j * 128:(j + 1) * 128] = o
                pc.later(AVLAG, lambda: pc.pin(o))
            return [functools.partial(piece, j) for j in range(NG)]

        def ln1_piece(row0, dst, c):
            rel = kind == 'mid' and dst is xn_n
            xn = _ln_packed(xs[pl.ds(row0 + c * 16, 16), :], att[DUMMY, 1, 0:8, :] if rel else None)
            dst[8 * c:8 * c + 8, :] = xn
            if rel:
                pc.later(LNLAG, lambda: pc.pin(xn))
            else:
                pc.pin(xn)

        if kind != 'last':
            aa = AA if kind == 'mid' else FAA
            for (qs, ks, ps, first, (t0, n)) in ((QA, KA, PA, True, LA), (QB, KB, PB, False, LB)):
                for c in range(NCH):
                    pcs, sm = logits_pieces(qs, ks, ps, c, first)
                    ts, dt = (t0 + c * n / NCH, n / NCH) if kind == 'mid' else FT[(0 if first else NCH) + c]
                    pc.spread(pcs, ts, dt)
                    pc.at(ts + dt + (LAG if kind == 'mid' else FLAG), sm)
            pc.spread([p for c in range(C // 16) for p in av_pieces(PA, VA, o_a, c)], *aa)
            n1b, n1n = (N1B, N1N) if kind == 'mid' else (FN1B, FN1N)
            pc.spread([functools.partial(ln1_piece, base + C, xn_b, c) for c in range(C // 16)], *n1b)
            pc.spread([functools.partial(ln1_piece, nbase, xn_n, c) for c in range(C // 16)], *n1n)
            att[KA, :, 0:HALO, :] = hk[...]
            att[VA, :, 0:HALO, :] = hv[...]
        if kind != 'first':
            pc.spread([p for c in range(C // 16) for p in av_pieces(PB, VB, o_b, c)], *AB)

        def proj(chain, part, half=None):
            slot = (QB if chain else QA) + part
            src = xn_b if chain else xn_a
            if half is None:
                xn, w_ref = _as_bf16(src[...]), wqkv_p.at[part]
            else:
                xn = _as_bf16(src[:, half * (D // 2):(half + 1) * (D // 2)])
                w_ref = wqkv_p.at[part, half * (D // 4):(half + 1) * (D // 4)]
            for j in range(NG):
                r = _dot(xn, w_ref, j)
                if half == 1:
                    r = r + att[slot, j, HALO:HALO + C, :]
                if part > 0 and half != 0:
                    if chain == 0:
                        att[QB + part, j, 0:HALO, :] = r[C - HALO:C]
                    else:
                        (hk if part == 1 else hv)[j] = r[C - HALO:C]
                pc.tile(r, slot, j, dur=1 if half is None else 0.5)

        def out_proj(chain):
            r0 = pbase + chain * C
            o = _as_bf16((o_b if chain else o_a)[...])
            for n in range(NG):
                if n % 2 == 0:
                    xr = xs[pl.ds(r0, C), n * 128:(n + 2) * 128]
                r = _dot(o, wo_p, n) + xr[:, (n % 2) * 128:(n % 2 + 1) * 128].astype(f32)
                pc.tile(r)
                xs[pl.ds(r0, C), n * 128:(n + 1) * 128] = r.astype(bf16)

        if kind == 'mid':
            proj(0, 0), proj(0, 1), out_proj(0), proj(1, 0), proj(1, 1), proj(0, 2), out_proj(1)
            xn_a[...] = xn_n[...]
            proj(1, 2)
        elif kind == 'first':
            proj(0, 0)
            kv_cps[0][0].wait()
            permute_xlu(1, 0, D // 2)
            proj(1, 0)
            kv_cps[0][1].wait()
            permute_xlu(1, D // 2, D // 2)
            proj(0, 1, 0), proj(1, 1, 0)
            kv_cps[1][0].wait()
            permute_xlu(2, 0, D // 2)
            proj(0, 1, 1), proj(1, 1, 1)
            kv_cps[1][1].wait()
            permute(2, 2 * rows, pc), permute(2, 3 * rows, pc)
            proj(0, 2, 0), proj(1, 2, 0)
            wo_cp.wait()
            pc.aux = wo_stage
            pc.spread([functools.partial(wo_stage_piece, j, g, g + 2)
                       for j in range(NG) for g in range(0, NG, 2)], *WOS)
            pc.spread([functools.partial(wo_gather_piece, jp, th, ah)
                       for jp in range(NG) for th in range(2) for ah in range(2)], *WOG)
            proj(0, 2, 1)
            xn_a[...] = xn_n[...]
            proj(1, 2, 1)
        else:
            out_proj(0), out_proj(1)
        assert not pc.events

    def _mlp_item():
        item = step - SKEW
        blk = item & (NB - 1)
        base = pl.multiple_of(blk * T, T)
        nbase = pl.multiple_of(((item + 1) & (NB - 1)) * T, T)

        pc = _Pacer(att, zero_ref[0])

        def ln_piece(row0, dst, c):
            xn = _ln_packed(xs[pl.ds(row0 + c * 16, 16), :])
            dst[8 * c:8 * c + 8, :] = xn
            pc.pin(xn, hard=True)

        pc.spread([functools.partial(ln_piece, base + C, xn2_b, c) for c in range(C // 16)], *N2B)
        pc.spread([functools.partial(ln_piece, nbase, xn2_a, c) for c in range(C // 16)], *N2A)

        def mish(h):
            ex = jnp.exp(jnp.minimum(h, 30.0))
            n = ex * (ex + 2.0)
            return (h * n * pl.reciprocal(n + 2.0, approx=True)).astype(bf16)

        def mlp1(xn):
            act = []
            for n in range(NF):
                r = _dot(pc.tie(xn), w1_v, n)
                pc.tile(r)
                act.append(mish(r + b1_v[n:n + 1, :].astype(f32)))
            return jnp.concatenate(act, axis=1)

        act_a = mlp1(_as_bf16(xn2_a[...]))
        act_b = mlp1(_as_bf16(xn2_b[...]))
        for act, r0 in ((act_a, base), (act_b, base + C)):
            for n in range(NG):
                if n % 2 == 0:
                    xr = xs[pl.ds(r0, C), n * 128:(n + 2) * 128]
                r = _dot(pc.tie(act), w2_v, n) + xr[:, (n % 2) * 128:(n % 2 + 1) * 128].astype(f32)
                pc.tile(r)
                xs[pl.ds(r0, C), n * 128:(n + 1) * 128] = r.astype(bf16)
                cuts = OUT_CUTS if r0 is not base else (NG,)
                if n + 1 in cuts:
                    n0 = ([0] + [c for c in cuts if c <= n])[-1]

                    @pl.when(item >= NITEM - NB)
                    def _():
                        out_copy(r0, n0 * 128, (n + 1 - n0) * 128).start()
        assert not pc.events

        @pl.when(item == NITEM - 1)
        def _():
            pltpu.make_async_copy(xs, out_hbm, sems.at[SEM_O]).wait()

    @pl.when((step <= SKEW + 1) | (step == NITEM + 1))
    def _():
        pl.when(step == 0)(prologue)
        pl.when(step == SKEW)(first_mlp_prep)
        for k in range(1, SKEW + 1):
            pl.when(step == k)(x_copy(k + 1).wait)

        @pl.when(step == SKEW + 1)
        def _():
            for k in range(SKEW + 2, NB + 1):
                x_copy(k).wait()

        pl.when(step == NITEM + 1)(functools.partial(attention, 'last'))

    pl.when(step >= SKEW)(_mlp_item)
    pl.when((step >= 1) & (step < NITEM))(functools.partial(attention, 'mid'))


@jax.jit
def pallas_interleave_layers__sliding_local_dilated__dense_activation_mish__prompt_kernel(A_x, A_wqkv, A_wo, B_x, B_w1, B_b1, B_w2):
    x = A_x.reshape(S, D)
    b1 = B_b1.reshape(NF, 128)
    out = pl.pallas_call(
        _kernel,
        grid=(NITEM + SKEW,),
        in_specs=[pl.BlockSpec(memory_space=pl.ANY)] * 6,
        out_specs=pl.BlockSpec(memory_space=pl.ANY),
        out_shape=jax.ShapeDtypeStruct((S, D), bf16),
        scratch_shapes=[
            pltpu.VMEM((3, D, D), bf16), pltpu.VMEM((3, D // 2, D), i32),
            pltpu.VMEM((D, D), bf16), pltpu.VMEM((NG, NG * PITCH + 8, 128), i32), pltpu.VMEM((NG, 128, 128), bf16),
            pltpu.VMEM((D // 2, D), i32),
            pltpu.VMEM((D, F), bf16), pltpu.VMEM((F, D), bf16), pltpu.VMEM((NF, 128), bf16),
            pltpu.VMEM((S, D), bf16), pltpu.VMEM((3, C // 2, D), i32),
            pltpu.VMEM((C // 2, D), i32), pltpu.VMEM((C // 2, D), i32),
            pltpu.VMEM((NSLOT, NG, AROWS, 128), f32),
            pltpu.VMEM((C // 2, D), i32), pltpu.VMEM((C // 2, D), i32),
            pltpu.VMEM((NG, HALO, 128), f32), pltpu.VMEM((NG, HALO, 128), f32),
            pltpu.SMEM((1,), i32),
            pltpu.SemaphoreType.DMA((NSEM,)),
        ],
        compiler_params=pltpu.CompilerParams(
            dimension_semantics=("arbitrary",), vmem_limit_bytes=100 * 1024 * 1024, disable_semaphore_checks=True),
        name="fused",
    )(x, b1, A_wqkv, A_wo, B_w1, B_w2)
    return out.reshape(1, S, D)
```

```python
import functools
import jax
import jax.numpy as jnp
from jax import lax
import jax.experimental.pallas as pl
import jax.experimental.pallas.tpu as pltpu

S, D, F = 2048, 1024, 3584
H, DH, W, DIL = 32, 32, 8, 2
NG = D // 128
NF = F // 128
HALO = 16
T = 256
C = T // 2
R = 8
NCH = C // R
NB = S // T
NITEM = 2 * NB
SKEW = 3
EPS = 1e-5
f32, bf16, i32 = jnp.float32, jnp.bfloat16, jnp.int32
QA, KA, VA, QB, KB, VB, PA, PB, DUMMY, PIN = range(10)
NSLOT = PIN + 1
LA, AA, LB, AB = (15, 16), (55.3, 7.2), (39, 16), (0.3, 7.5)
N1B, N1N, N2A, N2B = (8, 7), (32, 5), (57, 8), (2, 22)
FAA = (48.3, 3.5)
FN1B, FN1N = (0, 3.5), (3.5, 3)
LAG = 1.5
AVLAG = 0.2
OUT_CUTS = (4, 6, 7, 8)
LNLAG = 1.0
WOS, WOG = (44, 4), (48, 3.8)
FT = [(t0 + i * dt, dt) for t0, dt, n in ((28, 0.5, 6), (32, 0.56, 20), (44, 0.6, 6)) for i in range(n)]
FLAG = 1.4
AROWS = C + HALO + 8
RAWPAD = 128
NWCH = 4
SEM_X, SEM_W, SEM_O, SEM_Q, NSEM = 0, NB + 1, NB + 5, NB + 6, NB + 10 + NWCH
PITCH = 65


def _layernorm(x):
    m = jnp.mean(x, axis=-1, keepdims=True)
    xc = x - m
    v = jnp.mean(xc * xc, axis=-1, keepdims=True)
    return xc * lax.rsqrt(v + EPS)


def _ln_packed(x, zeros=None):
    x = x.astype(f32)
    if zeros is not None:
        x = jnp.concatenate([x[:, 0:128] + jnp.concatenate([zeros, zeros], axis=0), x[:, 128:]], axis=1)
    return pltpu.bitcast(_layernorm(x).astype(bf16), i32)


def _perm_matrix(j):
    src = lax.broadcasted_iota(i32, (128, 128), 0)
    m = lax.broadcasted_iota(i32, (128, 128), 1)
    jp = (j + 128 - m) & 7
    l = (m + jp) & 127
    want = 32 * ((l >> 3) & 3) + 4 * jp + (l >> 5)
    return jnp.where(src == want, 1.0, 0.0).astype(bf16)


def _perm_pattern(j, r):
    m = lax.broadcasted_iota(i32, (r, 128), 1)
    jp = (j + 128 - m) & 7
    l = (m + jp) & 127
    return 32 * ((l >> 3) & 3) + 4 * jp + (l >> 5)


def _exchange_and_roll(mid):
    lane = lax.broadcasted_iota(i32, mid[0].shape, 1)
    for b in (1, 2, 4):
        m = (lane & b) != 0
        mid = [jnp.where(m, mid[(j + b) % 8], mid[j]) for j in range(8)]
    return [g if j == 0 else pltpu.roll(g, j, 1) for j, g in enumerate(mid)]


def _as_bf16(v):
    return v if v.dtype == bf16 else pltpu.bitcast(v, bf16)


def _dot(x, w_ref, n):
    return jnp.dot(x, _as_bf16(w_ref[:, n * 128:(n + 1) * 128]), preferred_element_type=f32)


class _Pacer:
    def __init__(self, att, z):
        self.att, self.z, self.events, self.t, self.now = att, z, [], 0, 0

    def at(self, t, piece):
        self.events.append((t, len(self.events), piece))
        self.events.sort(key=lambda e: e[:2])

    def spread(self, pieces, t0, dur):
        for i, p in enumerate(pieces):
            self.at(t0 + dur * (i + 0.5) / len(pieces), p)

    def later(self, dt, piece):
        self.at(self.now + dt, piece)

    def tie(self, lhs):
        if not self.tied:
            return lhs
        dep = functools.reduce(jnp.bitwise_or, self.tied) & self.z
        self.tied = []
        a00 = pltpu.bitcast(pltpu.bitcast(lhs[0:16, 0:128], i32) | dep, bf16)
        return jnp.concatenate([jnp.concatenate([a00, lhs[0:16, 128:]], axis=1), lhs[16:]], axis=0)

    def pin(self, words, hard=False):
        v = functools.reduce(jnp.bitwise_or, [words[:, j * 128:(j + 1) * 128] for j in range(words.shape[1] // 128)])
        if hard:
            self.tied = self.tied + [v]
            return
        k, self.npin = self.npin, self.npin + 1
        per = (C + HALO) // 8
        self.att[PIN + k // (NG * per), (k // per) % NG, 8 * (k % per):8 * (k % per) + 8, :] = pltpu.bitcast(v, f32)

    def tile(self, r, slot=None, j=None, dur=1):
        nst = C // 8
        for i in range(nst):
            lim = self.t + dur * (i + 1) / nst
            fence = self.events and self.events[0][0] < lim
            if slot is not None:
                self.att[slot + self.z if fence else slot, j, HALO + 8 * i:HALO + 8 * i + 8, :] = r[8 * i:8 * i + 8]
            elif fence:
                self.att[DUMMY + self.z, 0, 0:8, :] = r[8 * i:8 * i + 8]
            if fence and self.aux is not None:
                n = self.aux.shape[1]
                self.aux[self.z, n - 8:n, :] = pltpu.bitcast(r[8 * i:8 * i + 8], i32)
            self.now = lim
            while self.events and self.events[0][0] < lim:
                self.events.pop(0)[2]()
        self.t += dur

    npin = 0
    aux = None
    tied = []


def _kernel(x_hbm, b1_hbm, wqkv_hbm, wo_hbm, w1_hbm, w2_hbm, out_hbm,
            wqkv_raw, wqkv_p, wo_raw, wo_stage, pm, wo_p, w1_v, w2_v, b1_v,
            xs, xn1, xn2_a, xn2_b, att, o_a, o_b, hk, hv, zero_ref, sems):
    step = pl.program_id(0)
    xn_a, xn_b, xn_n = xn1.at[0], xn1.at[1], xn1.at[2]

    def x_copy(k):
        r0, r1 = max(k * T - C, 0), min(k * T + C, S)
        return pltpu.make_async_copy(x_hbm.at[pl.ds(r0, r1 - r0)], xs.at[pl.ds(r0, r1 - r0)], sems.at[SEM_X + k])

    def out_copy(r0, c0, nc):
        return pltpu.make_async_copy(xs.at[pl.ds(r0, C), pl.ds(c0, nc)], out_hbm.at[pl.ds(r0, C), pl.ds(c0, nc)],
                                     sems.at[SEM_O])

    rows = D // NWCH

    def q_copy(p, r0, n, k):
        return pltpu.make_async_copy(wqkv_hbm.at[pl.ds(r0, n), pl.ds(p * D, D)],
                                     wqkv_raw.at[p, pl.ds(r0, n), pl.ds(0, D)], sems.at[SEM_Q + k])

    kv_cps = [[q_copy(p, h * (D // 2), D // 2, NWCH + 2 * (p - 1) + h) for h in range(2)] for p in (1, 2)]
    wo_cp = pltpu.make_async_copy(wo_hbm, wo_raw.at[:, pl.ds(0, D)], sems.at[SEM_W + 0])
    w1_cp = pltpu.make_async_copy(w1_hbm, w1_v, sems.at[SEM_W + 1])
    w2_cp = pltpu.make_async_copy(w2_hbm, w2_v, sems.at[SEM_W + 2])
    b1_cp = pltpu.make_async_copy(b1_hbm, b1_v, sems.at[SEM_W + 3])

    def permute(p, r0, pc=None):
        r1 = r0 // 2 if isinstance(r0, int) else pl.multiple_of(r0 >> 1, rows // 2)
        mid = []
        for j in range(NG):
            r = jnp.dot(wqkv_raw[p, pl.ds(r0, rows), j * 128:(j + 1) * 128], pm[j], preferred_element_type=f32)
            if pc is not None and j % 4 == 3:
                pc.tile(r[rows - C:rows])
            mid.append(pltpu.bitcast(r.astype(bf16), i32))
        outs = _exchange_and_roll(mid)
        for j in range(NG):
            wqkv_p[p, pl.ds(r1, rows // 2), j * 128:(j + 1) * 128] = outs[j]

    def permute_xlu(p, r0, n):
        w0, w1 = r0 // 2, (r0 + n) // 2
        for j in range(NG):
            words = pltpu.bitcast(wqkv_raw[p, r0:r0 + n, j * 128:(j + 1) * 128], i32)
            wqkv_p[p, w0:w1, j * 128:(j + 1) * 128] = jnp.take_along_axis(
                words, _perm_pattern(j, n // 2), axis=1, mode="promise_in_bounds")
        for w in range(w0, w1, 8):
            outs = _exchange_and_roll([wqkv_p[p, w:w + 8, j * 128:(j + 1) * 128] for j in range(NG)])
            for j in range(NG):
                wqkv_p[p, w:w + 8, j * 128:(j + 1) * 128] = outs[j]

    def prologue():
        x_copy(0).start()
        for k in range(NWCH):
            q_copy(0, k * rows, rows, k).start()
        x_copy(1).start()
        for cp in kv_cps[0] + kv_cps[1]:
            cp.start()
        wo_cp.start()
        for k in range(2, SKEW + 1):
            x_copy(k).start()
        b1_cp.start()
        w1_cp.start()
        w2_cp.start()
        for k in range(SKEW + 1, NB + 1):
            x_copy(k).start()
        zero_ref[0] = 0
        hk[...] = jnp.zeros(hk.shape, f32)
        att[DUMMY, 1, 0:8, :] = jnp.zeros((8, 128), f32)
        hv[...] = jnp.zeros(hv.shape, f32)
        for j in range(NG):
            pm[j] = _perm_matrix(j)
        x_copy(0).wait()
        xn_a[...] = _ln_packed(xs[0:C, :])

        def body(k, c):
            r0 = pl.multiple_of(k * rows, rows)
            q_copy(0, r0, rows, k).wait()
            permute(0, r0)
            return c
        lax.fori_loop(0, NWCH, body, 0)
        x_copy(1).wait()

        attention('first')

    def wo_stage_piece(j, g0, g1):
        words = pltpu.bitcast(wo_raw[j * 128:(j + 1) * 128, g0 * 128:g1 * 128], i32)
        for g in range(g0, g1):
            for a in range(4):
                r0 = PITCH * (j // 2 + 4 * (a % 2)) + 32 * (j % 2) + 16 * (a // 2)
                wo_stage[g, r0:r0 + 16, :] = words[16 * a:16 * a + 16, (g - g0) * 128:(g - g0 + 1) * 128]

    def wo_gather_piece(jp, th, ah):
        for g in range(NG):
            ev = wo_stage[g, pl.ds(16 * ah + 2 * jp + th, 8, stride=PITCH), :]
            od = wo_stage[g, pl.ds(32 + 16 * ah + 2 * jp + th, 8, stride=PITCH), :]
            lo = (ev & 0xFFFF) | lax.shift_left(od, 16)
            hi = lax.shift_right_logical(ev, 16) | (od & -0x10000)
            for t, v in ((2 * th, lo), (2 * th + 1, hi)):
                w0 = jp * 64 + 16 * t + 8 * ah
                wo_p[w0:w0 + 8, g * 128:(g + 1) * 128] = v

    def first_mlp_prep():
        xn2_a[...] = _ln_packed(xs[0:C, :])
        b1_cp.wait()
        w1_cp.wait()
        w2_cp.wait()

    def attention(kind):
        if kind == 'mid':
            blk = step & (NB - 1)
            base = pl.multiple_of(blk * T, T)
            nbase = pl.multiple_of(((step + 1) & (NB - 1)) * T, T)
            pbase = pl.multiple_of(((step - 1) & (NB - 1)) * T, T)
        elif kind == 'first':
            blk, base, nbase = 0, 0, T
        else:
            pbase = S - T

        pc = _Pacer(att, zero_ref[0])
        scale = DH ** -0.5

        def logits_pieces(qs, ks, ps, c, first):
            r0 = c * R
            st = {}

            def piece(w):
                if w == 0:
                    st['q'] = att[qs, :, HALO + r0:HALO + r0 + R, :]
                    st['lg'] = []
                kw = att[ks, :, pl.ds(HALO + r0 - DIL * w, R), :]
                p = jnp.sum(st['q'] * kw, axis=0)
                p = p + pltpu.roll(p, 64, 1)
                p = p + pltpu.roll(p, 32, 1)
                if first and r0 < DIL * w:
                    row = lax.broadcasted_iota(i32, (R, 128), 0) + blk * T
                    p = jnp.where(row + r0 >= DIL * w, p, -1e9 / scale)
                st['lg'].append(p)

            def softmax():
                lg = st['lg']
                m = functools.reduce(jnp.maximum, lg)
                e = [jnp.exp2((p - m) * (scale * 1.4426950408889634)) for p in lg]
                inv = pl.reciprocal(functools.reduce(jnp.add, e), approx=True)
                for w in range(W):
                    att[ps, w, r0:r0 + R, :] = e[w] * inv
            return [functools.partial(piece, w) for w in range(W)], softmax

        def av_pieces(ps, vs, o_s, c):
            r0 = c * 16
            st = {}

            def piece(j):
                if j == 0:
                    st['a'] = att[ps, :, r0:r0 + 16, :]
                a = st['a']
                acc = a[0] * att[vs, j, pl.ds(HALO + r0, 16), :]
                for w in range(1, W):
                    acc = acc + a[w] * att[vs, j, pl.ds(HALO + r0 - DIL * w, 16), :]
                o = pltpu.bitcast(acc.astype(bf16), i32)
                o_s[r0 // 2:r0 // 2 + 8, j * 128:(j + 1) * 128] = o
                pc.later(AVLAG, lambda: pc.pin(o))
            return [functools.partial(piece, j) for j in range(NG)]

        def ln1_piece(row0, dst, c):
            rel = kind == 'mid' and dst is xn_n
            xn = _ln_packed(xs[pl.ds(row0 + c * 16, 16), :], att[DUMMY, 1, 0:8, :] if rel else None)
            dst[8 * c:8 * c + 8, :] = xn
            if rel:
                pc.later(LNLAG, lambda: pc.pin(xn))
            else:
                pc.pin(xn)

        if kind != 'last':
            aa = AA if kind == 'mid' else FAA
            for (qs, ks, ps, first, (t0, n)) in ((QA, KA, PA, True, LA), (QB, KB, PB, False, LB)):
                for c in range(NCH):
                    pcs, sm = logits_pieces(qs, ks, ps, c, first)
                    ts, dt = (t0 + c * n / NCH, n / NCH) if kind == 'mid' else FT[(0 if first else NCH) + c]
                    pc.spread(pcs, ts, dt)
                    pc.at(ts + dt + (LAG if kind == 'mid' else FLAG), sm)
            pc.spread([p for c in range(C // 16) for p in av_pieces(PA, VA, o_a, c)], *aa)
            n1b, n1n = (N1B, N1N) if kind == 'mid' else (FN1B, FN1N)
            pc.spread([functools.partial(ln1_piece, base + C, xn_b, c) for c in range(C // 16)], *n1b)
            pc.spread([functools.partial(ln1_piece, nbase, xn_n, c) for c in range(C // 16)], *n1n)
            att[KA, :, 0:HALO, :] = hk[...]
            att[VA, :, 0:HALO, :] = hv[...]
        if kind != 'first':
            pc.spread([p for c in range(C // 16) for p in av_pieces(PB, VB, o_b, c)], *AB)

        def proj(chain, part, half=None):
            slot = (QB if chain else QA) + part
            src = xn_b if chain else xn_a
            if half is None:
                xn, w_ref = _as_bf16(src[...]), wqkv_p.at[part]
            else:
                xn = _as_bf16(src[:, half * (D // 2):(half + 1) * (D // 2)])
                w_ref = wqkv_p.at[part, half * (D // 4):(half + 1) * (D // 4)]
            for j in range(NG):
                r = _dot(xn, w_ref, j)
                if half == 1:
                    r = r + att[slot, j, HALO:HALO + C, :]
                if part > 0 and half != 0:
                    if chain == 0:
                        att[QB + part, j, 0:HALO, :] = r[C - HALO:C]
                    else:
                        (hk if part == 1 else hv)[j] = r[C - HALO:C]
                pc.tile(r, slot, j, dur=1 if half is None else 0.5)

        def out_proj(chain):
            r0 = pbase + chain * C
            o = _as_bf16((o_b if chain else o_a)[...])
            for n in range(NG):
                if n % 2 == 0:
                    xr = xs[pl.ds(r0, C), n * 128:(n + 2) * 128]
                r = _dot(o, wo_p, n) + xr[:, (n % 2) * 128:(n % 2 + 1) * 128].astype(f32)
                pc.tile(r)
                xs[pl.ds(r0, C), n * 128:(n + 1) * 128] = r.astype(bf16)

        if kind == 'mid':
            proj(0, 0), proj(0, 1), out_proj(0), proj(1, 0), proj(1, 1), proj(0, 2), out_proj(1)
            xn_a[...] = xn_n[...]
            proj(1, 2)
        elif kind == 'first':
            proj(0, 0)
            kv_cps[0][0].wait()
            permute_xlu(1, 0, D // 2)
            proj(1, 0)
            kv_cps[0][1].wait()
            permute_xlu(1, D // 2, D // 2)
            proj(0, 1, 0), proj(1, 1, 0)
            kv_cps[1][0].wait()
            permute_xlu(2, 0, D // 2)
            proj(0, 1, 1), proj(1, 1, 1)
            kv_cps[1][1].wait()
            permute(2, 2 * rows, pc), permute(2, 3 * rows, pc)
            proj(0, 2, 0), proj(1, 2, 0)
            wo_cp.wait()
            pc.aux = wo_stage
            pc.spread([functools.partial(wo_stage_piece, j, g, g + 2)
                       for j in range(NG) for g in range(0, NG, 2)], *WOS)
            pc.spread([functools.partial(wo_gather_piece, jp, th, ah)
                       for jp in range(NG) for th in range(2) for ah in range(2)], *WOG)
            proj(0, 2, 1)
            xn_a[...] = xn_n[...]
            proj(1, 2, 1)
        else:
            out_proj(0), out_proj(1)
        assert not pc.events

    def _mlp_item():
        item = step - SKEW
        blk = item & (NB - 1)
        base = pl.multiple_of(blk * T, T)
        nbase = pl.multiple_of(((item + 1) & (NB - 1)) * T, T)

        pc = _Pacer(att, zero_ref[0])

        def ln_piece(row0, dst, c):
            xn = _ln_packed(xs[pl.ds(row0 + c * 16, 16), :])
            dst[8 * c:8 * c + 8, :] = xn
            pc.pin(xn, hard=True)

        pc.spread([functools.partial(ln_piece, base + C, xn2_b, c) for c in range(C // 16)], *N2B)
        pc.spread([functools.partial(ln_piece, nbase, xn2_a, c) for c in range(C // 16)], *N2A)

        def mish(h):
            ex = jnp.exp(jnp.minimum(h, 30.0))
            n = ex * (ex + 2.0)
            return (h * n * pl.reciprocal(n + 2.0, approx=True)).astype(bf16)

        def mlp1(xn):
            act = []
            for n in range(NF):
                r = _dot(pc.tie(xn), w1_v, n)
                pc.tile(r)
                act.append(mish(r + b1_v[n:n + 1, :].astype(f32)))
            return jnp.concatenate(act, axis=1)

        act_a = mlp1(_as_bf16(xn2_a[...]))
        act_b = mlp1(_as_bf16(xn2_b[...]))
        for act, r0 in ((act_a, base), (act_b, base + C)):
            for n in range(NG):
                if n % 2 == 0:
                    xr = xs[pl.ds(r0, C), n * 128:(n + 2) * 128]
                r = _dot(pc.tie(act), w2_v, n) + xr[:, (n % 2) * 128:(n % 2 + 1) * 128].astype(f32)
                pc.tile(r)
                xs[pl.ds(r0, C), n * 128:(n + 1) * 128] = r.astype(bf16)
                cuts = OUT_CUTS if r0 is not base else (NG,)
                if n + 1 in cuts:
                    n0 = ([0] + [c for c in cuts if c <= n])[-1]

                    @pl.when(item >= NITEM - NB)
                    def _():
                        out_copy(r0, n0 * 128, (n + 1 - n0) * 128).start()
        assert not pc.events

        @pl.when(item == NITEM - 1)
        def _():
            pltpu.make_async_copy(xs, out_hbm, sems.at[SEM_O]).wait()

    @pl.when((step <= SKEW + 1) | (step == NITEM + 1))
    def _():
        pl.when(step == 0)(prologue)
        pl.when(step == SKEW)(first_mlp_prep)
        for k in range(1, SKEW + 1):
            pl.when(step == k)(x_copy(k + 1).wait)

        @pl.when(step == SKEW + 1)
        def _():
            for k in range(SKEW + 2, NB + 1):
                x_copy(k).wait()

        pl.when(step == NITEM + 1)(functools.partial(attention, 'last'))

    pl.when(step >= SKEW)(_mlp_item)
    pl.when((step >= 1) & (step < NITEM))(functools.partial(attention, 'mid'))


@jax.jit
def pallas_interleave_layers__sliding_local_dilated__dense_activation_mish__prompt_kernel(A_x, A_wqkv, A_wo, B_x, B_w1, B_b1, B_w2):
    x = A_x.reshape(S, D)
    b1 = B_b1.reshape(NF, 128)
    out = pl.pallas_call(
        _kernel,
        grid=(NITEM + SKEW,),
        in_specs=[pl.BlockSpec(memory_space=pl.ANY)] * 6,
        out_specs=pl.BlockSpec(memory_space=pl.ANY),
        out_shape=jax.ShapeDtypeStruct((S, D), bf16),
        scratch_shapes=[
            pltpu.VMEM((3, D, D + RAWPAD), bf16), pltpu.VMEM((3, D // 2, D), i32),
            pltpu.VMEM((D, D + RAWPAD), bf16), pltpu.VMEM((NG, NG * PITCH + 72, 128), i32), pltpu.VMEM((NG, 128, 128), bf16),
            pltpu.VMEM((D // 2, D), i32),
            pltpu.VMEM((D, F), bf16), pltpu.VMEM((F, D), bf16), pltpu.VMEM((NF, 128), bf16),
            pltpu.VMEM((S, D), bf16), pltpu.VMEM((3, C // 2, D), i32),
            pltpu.VMEM((C // 2, D), i32), pltpu.VMEM((C // 2, D), i32),
            pltpu.VMEM((NSLOT, NG, AROWS, 128), f32),
            pltpu.VMEM((C // 2, D), i32), pltpu.VMEM((C // 2, D), i32),
            pltpu.VMEM((NG, HALO, 128), f32), pltpu.VMEM((NG, HALO, 128), f32),
            pltpu.SMEM((1,), i32),
            pltpu.SemaphoreType.DMA((NSEM,)),
        ],
        compiler_params=pltpu.CompilerParams(
            dimension_semantics=("arbitrary",), vmem_limit_bytes=100 * 1024 * 1024, disable_semaphore_checks=True),
        name="fused",
    )(x, b1, A_wqkv, A_wo, B_w1, B_w2)
    return out.reshape(1, S, D)
```

```python
import functools
import jax
import jax.numpy as jnp
from jax import lax
import jax.experimental.pallas as pl
import jax.experimental.pallas.tpu as pltpu

S, D, F = 2048, 1024, 3584
H, DH, W, DIL = 32, 32, 8, 2
NG = D // 128
NF = F // 128
HALO = 16
T = 256
C = T // 2
R = 8
NCH = C // R
NB = S // T
NITEM = 2 * NB
SKEW = 3
EPS = 1e-5
f32, bf16, i32 = jnp.float32, jnp.bfloat16, jnp.int32
QA, KA, VA, QB, KB, VB, PA, PB, DUMMY, PIN = range(10)
NSLOT = PIN + 1
LA, AA, LB, AB = (16, 15), (55.3, 7.2), (39, 16), (0.3, 7.5)
N1B, N1N, N2A, N2B = (8, 4), (12, 4), (57, 8), (2, 22)
FAA = (48.3, 3.5)
FN1B, FN1N = (0, 3.5), (3.5, 3)
LAG = 1.5
AVLAG = 0.2
OUT_CUTS = (4, 6, 7, 8)
WOS, WOG = (44, 4), (48, 3.8)
FT = [(t0 + i * dt, dt) for t0, dt, n in ((28, 0.5, 6), (32, 0.56, 20), (44, 0.6, 6)) for i in range(n)]
FLAG = 1.4
AROWS = C + HALO + 8
RAWPAD = 128
NWCH = 4
SEM_X, SEM_W, SEM_O, SEM_Q, NSEM = 0, NB + 1, NB + 5, NB + 6, NB + 10 + NWCH
PITCH = 65


def _layernorm(x):
    m = jnp.mean(x, axis=-1, keepdims=True)
    xc = x - m
    v = jnp.mean(xc * xc, axis=-1, keepdims=True)
    return xc * lax.rsqrt(v + EPS)


def _ln_packed(x):
    return pltpu.bitcast(_layernorm(x.astype(f32)).astype(bf16), i32)


def _perm_matrix(j):
    src = lax.broadcasted_iota(i32, (128, 128), 0)
    m = lax.broadcasted_iota(i32, (128, 128), 1)
    jp = (j + 128 - m) & 7
    l = (m + jp) & 127
    want = 32 * ((l >> 3) & 3) + 4 * jp + (l >> 5)
    return jnp.where(src == want, 1.0, 0.0).astype(bf16)


def _perm_pattern(j, r):
    m = lax.broadcasted_iota(i32, (r, 128), 1)
    jp = (j + 128 - m) & 7
    l = (m + jp) & 127
    return 32 * ((l >> 3) & 3) + 4 * jp + (l >> 5)


def _exchange_and_roll(mid):
    lane = lax.broadcasted_iota(i32, mid[0].shape, 1)
    for b in (1, 2, 4):
        m = (lane & b) != 0
        mid = [jnp.where(m, mid[(j + b) % 8], mid[j]) for j in range(8)]
    return [g if j == 0 else pltpu.roll(g, j, 1) for j, g in enumerate(mid)]


def _as_bf16(v):
    return v if v.dtype == bf16 else pltpu.bitcast(v, bf16)


def _dot(x, w_ref, n):
    return jnp.dot(x, _as_bf16(w_ref[:, n * 128:(n + 1) * 128]), preferred_element_type=f32)


class _Pacer:
    def __init__(self, att, z):
        self.att, self.z, self.events, self.t, self.now = att, z, [], 0, 0

    def at(self, t, piece):
        self.events.append((t, len(self.events), piece))
        self.events.sort(key=lambda e: e[:2])

    def spread(self, pieces, t0, dur):
        for i, p in enumerate(pieces):
            self.at(t0 + dur * (i + 0.5) / len(pieces), p)

    def later(self, dt, piece):
        self.at(self.now + dt, piece)

    def tie(self, lhs):
        if not self.tied:
            return lhs
        dep = functools.reduce(jnp.bitwise_or, self.tied) & self.z
        self.tied = []
        a00 = pltpu.bitcast(pltpu.bitcast(lhs[0:16, 0:128], i32) | dep, bf16)
        return jnp.concatenate([jnp.concatenate([a00, lhs[0:16, 128:]], axis=1), lhs[16:]], axis=0)

    def pin(self, words, hard=False):
        v = functools.reduce(jnp.bitwise_or, [words[:, j * 128:(j + 1) * 128] for j in range(words.shape[1] // 128)])
        if hard:
            self.tied = self.tied + [v]
            return
        k, self.npin = self.npin, self.npin + 1
        per = (C + HALO) // 8
        self.att[PIN + k // (NG * per), (k // per) % NG, 8 * (k % per):8 * (k % per) + 8, :] = pltpu.bitcast(v, f32)

    def tile(self, r, slot=None, j=None, dur=1):
        nst = C // 8
        for i in range(nst):
            lim = self.t + dur * (i + 1) / nst
            fence = self.events and self.events[0][0] < lim
            if slot is not None:
                self.att[slot + self.z if fence else slot, j, HALO + 8 * i:HALO + 8 * i + 8, :] = r[8 * i:8 * i + 8]
            elif fence:
                self.att[DUMMY + self.z, 0, 0:8, :] = r[8 * i:8 * i + 8]
            if fence and self.aux is not None:
                n = self.aux.shape[1]
                self.aux[self.z, n - 8:n, :] = pltpu.bitcast(r[8 * i:8 * i + 8], i32)
            self.now = lim
            while self.events and self.events[0][0] < lim:
                self.events.pop(0)[2]()
        self.t += dur

    npin = 0
    aux = None
    tied = []


def _kernel(x_hbm, b1_hbm, wqkv_hbm, wo_hbm, w1_hbm, w2_hbm, out_hbm,
            wqkv_raw, wqkv_p, wo_raw, wo_stage, pm, wo_p, w1_v, w2_v, b1_v,
            xs, xn1, xn2_a, xn2_b, att, o_a, o_b, hk, hv, zero_ref, sems):
    step = pl.program_id(0)
    xn_a, xn_b, xn_n = xn1.at[0], xn1.at[1], xn1.at[2]

    def x_copy(k):
        r0, r1 = max(k * T - C, 0), min(k * T + C, S)
        return pltpu.make_async_copy(x_hbm.at[pl.ds(r0, r1 - r0)], xs.at[pl.ds(r0, r1 - r0)], sems.at[SEM_X + k])

    def out_copy(r0, c0, nc):
        return pltpu.make_async_copy(xs.at[pl.ds(r0, C), pl.ds(c0, nc)], out_hbm.at[pl.ds(r0, C), pl.ds(c0, nc)],
                                     sems.at[SEM_O])

    rows = D // NWCH

    def q_copy(p, r0, n, k):
        return pltpu.make_async_copy(wqkv_hbm.at[pl.ds(r0, n), pl.ds(p * D, D)],
                                     wqkv_raw.at[p, pl.ds(r0, n), pl.ds(0, D)], sems.at[SEM_Q + k])

    kv_cps = [[q_copy(p, h * (D // 2), D // 2, NWCH + 2 * (p - 1) + h) for h in range(2)] for p in (1, 2)]
    wo_cp = pltpu.make_async_copy(wo_hbm, wo_raw.at[:, pl.ds(0, D)], sems.at[SEM_W + 0])
    w1_cp = pltpu.make_async_copy(w1_hbm, w1_v, sems.at[SEM_W + 1])
    w2_cp = pltpu.make_async_copy(w2_hbm, w2_v, sems.at[SEM_W + 2])
    b1_cp = pltpu.make_async_copy(b1_hbm, b1_v, sems.at[SEM_W + 3])

    def permute(p, r0, pc=None):
        r1 = r0 // 2 if isinstance(r0, int) else pl.multiple_of(r0 >> 1, rows // 2)
        mid = []
        for j in range(NG):
            r = jnp.dot(wqkv_raw[p, pl.ds(r0, rows), j * 128:(j + 1) * 128], pm[j], preferred_element_type=f32)
            if pc is not None and j % 4 == 3:
                pc.tile(r[rows - C:rows])
            mid.append(pltpu.bitcast(r.astype(bf16), i32))
        outs = _exchange_and_roll(mid)
        for j in range(NG):
            wqkv_p[p, pl.ds(r1, rows // 2), j * 128:(j + 1) * 128] = outs[j]

    def permute_xlu(p, r0, n):
        w0, w1 = r0 // 2, (r0 + n) // 2
        for j in range(NG):
            words = pltpu.bitcast(wqkv_raw[p, r0:r0 + n, j * 128:(j + 1) * 128], i32)
            wqkv_p[p, w0:w1, j * 128:(j + 1) * 128] = jnp.take_along_axis(
                words, _perm_pattern(j, n // 2), axis=1, mode="promise_in_bounds")
        for w in range(w0, w1, 8):
            outs = _exchange_and_roll([wqkv_p[p, w:w + 8, j * 128:(j + 1) * 128] for j in range(NG)])
            for j in range(NG):
                wqkv_p[p, w:w + 8, j * 128:(j + 1) * 128] = outs[j]

    def prologue():
        x_copy(0).start()
        for k in range(NWCH):
            q_copy(0, k * rows, rows, k).start()
        x_copy(1).start()
        for cp in kv_cps[0] + kv_cps[1]:
            cp.start()
        wo_cp.start()
        for k in range(2, SKEW + 1):
            x_copy(k).start()
        b1_cp.start()
        w1_cp.start()
        w2_cp.start()
        for k in range(SKEW + 1, NB + 1):
            x_copy(k).start()
        zero_ref[0] = 0
        hk[...] = jnp.zeros(hk.shape, f32)
        hv[...] = jnp.zeros(hv.shape, f32)
        for j in range(NG):
            pm[j] = _perm_matrix(j)
        x_copy(0).wait()
        xn_a[...] = _ln_packed(xs[0:C, :])

        def body(k, c):
            r0 = pl.multiple_of(k * rows, rows)
            q_copy(0, r0, rows, k).wait()
            permute(0, r0)
            return c
        lax.fori_loop(0, NWCH, body, 0)
        x_copy(1).wait()

        attention('first')

    def wo_stage_piece(j, g0, g1):
        words = pltpu.bitcast(wo_raw[j * 128:(j + 1) * 128, g0 * 128:g1 * 128], i32)
        for g in range(g0, g1):
            for a in range(4):
                r0 = PITCH * (j // 2 + 4 * (a % 2)) + 32 * (j % 2) + 16 * (a // 2)
                wo_stage[g, r0:r0 + 16, :] = words[16 * a:16 * a + 16, (g - g0) * 128:(g - g0 + 1) * 128]

    def wo_gather_piece(jp, th, ah):
        for g in range(NG):
            ev = wo_stage[g, pl.ds(16 * ah + 2 * jp + th, 8, stride=PITCH), :]
            od = wo_stage[g, pl.ds(32 + 16 * ah + 2 * jp + th, 8, stride=PITCH), :]
            lo = (ev & 0xFFFF) | lax.shift_left(od, 16)
            hi = lax.shift_right_logical(ev, 16) | (od & -0x10000)
            for t, v in ((2 * th, lo), (2 * th + 1, hi)):
                w0 = jp * 64 + 16 * t + 8 * ah
                wo_p[w0:w0 + 8, g * 128:(g + 1) * 128] = v

    def first_mlp_prep():
        xn2_a[...] = _ln_packed(xs[0:C, :])
        b1_cp.wait()
        w1_cp.wait()
        w2_cp.wait()

    def attention(kind):
        if kind == 'mid':
            blk = step & (NB - 1)
            base = pl.multiple_of(blk * T, T)
            nbase = pl.multiple_of(((step + 1) & (NB - 1)) * T, T)
            pbase = pl.multiple_of(((step - 1) & (NB - 1)) * T, T)
        elif kind == 'first':
            blk, base, nbase = 0, 0, T
        else:
            pbase = S - T

        pc = _Pacer(att, zero_ref[0])
        scale = DH ** -0.5

        def logits_pieces(qs, ks, ps, c, first):
            r0 = c * R
            st = {}

            def piece(w):
                if w == 0:
                    st['q'] = att[qs, :, HALO + r0:HALO + r0 + R, :]
                    st['lg'] = []
                kw = att[ks, :, pl.ds(HALO + r0 - DIL * w, R), :]
                p = jnp.sum(st['q'] * kw, axis=0)
                p = p + pltpu.roll(p, 64, 1)
                p = p + pltpu.roll(p, 32, 1)
                if first and r0 < DIL * w:
                    row = lax.broadcasted_iota(i32, (R, 128), 0) + blk * T
                    p = jnp.where(row + r0 >= DIL * w, p, -1e9 / scale)
                st['lg'].append(p)

            def softmax():
                lg = st['lg']
                m = functools.reduce(jnp.maximum, lg)
                e = [jnp.exp2((p - m) * (scale * 1.4426950408889634)) for p in lg]
                inv = pl.reciprocal(functools.reduce(jnp.add, e), approx=True)
                for w in range(W):
                    att[ps, w, r0:r0 + R, :] = e[w] * inv
            return [functools.partial(piece, w) for w in range(W)], softmax

        def av_pieces(ps, vs, o_s, c):
            r0 = c * 16
            st = {}

            def piece(j):
                if j == 0:
                    st['a'] = att[ps, :, r0:r0 + 16, :]
                a = st['a']
                acc = a[0] * att[vs, j, pl.ds(HALO + r0, 16), :]
                for w in range(1, W):
                    acc = acc + a[w] * att[vs, j, pl.ds(HALO + r0 - DIL * w, 16), :]
                o = pltpu.bitcast(acc.astype(bf16), i32)
                o_s[r0 // 2:r0 // 2 + 8, j * 128:(j + 1) * 128] = o
                pc.later(AVLAG, lambda: pc.pin(o))
            return [functools.partial(piece, j) for j in range(NG)]

        def ln1_piece(row0, dst, c):
            xn = _ln_packed(xs[pl.ds(row0 + c * 16, 16), :])
            dst[8 * c:8 * c + 8, :] = xn
            pc.pin(xn)

        if kind != 'last':
            aa = AA if kind == 'mid' else FAA
            for (qs, ks, ps, first, (t0, n)) in ((QA, KA, PA, True, LA), (QB, KB, PB, False, LB)):
                for c in range(NCH):
                    pcs, sm = logits_pieces(qs, ks, ps, c, first)
                    ts, dt = (t0 + c * n / NCH, n / NCH) if kind == 'mid' else FT[(0 if first else NCH) + c]
                    pc.spread(pcs, ts, dt)
                    pc.at(ts + dt + (LAG if kind == 'mid' else FLAG), sm)
            pc.spread([p for c in range(C // 16) for p in av_pieces(PA, VA, o_a, c)], *aa)
            n1b, n1n = (N1B, N1N) if kind == 'mid' else (FN1B, FN1N)
            pc.spread([functools.partial(ln1_piece, base + C, xn_b, c) for c in range(C // 16)], *n1b)
            pc.spread([functools.partial(ln1_piece, nbase, xn_n, c) for c in range(C // 16)], *n1n)
            att[KA, :, 0:HALO, :] = hk[...]
            att[VA, :, 0:HALO, :] = hv[...]
        if kind != 'first':
            pc.spread([p for c in range(C // 16) for p in av_pieces(PB, VB, o_b, c)], *AB)

        def proj(chain, part, half=None):
            slot = (QB if chain else QA) + part
            src = xn_b if chain else xn_a
            if half is None:
                xn, w_ref = _as_bf16(src[...]), wqkv_p.at[part]
            else:
                xn = _as_bf16(src[:, half * (D // 2):(half + 1) * (D // 2)])
                w_ref = wqkv_p.at[part, half * (D // 4):(half + 1) * (D // 4)]
            for j in range(NG):
                r = _dot(xn, w_ref, j)
                if half == 1:
                    r = r + att[slot, j, HALO:HALO + C, :]
                if part > 0 and half != 0:
                    if chain == 0:
                        att[QB + part, j, 0:HALO, :] = r[C - HALO:C]
                    else:
                        (hk if part == 1 else hv)[j] = r[C - HALO:C]
                pc.tile(r, slot, j, dur=1 if half is None else 0.5)

        def out_proj(chain):
            r0 = pbase + chain * C
            o = _as_bf16((o_b if chain else o_a)[...])
            for n in range(NG):
                if n % 2 == 0:
                    xr = xs[pl.ds(r0, C), n * 128:(n + 2) * 128]
                r = _dot(o, wo_p, n) + xr[:, (n % 2) * 128:(n % 2 + 1) * 128].astype(f32)
                pc.tile(r)
                xs[pl.ds(r0, C), n * 128:(n + 1) * 128] = r.astype(bf16)

        if kind == 'mid':
            proj(0, 0), proj(0, 1), out_proj(0), proj(1, 0), proj(1, 1), proj(0, 2), out_proj(1)
            xn_a[...] = xn_n[...]
            proj(1, 2)
        elif kind == 'first':
            proj(0, 0)
            kv_cps[0][0].wait()
            permute_xlu(1, 0, D // 2)
            proj(1, 0)
            kv_cps[0][1].wait()
            permute_xlu(1, D // 2, D // 2)
            proj(0, 1, 0), proj(1, 1, 0)
            kv_cps[1][0].wait()
            permute_xlu(2, 0, D // 2)
            proj(0, 1, 1), proj(1, 1, 1)
            kv_cps[1][1].wait()
            permute(2, 2 * rows, pc), permute(2, 3 * rows, pc)
            proj(0, 2, 0), proj(1, 2, 0)
            wo_cp.wait()
            pc.aux = wo_stage
            pc.spread([functools.partial(wo_stage_piece, j, g, g + 2)
                       for j in range(NG) for g in range(0, NG, 2)], *WOS)
            pc.spread([functools.partial(wo_gather_piece, jp, th, ah)
                       for jp in range(NG) for th in range(2) for ah in range(2)], *WOG)
            proj(0, 2, 1)
            xn_a[...] = xn_n[...]
            proj(1, 2, 1)
        else:
            out_proj(0), out_proj(1)
        assert not pc.events

    def _mlp_item():
        item = step - SKEW
        blk = item & (NB - 1)
        base = pl.multiple_of(blk * T, T)
        nbase = pl.multiple_of(((item + 1) & (NB - 1)) * T, T)

        pc = _Pacer(att, zero_ref[0])

        def ln_piece(row0, dst, c):
            xn = _ln_packed(xs[pl.ds(row0 + c * 16, 16), :])
            dst[8 * c:8 * c + 8, :] = xn
            pc.pin(xn, hard=True)

        pc.spread([functools.partial(ln_piece, base + C, xn2_b, c) for c in range(C // 16)], *N2B)
        pc.spread([functools.partial(ln_piece, nbase, xn2_a, c) for c in range(C // 16)], *N2A)

        def mish(h):
            ex = jnp.exp(jnp.minimum(h, 30.0))
            n = ex * (ex + 2.0)
            return (h * n * pl.reciprocal(n + 2.0, approx=True)).astype(bf16)

        def mlp1(xn):
            act = []
            for n in range(NF):
                r = _dot(pc.tie(xn), w1_v, n)
                pc.tile(r)
                act.append(mish(r + b1_v[n:n + 1, :].astype(f32)))
            return jnp.concatenate(act, axis=1)

        act_a = mlp1(_as_bf16(xn2_a[...]))
        act_b = mlp1(_as_bf16(xn2_b[...]))
        for act, r0 in ((act_a, base), (act_b, base + C)):
            for n in range(NG):
                if n % 2 == 0:
                    xr = xs[pl.ds(r0, C), n * 128:(n + 2) * 128]
                r = _dot(pc.tie(act), w2_v, n) + xr[:, (n % 2) * 128:(n % 2 + 1) * 128].astype(f32)
                pc.tile(r)
                xs[pl.ds(r0, C), n * 128:(n + 1) * 128] = r.astype(bf16)
                cuts = OUT_CUTS if r0 is not base else (NG,)
                if n + 1 in cuts:
                    n0 = ([0] + [c for c in cuts if c <= n])[-1]

                    @pl.when(item >= NITEM - NB)
                    def _():
                        out_copy(r0, n0 * 128, (n + 1 - n0) * 128).start()
        assert not pc.events

        @pl.when(item == NITEM - 1)
        def _():
            pltpu.make_async_copy(xs, out_hbm, sems.at[SEM_O]).wait()

    @pl.when((step <= SKEW + 1) | (step == NITEM + 1))
    def _():
        pl.when(step == 0)(prologue)
        pl.when(step == SKEW)(first_mlp_prep)
        for k in range(1, SKEW + 1):
            pl.when(step == k)(x_copy(k + 1).wait)

        @pl.when(step == SKEW + 1)
        def _():
            for k in range(SKEW + 2, NB + 1):
                x_copy(k).wait()

        pl.when(step == NITEM + 1)(functools.partial(attention, 'last'))

    pl.when(step >= SKEW)(_mlp_item)
    pl.when((step >= 1) & (step < NITEM))(functools.partial(attention, 'mid'))


@jax.jit
def pallas_interleave_layers__sliding_local_dilated__dense_activation_mish__prompt_kernel(A_x, A_wqkv, A_wo, B_x, B_w1, B_b1, B_w2):
    x = A_x.reshape(S, D)
    b1 = B_b1.reshape(NF, 128)
    out = pl.pallas_call(
        _kernel,
        grid=(NITEM + SKEW,),
        in_specs=[pl.BlockSpec(memory_space=pl.ANY)] * 6,
        out_specs=pl.BlockSpec(memory_space=pl.ANY),
        out_shape=jax.ShapeDtypeStruct((S, D), bf16),
        scratch_shapes=[
            pltpu.VMEM((3, D, D + RAWPAD), bf16), pltpu.VMEM((3, D // 2, D), i32),
            pltpu.VMEM((D, D + RAWPAD), bf16), pltpu.VMEM((NG, NG * PITCH + 72, 128), i32), pltpu.VMEM((NG, 128, 128), bf16),
            pltpu.VMEM((D // 2, D), i32),
            pltpu.VMEM((D, F), bf16), pltpu.VMEM((F, D), bf16), pltpu.VMEM((NF, 128), bf16),
            pltpu.VMEM((S, D), bf16), pltpu.VMEM((3, C // 2, D), i32),
            pltpu.VMEM((C // 2, D), i32), pltpu.VMEM((C // 2, D), i32),
            pltpu.VMEM((NSLOT, NG, AROWS, 128), f32),
            pltpu.VMEM((C // 2, D), i32), pltpu.VMEM((C // 2, D), i32),
            pltpu.VMEM((NG, HALO, 128), f32), pltpu.VMEM((NG, HALO, 128), f32),
            pltpu.SMEM((1,), i32),
            pltpu.SemaphoreType.DMA((NSEM,)),
        ],
        compiler_params=pltpu.CompilerParams(
            dimension_semantics=("arbitrary",), vmem_limit_bytes=100 * 1024 * 1024, disable_semaphore_checks=True),
        name="fused",
    )(x, b1, A_wqkv, A_wo, B_w1, B_w2)
    return out.reshape(1, S, D)
```
